```python
import jax
import jax.numpy as jnp

def _softmax(x, axis=-1):
    return jax.nn.softmax(x, axis=axis)
def _gelu(x):
    return jax.nn.gelu(x, approximate=True)
def _silu(x):
    return jax.nn.silu(x)
def _sigmoid(x):
    return jax.nn.sigmoid(x)
def _layernorm(x, axis=-1, eps=1e-5):
    m = jnp.mean(x, axis=axis, keepdims=True)
    v = jnp.var(x, axis=axis, keepdims=True)
    return (x - m) / jnp.sqrt(v + eps)
def _scatter_add(tgt, idx, src, axis=0):
    return tgt.at[idx].add(src)
def _segment_sum(src, seg, n):
    return jax.ops.segment_sum(src, seg, n)
class _Rng:
    def __init__(self, key):
        self._k = key
    def _next(self):
        self._k, sub = jax.random.split(self._k)
        return sub
    def normal(self, shape):
        return jax.random.normal(self._next(), shape, dtype=jnp.bfloat16)
    def randint(self, lo, hi, shape):
        return jax.random.randint(self._next(), shape, lo, hi, dtype=jnp.int32)
    def uniform(self, shape, lo=0.0, hi=1.0):
        return jax.random.uniform(self._next(), shape, jnp.bfloat16, lo, hi)
    def permutation(self, n):
        return jax.random.permutation(self._next(), n)


kernel_name = 'parallel_sum__linear_kernel_hedgehog__glu_gated_bilinear__prompt'

def _fwd_setup_inputs():
    _rng = _Rng(jax.random.key(int.from_bytes(__import__("os").urandom(4), "little")))
    _w = (lambda a: (lambda t: t.astype(jnp.bfloat16) if jnp.issubdtype(t.dtype, jnp.floating) else t)(jnp.asarray(a)))
    def _A_setup():
        B, S, D, H = 1, 2048, 512, 32
        Dh = D // H
        return {
            "x": _w((lambda *s: _rng.normal(s) * 0.05)(B, S, D)),
            "wqkv": _w((lambda *s: _rng.normal(s) * 0.05)(D, 3 * D)),
            "w_phi": _w((lambda *s: _rng.normal(s) * 0.05)(H, Dh, Dh) * (Dh ** -0.5)),
            "wo": _w((lambda *s: _rng.normal(s) * 0.05)(D, D)),
        }
    _A_in = _A_setup()

    def _B_setup():
        B, S, D, F = 1, 2048, 512, 1792
        return {
            "x": _w((lambda *s: _rng.normal(s) * 0.05)(B, S, D)),
            "w_gate": _w((lambda *s: _rng.normal(s) * 0.05)(D, F) * (D ** -0.5)),
            "w_up": _w((lambda *s: _rng.normal(s) * 0.05)(D, F) * (D ** -0.5)),
            "w_down": _w((lambda *s: _rng.normal(s) * 0.05)(F, D) * (F ** -0.5)),
        }
    _B_in = _B_setup()

    return {
        "A_x": _A_in["x"],
        "A_wqkv": _A_in["wqkv"],
        "A_w_phi": _A_in["w_phi"],
        "A_wo": _A_in["wo"],
        "B_x": _B_in["x"],
        "B_w_gate": _B_in["w_gate"],
        "B_w_up": _B_in["w_up"],
        "B_w_down": _B_in["w_down"],
    }

def _fwd_reference(A_x, A_wqkv, A_w_phi, A_wo, B_x, B_w_gate, B_w_up, B_w_down):
    def _A_ref(x, wqkv, w_phi, wo):
        B, S, D = x.shape
        H = 32; Dh = D // H
        qkv = (lambda x, *d: x.transpose(*d))((x @ wqkv).reshape(B, S, 3, H, Dh), 2, 0, 3, 1, 4)
        q, k, v = qkv[0], qkv[1], qkv[2]
        pq = jnp.einsum("bhsd,hdf->bhsf", q, w_phi)
        pk = jnp.einsum("bhsd,hdf->bhsf", k, w_phi)
        phi_q = jnp.concatenate([_softmax(pq, axis=-1), _softmax(-pq, axis=-1)], axis=-1)
        phi_k = jnp.concatenate([_softmax(pk, axis=-1), _softmax(-pk, axis=-1)], axis=-1)
        kv = jnp.einsum("bhsf,bhsd->bhfd", phi_k, v)
        z  = jnp.einsum("bhsf->bhf", phi_k)
        num = jnp.einsum("bhqf,bhfd->bhqd", phi_q, kv)
        den = jnp.einsum("bhqf,bhf->bhq", phi_q, z)[..., None] + 1e-6
        o = num / den
        return (lambda x, *d: x.transpose(*d))(o, 0, 2, 1, 3).reshape(B, S, D) @ wo

    def _B_ref(x, w_gate, w_up, w_down):
        g = jnp.einsum("bsd,df->bsf", x, w_gate)
        u = jnp.einsum("bsd,df->bsf", x, w_up)
        h = g * u
        return jnp.einsum("bsf,fd->bsd", h, w_down)

    x = A_x
    xn = _layernorm(x, axis=-1)
    return x + _A_ref(xn, A_wqkv, A_w_phi, A_wo) + _B_ref(xn, B_w_gate, B_w_up, B_w_down)


def setup_inputs():
    _inp = _fwd_setup_inputs()
    _gk = jax.random.fold_in(jax.random.key(int.from_bytes(__import__("os").urandom(4), "little")), 2**31 - 1)
    _shapes = [[1, 2048, 512]]
    _dtypes = ['bfloat16']
    _gks = jax.random.split(_gk, len(_shapes))
    _gs = [jax.random.normal(k, s, dtype=jnp.dtype(d)) * 0.05 for k, s, d in zip(_gks, _shapes, _dtypes)]
    _inp["grad_out"] = _gs[0]
    return _inp

def reference(A_x, A_wqkv, A_w_phi, A_wo, B_w_gate, B_w_up, B_w_down, B_x, grad_out):
    _const = dict(B_x=B_x)
    def _f(*_d):
        return _fwd_reference(**{'A_x': _d[0], 'A_wqkv': _d[1], 'A_w_phi': _d[2], 'A_wo': _d[3], 'B_w_gate': _d[4], 'B_w_up': _d[5], 'B_w_down': _d[6], **_const})
    _out, _vjp = jax.vjp(_f, A_x, A_wqkv, A_w_phi, A_wo, B_w_gate, B_w_up, B_w_down)
    _grads = _vjp(grad_out)
    _out0 = jnp.asarray(_out)
    return (_out0, *[jnp.asarray(_g) for _g in _grads])
```

```python
import functools
import jax
import jax.numpy as jnp
import jax.experimental.pallas as pl
import jax.experimental.pallas.tpu as pltpu

S, D, H, DH, F = 2048, 512, 32, 16, 1792
NG = 4
T = 256
NTILE = S // T
FC = 256
FA = 768
FB = F - FA
NB = FB // 128
BPI = NB // NTILE

UNROLL2 = 2
U1 = 1
f32 = jnp.float32
bf16 = jnp.bfloat16
NN = (((1,), (0,)), ((), ()))
NT = (((1,), (1,)), ((), ()))
TN = (((0,), (0,)), ((), ()))


def _dot(a, b, dn=NN):
    return jax.lax.dot_general(a, b, dn, preferred_element_type=f32)


def _dual_softmax(p):
    p3 = p.reshape(16, 8, p.shape[-1])
    mx = jnp.max(p3, axis=0, keepdims=True)
    mn = jnp.min(p3, axis=0, keepdims=True)
    ea = jnp.exp(p3 - mx)
    eb = jnp.exp(mn - p3)
    a = ea * (1.0 / jnp.sum(ea, axis=0, keepdims=True))
    b = eb * (1.0 / jnp.sum(eb, axis=0, keepdims=True))
    return a, b


def _dual_softmax_bwd(a, b, da, db):
    ta = a * da
    tb = b * db
    return (ta - a * jnp.sum(ta, axis=0, keepdims=True)) - (tb - b * jnp.sum(tb, axis=0, keepdims=True))


def _iota(shape, dim):
    return jax.lax.broadcasted_iota(jnp.int32, shape, dim)


def kernel(x_hbm, wqkv_hbm, wphi_hbm, wo_hbm, wg_hbm, wu_hbm, wd_hbm, dout_hbm,
           out_hbm, dx_hbm, dwqkv_hbm, dwphi_hbm, dwo_hbm, dwg_hbm, dwu_hbm, dwd_hbm,
           x_v, dout_v, wqkv_v, wphi_v, wo_v, wg_v, wu_v, wd_v,
           out_v, dx_v, dwqkv_v, dwphi_v, dwo_v, dwg_v, dwu_v, dwd_v,
           wT_s, wop_s, pmT_s, xn_s, xnT_s, rstd_s, phik_s, vT_s, kvT_s, kvz_s, kv_s, zc_s,
           dkvT_s, dkvTm_s, dkv_s, dzc_s, gT_s, dwo_s, dwg_s, dwu_s, dwd_s, out_s, dxn_s,
           h_s, dgu_s, aphi_s,
           sem_w, sem_x, sem_do, sem_out, sem_dx, sem_a, sem_b, sem_e):
    cp = pltpu.make_async_copy

    def mo(v, m):
        return v if isinstance(v, int) else pl.multiple_of(v, m)

    def tile_rows(t):
        if isinstance(t, int):
            return pl.ds(t * T, T)
        return pl.ds(pl.multiple_of(t * T, T), T)

    c_wphi = cp(wphi_hbm, wphi_v, sem_w.at[0])
    c_wk = cp(wqkv_hbm.at[:, 512:1024], wqkv_v.at[:, 512:1024], sem_w.at[1])
    c_wv = cp(wqkv_hbm.at[:, 1024:1536], wqkv_v.at[:, 1024:1536], sem_w.at[10])
    c_wq = cp(wqkv_hbm.at[:, 0:512], wqkv_v.at[:, 0:512], sem_w.at[2])
    c_wo = cp(wo_hbm, wo_v, sem_w.at[3])
    c_wgA = cp(wg_hbm.at[:, 0:FA], wg_v.at[:, 0:FA], sem_w.at[4])
    c_wuA = cp(wu_hbm.at[:, 0:FA], wu_v.at[:, 0:FA], sem_w.at[5])
    c_wdA = cp(wd_hbm.at[0:FA, :], wd_v.at[0:FA, :], sem_w.at[6])
    c_wgB = cp(wg_hbm.at[:, FA:F], wg_v.at[:, FA:F], sem_w.at[7])
    c_wuB = cp(wu_hbm.at[:, FA:F], wu_v.at[:, FA:F], sem_w.at[8])
    c_wdB = cp(wd_hbm.at[FA:F, :], wd_v.at[FA:F, :], sem_w.at[9])

    def c_x(t):
        return cp(x_hbm.at[tile_rows(t), :], x_v.at[tile_rows(t), :], sem_x.at[t])

    def c_do(t):
        return cp(dout_hbm.at[tile_rows(t), :], dout_v.at[tile_rows(t), :], sem_do.at[t])

    c_wphi.start()
    c_x(0).start()
    c_x(1).start()
    c_wk.start()
    c_wv.start()

    def o_out(t):
        return cp(out_v.at[tile_rows(t), :], out_hbm.at[tile_rows(t), :], sem_out.at[t])

    def o_dx(t):
        return cp(dx_v.at[tile_rows(t), :], dx_hbm.at[tile_rows(t), :], sem_dx.at[t])

    RA = D // NTILE
    RD = FA // NTILE

    def o_a(t):
        ra = pl.ds(mo(t * RA, RA), RA)
        rd = pl.ds(mo(t * RD, RD), RD)
        return (cp(dwg_v.at[ra, 0:FA], dwg_hbm.at[ra, 0:FA], sem_a.at[0, t]),
                cp(dwu_v.at[ra, 0:FA], dwu_hbm.at[ra, 0:FA], sem_a.at[1, t]),
                cp(dwd_v.at[rd, :], dwd_hbm.at[rd, :], sem_a.at[2, t]))

    def o_b(t):
        cb = pl.ds(mo(FA + t * (128 * BPI), 128), 128 * BPI)
        return (cp(dwg_v.at[:, cb], dwg_hbm.at[:, cb], sem_b.at[0, t]),
                cp(dwu_v.at[:, cb], dwu_hbm.at[:, cb], sem_b.at[1, t]),
                cp(dwd_v.at[cb, :], dwd_hbm.at[cb, :], sem_b.at[2, t]))

    o_wq = cp(dwqkv_v.at[:, 0:512], dwqkv_hbm.at[:, 0:512], sem_e.at[0])
    o_wkv = cp(dwqkv_v.at[:, 512:1536], dwqkv_hbm.at[:, 512:1536], sem_e.at[1])
    o_wo = cp(dwo_v, dwo_hbm, sem_e.at[2])
    o_wphi = cp(dwphi_v, dwphi_hbm, sem_e.at[3])

    r_i = _iota((128, 128), 0)
    c_i = _iota((128, 128), 1)
    head_mask = (r_i % 8) == (c_i // 16)
    permT = jnp.where(head_mask & ((r_i // 8) == (c_i % 16)), 1.0, 0.0).astype(bf16)
    hsel = jnp.where(_iota((32, 512), 0) == (_iota((32, 512), 1) // 16), 1.0, 0.0).astype(bf16)
    dmask = (_iota((256, 512), 0) // 16) == (_iota((256, 512), 1) % 16)
    rsel = jnp.where((_iota((128, 256), 0) // 8) == (_iota((128, 256), 1) % 16), 1.0, 0.0).astype(bf16)
    hm4 = (_iota((128, 512), 0) % 8) == ((_iota((128, 512), 1) // 16) % 8)
    ones16 = jnp.ones((16, T), bf16)

    def fold(part):
        for g in range(NG):
            m = pmT_s[:, g * 128:(g + 1) * 128] if part < 2 else permT
            cs = slice(part * 512 + g * 128, part * 512 + (g + 1) * 128)
            wT_s[cs, :] = _dot(m, wqkv_v[:, cs], NT).astype(bf16)

    def ffn_dh(c, dout):
        return _dot(dout, wd_v[c * FC:(c + 1) * FC, :], NT)

    def ffn_gu(c, xn):
        cs = slice(c * FC, (c + 1) * FC)
        return _dot(xn, wg_v[:, cs]), _dot(xn, wu_v[:, cs])

    def ffn_elem(g_, u_, dh):
        return (g_ * u_).astype(bf16), (dh * u_).astype(bf16), (dh * g_).astype(bf16)

    def ffn_mm(c, h, dg, du):
        cs = slice(c * FC, (c + 1) * FC)
        o_c = _dot(h, wd_v[cs, :])
        d_c = _dot(dg, wg_v[:, cs], NT) + _dot(du, wu_v[:, cs], NT)
        return o_c, d_c

    def layernorm(t):
        LB = 32
        for r in range(T // LB):
            rows = pl.ds(mo(t * T + r * LB, LB), LB)
            x = x_v[rows, :].astype(f32)
            mu = jnp.mean(x, axis=-1, keepdims=True)
            xc = x - mu
            var = jnp.mean(xc * xc, axis=-1, keepdims=True)
            rstd = jax.lax.rsqrt(var + 1e-5)
            xn_s[rows, :] = (xc * rstd).astype(bf16)
            rstd_s[rows, :] = rstd
        rows = tile_rows(t)
        xn = xn_s[rows, :]
        xnT_s[:, rows] = xn.T
        return xn

    def k_soft(t, pkv, g):
        a, b = _dual_softmax(pkv[g * 128:(g + 1) * 128])
        phi = jnp.concatenate([a.reshape(128, T), b.reshape(128, T)], axis=0).astype(bf16)
        phik_s[t, g] = phi
        v = pkv[512 + g * 128: 512 + (g + 1) * 128].astype(bf16)
        vT_s[t, g] = v
        return phi, v

    def k_acc(g, phi, v, first=False):
        r = _dot(jnp.concatenate([v, ones16], axis=0), phi, NT)
        if first:
            kvT_s[g] = r
        else:
            kvT_s[g] += r

    def phase1(t, nxt, extra=None):
        rows = tile_rows(t)
        if nxt is not None:
            xn1 = layernorm(nxt)
        dout = dout_v[rows, :]
        xn = xn_s[rows, :]
        xnT = xnT_s[:, rows]
        nchunk = FA // FC
        st = (ffn_dh(0, dout),) + ffn_gu(0, xn)
        if extra is not None:
            extra[0]()
        if nxt is not None:
            pk = _dot(wT_s[512:1536, :], xn1, NT)
        o_acc = x_v[rows, :].astype(f32)
        d_acc = None
        pv = []
        for c in range(nchunk):
            cs = slice(c * FC, (c + 1) * FC)
            dh, g_, u_ = st
            h, dg, du = ffn_elem(g_, u_, dh)
            if nxt is not None:
                gs = ([0, 1], [2, 3], [])[c]
                pv = [(g, k_soft(nxt, pk, g)) for g in gs]
            if c + 1 < nchunk:
                st = (ffn_dh(c + 1, dout),) + ffn_gu(c + 1, xn)
            if extra is not None and c == 0:
                extra[1]()
            dwg_s[:, cs] += _dot(xnT, dg)
            dwu_s[:, cs] += _dot(xnT, du)
            dwd_s[cs, :] += _dot(h, dout, TN)
            for g, (phi, v) in pv:
                k_acc(g, phi, v)
            o_c, d_c = ffn_mm(c, h, dg, du)
            o_acc = o_acc + o_c
            d_acc = d_c if d_acc is None else d_acc + d_c
        out_s[rows, :] = o_acc
        dxn_s[rows, :] = d_acc

    rr = _iota((144, 256), 0)
    cc = _iota((144, 256), 1)
    m144 = ((rr % 8) == (cc % 8)) & (rr < 136)

    def finish(acc_s, accm_s, accmT_s, col_s):
        for g in range(NG):
            m = jnp.where(m144, acc_s[g], 0.0)
            accm_s[g] = m.astype(bf16)
            mT = m.T
            accmT_s[g] = mT[:, 0:128].astype(bf16)
            col_s[g] = jnp.broadcast_to(jnp.sum(mT[:, 128:144], axis=1, keepdims=True), (256, 128))

    dwg_s[...] = jnp.zeros_like(dwg_s)
    dwu_s[...] = jnp.zeros_like(dwu_s)
    dwd_s[...] = jnp.zeros_like(dwd_s)
    dkvT_s[...] = jnp.zeros_like(dkvT_s)
    gT_s[...] = jnp.zeros_like(gT_s)
    dwo_s[...] = jnp.zeros_like(dwo_s)
    c_wphi.wait()
    w3 = wphi_v[...].reshape(256, 32)
    ym = jnp.where(dmask, _dot(w3, hsel), 0.0).astype(bf16)
    pmT_s[...] = jnp.where(hm4, _dot(rsel, ym), 0.0).astype(bf16)
    c_x(0).wait()
    xn0 = layernorm(0)
    c_wk.wait()
    c_wv.wait()
    c_x(1).wait()
    c_wdA.start()
    c_wgA.start()
    c_wuA.start()
    c_do(0).start()
    c_x(2).start()
    xn1 = layernorm(1)
    fold(1)
    fold(2)
    pk0 = _dot(wT_s[512:1536, :], xn0, NT)
    pv0 = [k_soft(0, pk0, g) for g in range(NG)]
    pk1 = _dot(wT_s[512:1536, :], xn1, NT)
    for g in range(NG):
        k_acc(g, *pv0[g], first=True)
    for g in range(NG):
        k_acc(g, *k_soft(1, pk1, g))
    c_wdA.wait()
    c_wgA.wait()
    c_wuA.wait()
    c_do(1).start()
    c_do(2).start()
    for t in range(3, NTILE):
        c_x(t).start()
        c_do(t).start()
    c_wq.start()
    c_wo.start()
    c_wgB.start()
    c_wuB.start()
    c_wdB.start()

    def p1_body(i, carry):
        ts = [i * U1 + k for k in range(U1)]
        for t in ts:
            c_do(t).wait()
            c_x(t + 2).wait()
        for t in ts:
            phase1(t, t + 2)
        return carry

    jax.lax.fori_loop(0, (NTILE - 2) // U1, p1_body, 0)
    c_do(NTILE - 2).wait()
    c_do(NTILE - 1).wait()

    c_wq.wait()
    c_wo.wait()

    def extra0():
        finish(kvT_s, kvz_s, kv_s, zc_s)

    def extra1():
        fold(0)
        for g in range(NG):
            wop_s[g * 128:(g + 1) * 128, :] = _dot(permT, wo_v[g * 128:(g + 1) * 128, :]).astype(bf16)

    phase1(NTILE - 2, None, (extra0, extra1))
    phase1(NTILE - 1, None)
    c_wgB.wait()
    c_wuB.wait()
    c_wdB.wait()

    c0 = FA // FC

    def phase2(t, carry):
        rows = tile_rows(t)
        xn = xn_s[rows, :]
        dout = dout_v[rows, :]
        acc = {}

        def ffn1(c):
            return (ffn_dh(c, dout),) + ffn_gu(c, xn)

        def elem(c, st):
            dh, g_, u_ = st
            h, dg, du = ffn_elem(g_, u_, dh)
            for j in range(FC // 128):
                blk = (c - c0) * (FC // 128) + j
                js = slice(j * 128, (j + 1) * 128)
                h_s[blk, rows, :] = h[:, js]
                dgu_s[blk, rows, 0:128] = dg[:, js]
                dgu_s[blk, rows, 128:256] = du[:, js]
            return h, dg, du

        def mm(c, e):
            o_c, d_c = ffn_mm(c, *e)
            acc['o'] = o_c + acc['o'] if 'o' in acc else o_c
            acc['d'] = d_c + acc['d'] if 'd' in acc else d_c

        pq = _dot(wT_s[0:512, :], xn, NT)
        ab = [_dual_softmax(pq[g * 128:(g + 1) * 128]) for g in range(NG)]
        phis = [jnp.concatenate([a.reshape(128, T), b.reshape(128, T)], axis=0).astype(bf16) for a, b in ab]
        doT = _dot(wop_s[...], dout, NT)
        st0 = ffn1(c0)
        nds = [_dot(kvz_s[g], phis[g]) for g in range(NG)]
        e0 = elem(c0, st0)
        oTs, dnums, ddens = [], [], []
        for g in range(NG):
            nd = nds[g]
            rden = 1.0 / (nd[128:136] + 1e-6)
            o3 = nd[0:128].reshape(16, 8, T) * rden[None]
            do3 = doT[g * 128:(g + 1) * 128].reshape(16, 8, T)
            dnums.append((do3 * rden[None]).reshape(128, T).astype(bf16))
            ddens.append(-jnp.sum(do3 * o3, axis=0) * rden)
            oTs.append(o3.reshape(128, T).astype(bf16))
        st1 = ffn1(c0 + 1)
        dphis = [_dot(kv_s[g], dnums[g]) for g in range(NG)]
        dpqs = []
        for g in range(NG):
            zc = jnp.concatenate([zc_s[g]] * (T // 128), axis=1).reshape(32, 8, T)
            dphi = dphis[g].reshape(32, 8, T) + zc * ddens[g][None]
            a, b = ab[g]
            dp = _dual_softmax_bwd(a, b, dphi[0:16], dphi[16:32])
            dpqs.append(dp.reshape(128, T).astype(bf16))
        dpq = jnp.concatenate(dpqs, axis=0)
        mm(c0, e0)
        oT = jnp.concatenate(oTs, axis=0)
        for g in range(NG):
            dd16 = jnp.concatenate([ddens[g], jnp.zeros_like(ddens[g])], axis=0).astype(bf16)
            dkvT_s[g] += _dot(jnp.concatenate([dnums[g], dd16], axis=0), phis[g], NT)
        e1 = elem(c0 + 1, st1)
        dwo_s[...] += _dot(oT, dout)
        acc['o'] = acc['o'] + _dot(oT, wop_s[...], TN)
        st2 = ffn1(c0 + 2)
        ra = pl.ds(pl.multiple_of(t * RA, RA), RA)
        rd = pl.ds(pl.multiple_of(t * RD, RD), RD)
        dwg_v[ra, 0:FA] = dwg_s[ra, :].astype(bf16)
        dwu_v[ra, 0:FA] = dwu_s[ra, :].astype(bf16)
        dwd_v[rd, :] = dwd_s[rd, :].astype(bf16)
        mm(c0 + 1, e1)
        e2 = elem(c0 + 2, st2)
        st3 = ffn1(c0 + 3)
        mm(c0 + 2, e2)
        e3 = elem(c0 + 3, st3)
        gT_s[0:512, :] += _dot(dpq, xn)
        mm(c0 + 3, e3)
        out_v[rows, :] = (out_s[rows, :] + acc['o']).astype(bf16)
        dxn_s[rows, :] += acc['d'] + _dot(dpq, wT_s[0:512, :], TN)
        return carry

    jax.lax.fori_loop(0, NTILE, phase2, 0, unroll=UNROLL2)
    for t in range(NTILE):
        for cpy in o_a(t):
            cpy.start()
        o_out(t).start()

    finish(dkvT_s, dkvTm_s, dkv_s, dzc_s)

    def unfold(part):
        for g in range(NG):
            m = pmT_s[:, g * 128:(g + 1) * 128] if part < 2 else permT
            cs = slice(part * 512 + g * 128, part * 512 + (g + 1) * 128)
            gblk = gT_s[cs, :].astype(bf16)
            dwqkv_v[:, cs] = _dot(gblk, m, TN).astype(bf16)
            if part == 0:
                aphi_s[:, g * 128:(g + 1) * 128] = _dot(gblk, wqkv_v[:, cs])
            elif part == 1:
                aphi_s[:, g * 128:(g + 1) * 128] += _dot(gblk, wqkv_v[:, cs])
        if part == 1:
            accm = jnp.where(hm4, aphi_s[...], 0.0).astype(bf16)
            z = jnp.where(dmask, _dot(rsel, accm, TN), 0.0).astype(bf16)
            dwphi_v[...] = _dot(z, hsel, NT).astype(bf16).reshape(16, 16, 32)

    unfold(0)
    for g in range(NG):
        dwo_v[g * 128:(g + 1) * 128, :] = _dot(permT, dwo_s[g * 128:(g + 1) * 128, :].astype(bf16), TN).astype(bf16)
    o_wq.start()
    o_wo.start()

    def wgrad_gu(t):
        for j in range(BPI):
            blk = t * BPI + j
            cb = pl.ds(mo(FA + blk * 128, 128), 128)
            dgu = _dot(xnT_s[...], dgu_s[blk])
            dwg_v[:, cb] = dgu[:, 0:128].astype(bf16)
            dwu_v[:, cb] = dgu[:, 128:256].astype(bf16)

    def wgrad_d(t):
        for j in range(BPI):
            blk = t * BPI + j
            cb = pl.ds(mo(FA + blk * 128, 128), 128)
            dwd_v[cb, :] = _dot(h_s[blk], dout_v[...], TN).astype(bf16)

    def phase3(t, last):
        rows = tile_rows(t)
        xn = xn_s[rows, :]
        dout = dout_v[rows, :]
        phis = [phik_s[t, g] for g in range(NG)]
        dphis = [_dot(dkv_s[g], vT_s[t, g]) for g in range(NG)]
        dps = []
        for g in range(NG):
            phif = phis[g].astype(f32).reshape(32, 8, T)
            dzc = jnp.concatenate([dzc_s[g]] * (T // 128), axis=1)
            dphi = (dphis[g] + dzc).reshape(32, 8, T)
            dp = _dual_softmax_bwd(phif[0:16], phif[16:32], dphi[0:16], dphi[16:32])
            dps.append(dp.reshape(128, T).astype(bf16))
        dvs = [_dot(dkvTm_s[g, 0:128, :], phis[g]).astype(bf16) for g in range(NG)]
        wgrad_d(t)
        dpkv = jnp.concatenate(dps + dvs, axis=0)
        dxn = dxn_s[rows, :] + _dot(dpkv, wT_s[512:1536, :], TN)
        xnf = xn.astype(f32)
        m1 = jnp.mean(dxn, axis=-1, keepdims=True)
        m2 = jnp.mean(dxn * xnf, axis=-1, keepdims=True)
        dx = rstd_s[rows, :] * (dxn - m1 - xnf * m2) + dout.astype(f32)
        dx_v[rows, :] = dx.astype(bf16)
        gT_s[512:1536, :] += _dot(dpkv, xn)
        if last:
            ob = o_b(t)
            o_dx(t).start()
            ob[2].start()
            unfold(1)
            unfold(2)
            o_wkv.start()
            o_wphi.start()
            wgrad_gu(t)
            ob[0].start()
            ob[1].start()
        else:
            wgrad_gu(t)
            o_dx(t).start()
            for cpy in o_b(t):
                cpy.start()

    def p3_body(t, carry):
        phase3(t, False)
        return carry

    jax.lax.fori_loop(0, NTILE - 1, p3_body, 0)
    phase3(NTILE - 1, True)

    for t in range(NTILE):
        o_out(t).wait()
        for cpy in o_a(t):
            cpy.wait()
    o_wq.wait()
    o_wo.wait()
    for t in range(NTILE):
        o_dx(t).wait()
    o_wkv.wait()
    o_wphi.wait()
    for t in range(NTILE):
        for cpy in o_b(t):
            cpy.wait()


@jax.jit
def pallas_parallel_sum__linear_kernel_hedgehog__glu_gated_bilinear__prompt_kernel(A_x, A_wqkv, A_w_phi, A_wo, B_x, B_w_gate, B_w_up, B_w_down, grad_out):
    x = A_x.reshape(S, D)
    dout = grad_out.reshape(S, D)
    wphi = jnp.transpose(A_w_phi, (1, 2, 0))
    sds = jax.ShapeDtypeStruct
    io_shapes = ((S, D), (S, D), (D, 3 * D), (DH, DH, H), (D, D), (D, F), (D, F), (F, D))
    any_spec = pl.BlockSpec(memory_space=pl.ANY)
    dma = pltpu.SemaphoreType.DMA
    outs = pl.pallas_call(
        kernel,
        out_shape=tuple(sds(s, bf16) for s in io_shapes),
        in_specs=[any_spec] * 8,
        out_specs=tuple([any_spec] * 8),
        scratch_shapes=[pltpu.VMEM(s, bf16) for s in io_shapes] + [pltpu.VMEM(s, bf16) for s in io_shapes] + [
            pltpu.VMEM((3 * D, D), bf16),
            pltpu.VMEM((D, D), bf16),
            pltpu.VMEM((128, 512), bf16),
            pltpu.VMEM((S, D), bf16),
            pltpu.VMEM((D, S), bf16),
            pltpu.VMEM((S, 1), f32),
            pltpu.VMEM((NTILE, NG, 256, T), bf16),
            pltpu.VMEM((NTILE, NG, 128, T), bf16),
            pltpu.VMEM((NG, 144, 256), f32),
            pltpu.VMEM((NG, 144, 256), bf16),
            pltpu.VMEM((NG, 256, 128), bf16),
            pltpu.VMEM((NG, 256, 128), f32),
            pltpu.VMEM((NG, 144, 256), f32),
            pltpu.VMEM((NG, 144, 256), bf16),
            pltpu.VMEM((NG, 256, 128), bf16),
            pltpu.VMEM((NG, 256, 128), f32),
            pltpu.VMEM((3 * D, D), f32),
            pltpu.VMEM((D, D), f32),
            pltpu.VMEM((D, FA), f32),
            pltpu.VMEM((D, FA), f32),
            pltpu.VMEM((FA, D), f32),
            pltpu.VMEM((S, D), f32),
            pltpu.VMEM((S, D), f32),
            pltpu.VMEM((NB, S, 128), bf16),
            pltpu.VMEM((NB, S, 256), bf16),
            pltpu.VMEM((128, 512), f32),
            dma((11,)), dma((NTILE,)), dma((NTILE,)), dma((NTILE,)), dma((NTILE,)),
            dma((3, NTILE)), dma((3, NTILE)), dma((4,)),
        ],
        compiler_params=pltpu.CompilerParams(vmem_limit_bytes=110 * 1024 * 1024),
    )(x, A_wqkv, wphi, A_wo, B_w_gate, B_w_up, B_w_down, dout)
    out, dx, dwqkv, dwphi, dwo, dwg, dwu, dwd = outs
    return (out.reshape(1, S, D), dx.reshape(1, S, D), dwqkv, jnp.transpose(dwphi, (2, 0, 1)), dwo, dwg, dwu, dwd)
```

```python
import functools
import jax
import jax.numpy as jnp
import jax.experimental.pallas as pl
import jax.experimental.pallas.tpu as pltpu

S, D, H, DH, F = 2048, 512, 32, 16, 1792
NG = 4
T = 256
NTILE = S // T
FC = 256
FA = 768
FB = F - FA
NB = FB // 128
BPI = NB // NTILE

UNROLL2 = 2
U1 = 1
SPLIT = 128
f32 = jnp.float32
bf16 = jnp.bfloat16
NN = (((1,), (0,)), ((), ()))
NT = (((1,), (1,)), ((), ()))
TN = (((0,), (0,)), ((), ()))


def _dot(a, b, dn=NN):
    return jax.lax.dot_general(a, b, dn, preferred_element_type=f32)


def _dual_softmax(p):
    p3 = p.reshape(16, 8, p.shape[-1])
    mx = jnp.max(p3, axis=0, keepdims=True)
    mn = jnp.min(p3, axis=0, keepdims=True)
    ea = jnp.exp(p3 - mx)
    eb = jnp.exp(mn - p3)
    a = ea * (1.0 / jnp.sum(ea, axis=0, keepdims=True))
    b = eb * (1.0 / jnp.sum(eb, axis=0, keepdims=True))
    return a, b


def _dual_softmax_bwd(a, b, da, db):
    ta = a * da
    tb = b * db
    return (ta - a * jnp.sum(ta, axis=0, keepdims=True)) - (tb - b * jnp.sum(tb, axis=0, keepdims=True))


class _Packed:
    def __init__(self, ref):
        self.ref = ref

    def _idx(self, idx):
        if idx is Ellipsis:
            return idx
        if not isinstance(idx, tuple):
            idx = (idx,)
        nd = len(self.ref.shape)
        idx = list(idx) + [slice(None)] * (nd - len(idx))
        r = idx[nd - 2]
        if isinstance(r, slice):
            r = slice(None if r.start is None else r.start // 2, None if r.stop is None else r.stop // 2)
        elif isinstance(r.start, int):
            r = pl.ds(r.start // 2, r.size // 2)
        else:
            r = pl.ds(pl.multiple_of(r.start // 2, r.size // 2), r.size // 2)
        idx[nd - 2] = r
        return tuple(idx)

    def view(self, *idx):
        return self.ref.at[self._idx(idx)] if idx else self.ref

    def __getitem__(self, idx):
        return pltpu.bitcast(self.ref[self._idx(idx)], bf16)

    def __setitem__(self, idx, v):
        self.ref[self._idx(idx)] = pltpu.bitcast(v, jnp.uint32)


def _iota(shape, dim):
    return jax.lax.broadcasted_iota(jnp.int32, shape, dim)


def kernel(x_hbm, wqkv_hbm, wphi_hbm, wo_hbm, wg_hbm, wu_hbm, wd_hbm, dout_hbm,
           out_hbm, dx_hbm, dwqkv_hbm, dwphi_hbm, dwo_hbm, dwg_hbm, dwu_hbm, dwd_hbm,
           x_v, dout_v, wqkv_v, wphi_v, wo_v, wg_v, wu_v, wd_v,
           out_v, dx_v, dwqkv_v, dwphi_v, dwo_v, dwg_v, dwu_v, dwd_v,
           wT_s, wop_s, pmT_s, xn_s, xnT_s, rstd_s, phik_s, vT_s, kvT_s, kvz_s, kv_s, zc_s,
           dkvT_s, dkvTm_s, dkv_s, dzc_s, gT_s, dwo_s, dwg_s, dwu_s, dwd_s, out_s, dxn_s,
           h_s, dgu_s, aphi_s,
           sem_w, sem_x, sem_do, sem_out, sem_dx, sem_a, sem_b, sem_e):
    (wT_s, wop_s, pmT_s, xn_s, xnT_s, phik_s, vT_s, kvz_s, kv_s, dkvTm_s, dkv_s, h_s, dgu_s,
     x_v, dout_v, wqkv_v, wo_v, wg_v, wu_v, wd_v, out_v, dx_v, dwqkv_v, dwo_v, dwg_v, dwu_v, dwd_v) = map(_Packed, (
         wT_s, wop_s, pmT_s, xn_s, xnT_s, phik_s, vT_s, kvz_s, kv_s, dkvTm_s, dkv_s, h_s, dgu_s,
         x_v, dout_v, wqkv_v, wo_v, wg_v, wu_v, wd_v, out_v, dx_v, dwqkv_v, dwo_v, dwg_v, dwu_v, dwd_v))
    (x_hbm, dout_hbm, wqkv_hbm, wo_hbm, wg_hbm, wu_hbm, wd_hbm,
     out_hbm, dx_hbm, dwqkv_hbm, dwo_hbm, dwg_hbm, dwu_hbm, dwd_hbm) = [
         _Packed(r.bitcast(jnp.uint32)) for r in (
             x_hbm, dout_hbm, wqkv_hbm, wo_hbm, wg_hbm, wu_hbm, wd_hbm,
             out_hbm, dx_hbm, dwqkv_hbm, dwo_hbm, dwg_hbm, dwu_hbm, dwd_hbm)]
    ALL = slice(None)

    def cp(src, dst, sem, *idx):
        return pltpu.make_async_copy(src.view(*idx), dst.view(*idx), sem)

    def mo(v, m):
        return v if isinstance(v, int) else pl.multiple_of(v, m)

    def tile_rows(t):
        if isinstance(t, int):
            return pl.ds(t * T, T)
        return pl.ds(pl.multiple_of(t * T, T), T)

    c_wphi = pltpu.make_async_copy(wphi_hbm, wphi_v, sem_w.at[0])
    c_wk = cp(wqkv_hbm, wqkv_v, sem_w.at[1], ALL, slice(512, 1024))
    c_wv = cp(wqkv_hbm, wqkv_v, sem_w.at[10], ALL, slice(1024, 1536))
    c_wq = cp(wqkv_hbm, wqkv_v, sem_w.at[2], ALL, slice(0, 512))
    c_wo = cp(wo_hbm, wo_v, sem_w.at[3])
    c_wgA = cp(wg_hbm, wg_v, sem_w.at[4], ALL, slice(0, FA))
    c_wuA = cp(wu_hbm, wu_v, sem_w.at[5], ALL, slice(0, FA))
    c_wdA = cp(wd_hbm, wd_v, sem_w.at[6], slice(0, FA), ALL)
    c_wgB = cp(wg_hbm, wg_v, sem_w.at[7], ALL, slice(FA, F))
    c_wuB = cp(wu_hbm, wu_v, sem_w.at[8], ALL, slice(FA, F))
    c_wdB = cp(wd_hbm, wd_v, sem_w.at[9], slice(FA, F), ALL)

    def c_x(t):
        return cp(x_hbm, x_v, sem_x.at[t], tile_rows(t), ALL)

    def c_do(t):
        return cp(dout_hbm, dout_v, sem_do.at[t], tile_rows(t), ALL)

    c_wphi.start()
    c_x(0).start()
    c_wk.start()

    o_out = cp(out_v, out_hbm, sem_out.at[0])

    def o_dx(t):
        return cp(dx_v, dx_hbm, sem_dx.at[t], tile_rows(t), ALL)

    RA = D // NTILE
    RD = FA // NTILE

    o_a = (cp(dwg_v, dwg_hbm, sem_out.at[1], ALL, slice(0, FA)),
           cp(dwu_v, dwu_hbm, sem_out.at[2], ALL, slice(0, FA)),
           cp(dwd_v, dwd_hbm, sem_out.at[3], slice(0, FA), ALL))

    def o_b(t):
        cb = pl.ds(mo(FA + t * (128 * BPI), 128), 128 * BPI)
        return (cp(dwg_v, dwg_hbm, sem_b.at[0, t], ALL, cb),
                cp(dwu_v, dwu_hbm, sem_b.at[1, t], ALL, cb),
                cp(dwd_v, dwd_hbm, sem_b.at[2, t], cb, ALL))

    o_wq = cp(dwqkv_v, dwqkv_hbm, sem_e.at[0], ALL, slice(0, 512))
    o_wkv = cp(dwqkv_v, dwqkv_hbm, sem_e.at[1], ALL, slice(512, 1536))
    o_wo = cp(dwo_v, dwo_hbm, sem_e.at[2])
    o_wphi = pltpu.make_async_copy(dwphi_v, dwphi_hbm, sem_e.at[3])

    r_i = _iota((128, 128), 0)
    c_i = _iota((128, 128), 1)
    head_mask = (r_i % 8) == (c_i // 16)
    permT = jnp.where(head_mask & ((r_i // 8) == (c_i % 16)), 1.0, 0.0).astype(bf16)
    hsel = jnp.where(_iota((32, 512), 0) == (_iota((32, 512), 1) // 16), 1.0, 0.0).astype(bf16)
    dmask = (_iota((256, 512), 0) // 16) == (_iota((256, 512), 1) % 16)
    rsel = jnp.where((_iota((128, 256), 0) // 8) == (_iota((128, 256), 1) % 16), 1.0, 0.0).astype(bf16)
    hm4 = (_iota((128, 512), 0) % 8) == ((_iota((128, 512), 1) // 16) % 8)
    ones16 = jnp.ones((16, T), bf16)

    def fold(part):
        for g in range(NG):
            m = pmT_s[:, g * 128:(g + 1) * 128] if part < 2 else permT
            cs = slice(part * 512 + g * 128, part * 512 + (g + 1) * 128)
            wT_s[cs, :] = _dot(m, wqkv_v[:, cs], NT).astype(bf16)

    def w_g(c):
        return wg_v[:, c * FC:(c + 1) * FC]

    def w_u(c):
        return wu_v[:, c * FC:(c + 1) * FC]

    def w_d(c):
        return wd_v[c * FC:(c + 1) * FC, :]

    def ffn_dh(c, dout):
        return _dot(dout, w_d(c), NT)

    def ffn_gu(c, xn):
        return _dot(xn, w_g(c)), _dot(xn, w_u(c))

    def ffn_elem(g_, u_, dh):
        return (g_ * u_).astype(bf16), (dh * u_).astype(bf16), (dh * g_).astype(bf16)

    def ffn_mm(c, h, dg, du):
        o_c = _dot(h, w_d(c))
        d_c = _dot(dg, w_g(c), NT) + _dot(du, w_u(c), NT)
        return o_c, d_c

    def layernorm(t):
        LB = 32
        for r in range(T // LB):
            rows = pl.ds(mo(t * T + r * LB, LB), LB)
            x = x_v[rows, :].astype(f32)
            mu = jnp.mean(x, axis=-1, keepdims=True)
            xc = x - mu
            var = jnp.mean(xc * xc, axis=-1, keepdims=True)
            rstd = jax.lax.rsqrt(var + 1e-5)
            xn_s[rows, :] = (xc * rstd).astype(bf16)
            rstd_s[rows, :] = rstd
        rows = tile_rows(t)
        xn = xn_s[rows, :]
        xnT_s[:, rows] = xn.T
        return xn

    def k_soft(t, pkv, g):
        a, b = _dual_softmax(pkv[g * 128:(g + 1) * 128])
        phi = jnp.concatenate([a.reshape(128, T), b.reshape(128, T)], axis=0).astype(bf16)
        phik_s[t, g] = phi
        v = pkv[512 + g * 128: 512 + (g + 1) * 128].astype(bf16)
        vT_s[t, g] = v
        return phi, v

    def k_acc(g, phi, v, first=False):
        r = _dot(jnp.concatenate([v, ones16], axis=0), phi, NT)
        if first:
            kvT_s[g] = r
        else:
            kvT_s[g] += r

    def phase1(t, nxt, extra=None):
        rows = tile_rows(t)
        if nxt is not None:
            xn1 = layernorm(nxt)
        dout = dout_v[rows, :]
        xn = xn_s[rows, :]
        xnT = xnT_s[:, rows]
        nchunk = FA // FC
        st = (ffn_dh(0, dout),) + ffn_gu(0, xn)
        if extra is not None:
            extra[0]()
        if nxt is not None:
            pk = _dot(wT_s[512:1536, :], xn1, NT)
        o_acc = x_v[rows, :].astype(f32)
        d_acc = None
        pv = []
        for c in range(nchunk):
            cs = slice(c * FC, (c + 1) * FC)
            dh, g_, u_ = st
            h, dg, du = ffn_elem(g_, u_, dh)
            if nxt is not None:
                gs = ([0, 1], [2, 3], [])[c]
                pv = [(g, k_soft(nxt, pk, g)) for g in gs]
            if c + 1 < nchunk:
                st = (ffn_dh(c + 1, dout),) + ffn_gu(c + 1, xn)
            if extra is not None and c == 0:
                extra[1]()
            dwg_s[:, cs] += _dot(xnT, dg)
            dwu_s[:, cs] += _dot(xnT, du)
            dwd_s[cs, :] += _dot(h, dout, TN)
            for g, (phi, v) in pv:
                k_acc(g, phi, v)
            o_c, d_c = ffn_mm(c, h, dg, du)
            o_acc = o_acc + o_c
            d_acc = d_c if d_acc is None else d_acc + d_c
        out_s[rows, :] = o_acc
        dxn_s[rows, :] = d_acc

    rr = _iota((144, 256), 0)
    cc = _iota((144, 256), 1)
    m144 = ((rr % 8) == (cc % 8)) & (rr < 136)

    def finish(acc_s, accm_s, accmT_s, col_s):
        for g in range(NG):
            m = jnp.where(m144, acc_s[g], 0.0)
            accm_s[g] = m.astype(bf16)
            mT = m.T
            accmT_s[g] = mT[:, 0:128].astype(bf16)
            col_s[g] = jnp.broadcast_to(jnp.sum(mT[:, 128:144], axis=1, keepdims=True), (256, 128))

    dwg_s[...] = jnp.zeros_like(dwg_s)
    dwu_s[...] = jnp.zeros_like(dwu_s)
    dwd_s[...] = jnp.zeros_like(dwd_s)
    c_wphi.wait()
    w3 = wphi_v[...].reshape(256, 32)
    ym = jnp.where(dmask, _dot(w3, hsel), 0.0).astype(bf16)
    pmT_s[...] = jnp.where(hm4, _dot(rsel, ym), 0.0).astype(bf16)
    c_wv.start()
    c_x(1).start()
    c_x(0).wait()
    xn0 = layernorm(0)
    c_wk.wait()
    c_wdA.start()
    c_wgA.start()
    fold(1)
    pk0 = _dot(wT_s[512:1024, :], xn0, NT)
    phi0 = []
    for g in range(NG):
        a, b = _dual_softmax(pk0[g * 128:(g + 1) * 128])
        phik_s[0, g] = jnp.concatenate([a.reshape(128, T), b.reshape(128, T)], axis=0).astype(bf16)
    c_wv.wait()
    c_x(1).wait()
    c_wuA.start()
    c_do(0).start()
    c_x(2).start()
    xn1 = layernorm(1)
    fold(2)
    pv0 = _dot(wT_s[1024:1536, :], xn_s[0:T, :], NT)
    pk1 = _dot(wT_s[512:1536, :], xn1, NT)
    for g in range(NG):
        v = pv0[g * 128:(g + 1) * 128].astype(bf16)
        vT_s[0, g] = v
        k_acc(g, phik_s[0, g], v, first=True)
    for g in range(NG):
        k_acc(g, *k_soft(1, pk1, g))
    c_wdA.wait()
    c_wgA.wait()
    c_wuA.wait()
    c_do(1).start()
    c_do(2).start()
    for t in range(3, NTILE):
        c_x(t).start()
        c_do(t).start()
    c_wq.start()
    c_wo.start()
    c_wgB.start()
    c_wuB.start()
    c_wdB.start()

    def p1_body(i, carry):
        ts = [i * U1 + k for k in range(U1)]
        for t in ts:
            c_do(t).wait()
            c_x(t + 2).wait()
        for t in ts:
            phase1(t, t + 2)
        return carry

    jax.lax.fori_loop(0, (NTILE - 2) // U1, p1_body, 0)
    c_do(NTILE - 2).wait()
    c_do(NTILE - 1).wait()

    c_wq.wait()
    c_wo.wait()

    def extra0():
        finish(kvT_s, kvz_s, kv_s, zc_s)

    def extra1():
        dkvT_s[...] = jnp.zeros_like(dkvT_s)
        gT_s[...] = jnp.zeros_like(gT_s)
        dwo_s[...] = jnp.zeros_like(dwo_s)
        fold(0)
        for g in range(NG):
            wop_s[g * 128:(g + 1) * 128, :] = _dot(permT, wo_v[g * 128:(g + 1) * 128, :]).astype(bf16)

    phase1(NTILE - 2, None, (extra0, extra1))
    phase1(NTILE - 1, None)
    c_wgB.wait()
    c_wuB.wait()
    c_wdB.wait()

    c0 = FA // FC

    def phase2(t, carry):
        rows = tile_rows(t)
        xn = xn_s[rows, :]
        dout = dout_v[rows, :]
        acc = {}

        def ffn1(c):
            return (ffn_dh(c, dout),) + ffn_gu(c, xn)

        def elem(c, st):
            dh, g_, u_ = st
            h, dg, du = ffn_elem(g_, u_, dh)
            for j in range(FC // 128):
                blk = (c - c0) * (FC // 128) + j
                js = slice(j * 128, (j + 1) * 128)
                h_s[blk, rows, :] = h[:, js]
                dgu_s[blk, rows, 0:128] = dg[:, js]
                dgu_s[blk, rows, 128:256] = du[:, js]
            return h, dg, du

        def mm(c, e):
            o_c, d_c = ffn_mm(c, *e)
            acc['o'] = o_c + acc['o'] if 'o' in acc else o_c
            acc['d'] = d_c + acc['d'] if 'd' in acc else d_c

        pq = _dot(wT_s[0:512, :], xn, NT)
        ab = [_dual_softmax(pq[g * 128:(g + 1) * 128]) for g in range(NG)]
        phis = [jnp.concatenate([a.reshape(128, T), b.reshape(128, T)], axis=0).astype(bf16) for a, b in ab]
        doT = _dot(wop_s[...], dout, NT)
        st0 = ffn1(c0)
        nds = [_dot(kvz_s[g], phis[g]) for g in range(NG)]
        e0 = elem(c0, st0)
        oTs, dnums, ddens = [], [], []
        for g in range(NG):
            nd = nds[g]
            rden = 1.0 / (nd[128:136] + 1e-6)
            o3 = nd[0:128].reshape(16, 8, T) * rden[None]
            do3 = doT[g * 128:(g + 1) * 128].reshape(16, 8, T)
            dnums.append((do3 * rden[None]).reshape(128, T).astype(bf16))
            ddens.append(-jnp.sum(do3 * o3, axis=0) * rden)
            oTs.append(o3.reshape(128, T).astype(bf16))
        st1 = ffn1(c0 + 1)
        dphis = [_dot(kv_s[g], dnums[g]) for g in range(NG)]
        dpqs = []
        for g in range(NG):
            zc = jnp.concatenate([zc_s[g]] * (T // 128), axis=1).reshape(32, 8, T)
            dphi = dphis[g].reshape(32, 8, T) + zc * ddens[g][None]
            a, b = ab[g]
            dp = _dual_softmax_bwd(a, b, dphi[0:16], dphi[16:32])
            dpqs.append(dp.reshape(128, T).astype(bf16))
        dpq = jnp.concatenate(dpqs, axis=0)
        mm(c0, e0)
        oT = jnp.concatenate(oTs, axis=0)
        for g in range(NG):
            dd16 = jnp.concatenate([ddens[g], jnp.zeros_like(ddens[g])], axis=0).astype(bf16)
            dkvT_s[g] += _dot(jnp.concatenate([dnums[g], dd16], axis=0), phis[g], NT)
        e1 = elem(c0 + 1, st1)
        dwo_s[...] += _dot(oT, dout)
        acc['o'] = acc['o'] + _dot(oT, wop_s[...], TN)
        st2 = ffn1(c0 + 2)
        ra = pl.ds(pl.multiple_of(t * RA, RA), RA)
        rd = pl.ds(pl.multiple_of(t * RD, RD), RD)
        dwg_v[ra, 0:FA] = dwg_s[ra, :].astype(bf16)
        dwu_v[ra, 0:FA] = dwu_s[ra, :].astype(bf16)
        dwd_v[rd, :] = dwd_s[rd, :].astype(bf16)
        mm(c0 + 1, e1)
        e2 = elem(c0 + 2, st2)
        st3 = ffn1(c0 + 3)
        mm(c0 + 2, e2)
        e3 = elem(c0 + 3, st3)
        gT_s[0:512, :] += _dot(dpq, xn)
        mm(c0 + 3, e3)
        out_v[rows, :] = (out_s[rows, :] + acc['o']).astype(bf16)
        dxn_s[rows, :] += acc['d'] + _dot(dpq, wT_s[0:512, :], TN)
        return carry

    jax.lax.fori_loop(0, NTILE, phase2, 0, unroll=UNROLL2)
    o_out.start()
    for cpy in o_a:
        cpy.start()

    finish(dkvT_s, dkvTm_s, dkv_s, dzc_s)

    def unfold(part):
        for g in range(NG):
            m = pmT_s[:, g * 128:(g + 1) * 128] if part < 2 else permT
            cs = slice(part * 512 + g * 128, part * 512 + (g + 1) * 128)
            gblk = gT_s[cs, :].astype(bf16)
            dwqkv_v[:, cs] = _dot(gblk, m, TN).astype(bf16)
            if part == 0:
                aphi_s[:, g * 128:(g + 1) * 128] = _dot(gblk, wqkv_v[:, cs])
            elif part == 1:
                aphi_s[:, g * 128:(g + 1) * 128] += _dot(gblk, wqkv_v[:, cs])
        if part == 1:
            accm = jnp.where(hm4, aphi_s[...], 0.0).astype(bf16)
            z = jnp.where(dmask, _dot(rsel, accm, TN), 0.0).astype(bf16)
            dwphi_v[...] = _dot(z, hsel, NT).astype(bf16).reshape(16, 16, 32)

    unfold(0)
    for g in range(NG):
        dwo_v[g * 128:(g + 1) * 128, :] = _dot(permT, dwo_s[g * 128:(g + 1) * 128, :].astype(bf16), TN).astype(bf16)
    o_wq.start()
    o_wo.start()

    def wgrad_gu(t, r0=0, r1=D):
        for j in range(BPI):
            blk = t * BPI + j
            cb = pl.ds(mo(FA + blk * 128, 128), 128)
            dgu = _dot(xnT_s[r0:r1, :], dgu_s[blk])
            dwg_v[r0:r1, cb] = dgu[:, 0:128].astype(bf16)
            dwu_v[r0:r1, cb] = dgu[:, 128:256].astype(bf16)

    def wgrad_d(t):
        for j in range(BPI):
            blk = t * BPI + j
            cb = pl.ds(mo(FA + blk * 128, 128), 128)
            dwd_v[cb, :] = _dot(h_s[blk], dout_v[...], TN).astype(bf16)

    def phase3(t, last):
        rows = tile_rows(t)
        xn = xn_s[rows, :]
        dout = dout_v[rows, :]
        phis = [phik_s[t, g] for g in range(NG)]
        dphis = [_dot(dkv_s[g], vT_s[t, g]) for g in range(NG)]
        dps = []
        for g in range(NG):
            phif = phis[g].astype(f32).reshape(32, 8, T)
            dzc = jnp.concatenate([dzc_s[g]] * (T // 128), axis=1)
            dphi = (dphis[g] + dzc).reshape(32, 8, T)
            dp = _dual_softmax_bwd(phif[0:16], phif[16:32], dphi[0:16], dphi[16:32])
            dps.append(dp.reshape(128, T).astype(bf16))
        dvs = [_dot(dkvTm_s[g, 0:128, :], phis[g]).astype(bf16) for g in range(NG)]
        wgrad_d(t)
        dpkv = jnp.concatenate(dps + dvs, axis=0)
        dxn = dxn_s[rows, :] + _dot(dpkv, wT_s[512:1536, :], TN)
        xnf = xn.astype(f32)
        m1 = jnp.mean(dxn, axis=-1, keepdims=True)
        m2 = jnp.mean(dxn * xnf, axis=-1, keepdims=True)
        dx = rstd_s[rows, :] * (dxn - m1 - xnf * m2) + dout.astype(f32)
        dx_v[rows, :] = dx.astype(bf16)
        gT_s[512:1536, :] += _dot(dpkv, xn)
        if last:
            ob = o_b(t)
            unfold(1)
            unfold(2)
            wgrad_gu(t, 0, SPLIT)
            o_dx(t).start()
            ob[2].start()
            o_wkv.start()
            o_wphi.start()
            wgrad_gu(t, SPLIT, D)
            ob[0].start()
            ob[1].start()
        else:
            wgrad_gu(t)
            o_dx(t).start()
            for cpy in o_b(t):
                cpy.start()

    def p3_body(t, carry):
        phase3(t, False)
        return carry

    jax.lax.fori_loop(0, NTILE - 1, p3_body, 0)
    phase3(NTILE - 1, True)

    o_out.wait()
    for cpy in o_a:
        cpy.wait()
    o_wq.wait()
    o_wo.wait()
    for t in range(NTILE):
        o_dx(t).wait()
    o_wkv.wait()
    o_wphi.wait()
    for t in range(NTILE):
        for cpy in o_b(t):
            cpy.wait()


@jax.jit
def pallas_parallel_sum__linear_kernel_hedgehog__glu_gated_bilinear__prompt_kernel(A_x, A_wqkv, A_w_phi, A_wo, B_x, B_w_gate, B_w_up, B_w_down, grad_out):
    x = A_x.reshape(S, D)
    dout = grad_out.reshape(S, D)
    wphi = jnp.transpose(A_w_phi, (1, 2, 0))
    sds = jax.ShapeDtypeStruct
    io_shapes = ((S, D), (S, D), (D, 3 * D), (DH, DH, H), (D, D), (D, F), (D, F), (F, D))
    any_spec = pl.BlockSpec(memory_space=pl.ANY)
    io_scratch = [pltpu.VMEM(s, bf16) if len(s) == 3 else pltpu.VMEM((s[0] // 2, s[1]), jnp.uint32) for s in io_shapes]
    dma = pltpu.SemaphoreType.DMA
    outs = pl.pallas_call(
        kernel,
        out_shape=tuple(sds(s, bf16) for s in io_shapes),
        in_specs=[any_spec] * 8,
        out_specs=tuple([any_spec] * 8),
        scratch_shapes=io_scratch + io_scratch + [
            pltpu.VMEM((3 * D // 2, D), jnp.uint32),
            pltpu.VMEM((D // 2, D), jnp.uint32),
            pltpu.VMEM((64, 512), jnp.uint32),
            pltpu.VMEM((S // 2, D), jnp.uint32),
            pltpu.VMEM((D // 2, S), jnp.uint32),
            pltpu.VMEM((S, 1), f32),
            pltpu.VMEM((NTILE, NG, 128, T), jnp.uint32),
            pltpu.VMEM((NTILE, NG, 64, T), jnp.uint32),
            pltpu.VMEM((NG, 144, 256), f32),
            pltpu.VMEM((NG, 72, 256), jnp.uint32),
            pltpu.VMEM((NG, 128, 128), jnp.uint32),
            pltpu.VMEM((NG, 256, 128), f32),
            pltpu.VMEM((NG, 144, 256), f32),
            pltpu.VMEM((NG, 72, 256), jnp.uint32),
            pltpu.VMEM((NG, 128, 128), jnp.uint32),
            pltpu.VMEM((NG, 256, 128), f32),
            pltpu.VMEM((3 * D, D), f32),
            pltpu.VMEM((D, D), f32),
            pltpu.VMEM((D, FA), f32),
            pltpu.VMEM((D, FA), f32),
            pltpu.VMEM((FA, D), f32),
            pltpu.VMEM((S, D), f32),
            pltpu.VMEM((S, D), f32),
            pltpu.VMEM((NB, S // 2, 128), jnp.uint32),
            pltpu.VMEM((NB, S // 2, 256), jnp.uint32),
            pltpu.VMEM((128, 512), f32),
            dma((11,)), dma((NTILE,)), dma((NTILE,)), dma((NTILE,)), dma((NTILE,)),
            dma((3, NTILE)), dma((3, NTILE)), dma((4,)),
        ],
        compiler_params=pltpu.CompilerParams(vmem_limit_bytes=110 * 1024 * 1024),
    )(x, A_wqkv, wphi, A_wo, B_w_gate, B_w_up, B_w_down, dout)
    out, dx, dwqkv, dwphi, dwo, dwg, dwu, dwd = outs
    return (out.reshape(1, S, D), dx.reshape(1, S, D), dwqkv, jnp.transpose(dwphi, (2, 0, 1)), dwo, dwg, dwu, dwd)
```

```python
import functools
import jax
import jax.numpy as jnp
import jax.experimental.pallas as pl
import jax.experimental.pallas.tpu as pltpu

S, D, H, DH, F = 2048, 512, 32, 16, 1792
NG = 4
T = 256
NTILE = S // T
FC = 256
FA = 768
FB = F - FA
NB = FB // 128
BPI = NB // NTILE

UNROLL2 = 2
U1 = 1
SPLIT = 128
f32 = jnp.float32
bf16 = jnp.bfloat16
NN = (((1,), (0,)), ((), ()))
NT = (((1,), (1,)), ((), ()))
TN = (((0,), (0,)), ((), ()))


def _dot(a, b, dn=NN):
    return jax.lax.dot_general(a, b, dn, preferred_element_type=f32)


def _dual_softmax(p):
    p3 = p.reshape(16, 8, p.shape[-1])
    mx = jnp.max(p3, axis=0, keepdims=True)
    mn = jnp.min(p3, axis=0, keepdims=True)
    ea = jnp.exp(p3 - mx)
    eb = jnp.exp(mn - p3)
    a = ea * (1.0 / jnp.sum(ea, axis=0, keepdims=True))
    b = eb * (1.0 / jnp.sum(eb, axis=0, keepdims=True))
    return a, b


def _dual_softmax_bwd(a, b, da, db):
    ta = a * da
    tb = b * db
    return (ta - a * jnp.sum(ta, axis=0, keepdims=True)) - (tb - b * jnp.sum(tb, axis=0, keepdims=True))


def _iota(shape, dim):
    return jax.lax.broadcasted_iota(jnp.int32, shape, dim)


def kernel(x_hbm, wqkv_hbm, wphi_hbm, wo_hbm, wg_hbm, wu_hbm, wd_hbm, dout_hbm,
           out_hbm, dx_hbm, dwqkv_hbm, dwphi_hbm, dwo_hbm, dwg_hbm, dwu_hbm, dwd_hbm,
           x_v, dout_v, wqkv_v, wphi_v, wo_v, wg_v, wu_v, wd_v,
           out_v, dx_v, dwqkv_v, dwphi_v, dwo_v, dwg_v, dwu_v, dwd_v,
           wT_s, wop_s, pmT_s, xn_s, xnT_s, rstd_s, phik_s, vT_s, kvT_s, kvz_s, kv_s, zc_s,
           dkvT_s, dkvTm_s, dkv_s, dzc_s, gT_s, dwo_s, dwg_s, dwu_s, dwd_s, out_s, dxn_s,
           h_s, dg_s, du_s, aphi_s, dp_s,
           sem_w, sem_x, sem_do, sem_out, sem_dx, sem_a, sem_b, sem_e):
    (wT_s, wop_s, pmT_s, xn_s, xnT_s, phik_s, vT_s, kvz_s, kv_s, dkvTm_s, dkv_s, h_s, dg_s, du_s,
     x_v, dout_v, wqkv_v, wo_v, wg_v, wu_v, wd_v, out_v, dx_v, dwqkv_v, dwo_v, dwg_v, dwu_v, dwd_v) = [
         r.bitcast(bf16) for r in (
             wT_s, wop_s, pmT_s, xn_s, xnT_s, phik_s, vT_s, kvz_s, kv_s, dkvTm_s, dkv_s, h_s, dg_s, du_s,
             x_v, dout_v, wqkv_v, wo_v, wg_v, wu_v, wd_v, out_v, dx_v, dwqkv_v, dwo_v, dwg_v, dwu_v, dwd_v)]
    dp_s = dp_s.bitcast(bf16)
    ALL = slice(None)

    def cp(src, dst, sem, *idx):
        if idx:
            src, dst = src.at[idx], dst.at[idx]
        return pltpu.make_async_copy(src, dst, sem)

    def mo(v, m):
        return v if isinstance(v, int) else pl.multiple_of(v, m)

    def tile_rows(t):
        if isinstance(t, int):
            return pl.ds(t * T, T)
        return pl.ds(pl.multiple_of(t * T, T), T)

    c_wphi = pltpu.make_async_copy(wphi_hbm, wphi_v, sem_w.at[0])
    c_wk = cp(wqkv_hbm, wqkv_v, sem_w.at[1], ALL, slice(512, 1024))
    c_wv = cp(wqkv_hbm, wqkv_v, sem_w.at[10], ALL, slice(1024, 1536))
    c_wq = cp(wqkv_hbm, wqkv_v, sem_w.at[2], ALL, slice(0, 512))
    c_wo = cp(wo_hbm, wo_v, sem_w.at[3])
    c_wgA = cp(wg_hbm, wg_v, sem_w.at[4], ALL, slice(0, FA))
    c_wuA = cp(wu_hbm, wu_v, sem_w.at[5], ALL, slice(0, FA))
    c_wdA = cp(wd_hbm, wd_v, sem_w.at[6], slice(0, FA), ALL)
    c_wgB = cp(wg_hbm, wg_v, sem_w.at[7], ALL, slice(FA, F))
    c_wuB = cp(wu_hbm, wu_v, sem_w.at[8], ALL, slice(FA, F))
    c_wdB = cp(wd_hbm, wd_v, sem_w.at[9], slice(FA, F), ALL)

    def c_x(t):
        return cp(x_hbm, x_v, sem_x.at[t], tile_rows(t), ALL)

    def c_do(t):
        return cp(dout_hbm, dout_v, sem_do.at[t], tile_rows(t), ALL)

    c_wphi.start()
    c_x(0).start()
    c_wk.start()

    o_out = cp(out_v, out_hbm, sem_out.at[0])

    def o_dx(t):
        return cp(dx_v, dx_hbm, sem_dx.at[t], tile_rows(t), ALL)

    RA = D // NTILE
    RD = FA // NTILE

    o_a = (cp(dwg_v, dwg_hbm, sem_out.at[1], ALL, slice(0, FA)),
           cp(dwu_v, dwu_hbm, sem_out.at[2], ALL, slice(0, FA)),
           cp(dwd_v, dwd_hbm, sem_out.at[3], slice(0, FA), ALL))

    def o_b(t):
        cb = pl.ds(mo(FA + t * (128 * BPI), 128), 128 * BPI)
        return (cp(dwg_v, dwg_hbm, sem_b.at[0, t], ALL, cb),
                cp(dwu_v, dwu_hbm, sem_b.at[1, t], ALL, cb),
                cp(dwd_v, dwd_hbm, sem_b.at[2, t], cb, ALL))

    o_wq = cp(dwqkv_v, dwqkv_hbm, sem_e.at[0], ALL, slice(0, 512))
    o_wkv = cp(dwqkv_v, dwqkv_hbm, sem_e.at[1], ALL, slice(512, 1536))
    o_wo = cp(dwo_v, dwo_hbm, sem_e.at[2])
    o_wphi = pltpu.make_async_copy(dwphi_v, dwphi_hbm, sem_e.at[3])

    r_i = _iota((128, 128), 0)
    c_i = _iota((128, 128), 1)
    head_mask = (r_i % 8) == (c_i // 16)
    permT = jnp.where(head_mask & ((r_i // 8) == (c_i % 16)), 1.0, 0.0).astype(bf16)
    hsel = jnp.where(_iota((32, 512), 0) == (_iota((32, 512), 1) // 16), 1.0, 0.0).astype(bf16)
    dmask = (_iota((256, 512), 0) // 16) == (_iota((256, 512), 1) % 16)
    rsel = jnp.where((_iota((128, 256), 0) // 8) == (_iota((128, 256), 1) % 16), 1.0, 0.0).astype(bf16)
    hm4 = (_iota((128, 512), 0) % 8) == ((_iota((128, 512), 1) // 16) % 8)
    ones16 = jnp.ones((16, T), f32)

    def fold(part):
        for g in range(NG):
            m = pmT_s[:, g * 128:(g + 1) * 128] if part < 2 else permT
            cs = slice(part * 512 + g * 128, part * 512 + (g + 1) * 128)
            wT_s[cs, :] = _dot(m, wqkv_v[:, cs], NT).astype(bf16)

    def w_g(c):
        return wg_v[:, c * FC:(c + 1) * FC]

    def w_u(c):
        return wu_v[:, c * FC:(c + 1) * FC]

    def w_d(c):
        return wd_v[c * FC:(c + 1) * FC, :]

    def ffn_dh(c, dout):
        return _dot(dout, w_d(c), NT)

    def ffn_gu(c, xn):
        return _dot(xn, w_g(c)), _dot(xn, w_u(c))

    def ffn_elem(g_, u_, dh):
        return (g_ * u_).astype(bf16), (dh * u_).astype(bf16), (dh * g_).astype(bf16)

    def ffn_mm(c, h, dg, du):
        o_c = _dot(h, w_d(c))
        d_c = _dot(dg, w_g(c), NT) + _dot(du, w_u(c), NT)
        return o_c, d_c

    def layernorm(t):
        LB = 32
        for r in range(T // LB):
            rows = pl.ds(mo(t * T + r * LB, LB), LB)
            x = x_v[rows, :].astype(f32)
            mu = jnp.mean(x, axis=-1, keepdims=True)
            xc = x - mu
            var = jnp.mean(xc * xc, axis=-1, keepdims=True)
            rstd = jax.lax.rsqrt(var + 1e-5)
            xn_s[rows, :] = (xc * rstd).astype(bf16)
            rstd_s[rows, :] = rstd
        rows = tile_rows(t)
        xn = xn_s[rows, :]
        xnT_s[:, rows] = xn.T
        return xn

    def k_phi(t, pk, g):
        a, b = _dual_softmax(pk[g * 128:(g + 1) * 128])
        phi = jnp.concatenate([a.reshape(128, T), b.reshape(128, T)], axis=0).astype(bf16)
        phik_s[g * 256:(g + 1) * 256, tile_rows(t)] = phi
        return phi

    def k_v(t, pv, g):
        v1 = jnp.concatenate([pv[g * 128:(g + 1) * 128], ones16], axis=0).astype(bf16)
        vT_s[g * 144:(g + 1) * 144, tile_rows(t)] = v1
        return v1

    def k_soft(t, pkv, g):
        return k_phi(t, pkv, g), k_v(t, pkv[512:1024], g)

    def k_acc(g, phi, v1, first=False):
        r = _dot(v1, phi, NT)
        if first:
            kvT_s[g] = r
        else:
            kvT_s[g] += r

    def phase1(t, nxt, extra=None):
        rows = tile_rows(t)
        if nxt is not None:
            xn1 = layernorm(nxt)
        dout = dout_v[rows, :]
        xn = xn_s[rows, :]
        xnT = xnT_s[:, rows]
        nchunk = FA // FC
        phis = {}

        def kphi(g):
            if nxt is not None:
                pk = _dot(wT_s[512 + g * 128:512 + (g + 1) * 128, :], xn1, NT)
                a, b = _dual_softmax(pk)
                phi = jnp.concatenate([a.reshape(128, T), b.reshape(128, T)], axis=0).astype(bf16)
                phik_s[g * 256:(g + 1) * 256, tile_rows(nxt)] = phi
                phis[g] = phi

        st = (ffn_dh(0, dout),) + ffn_gu(0, xn)
        if extra is not None:
            extra[0]()
        kphi(0)
        o_acc = x_v[rows, :].astype(f32)
        d_acc = None
        for c in range(nchunk):
            cs = slice(c * FC, (c + 1) * FC)
            dh, g_, u_ = st
            if c + 1 < nchunk:
                dh1 = ffn_dh(c + 1, dout)
            h, dg, du = ffn_elem(g_, u_, dh)
            if c + 1 < nchunk:
                st = (dh1,) + ffn_gu(c + 1, xn)
            if extra is not None and c == 0:
                extra[1]()
            if c == 0:
                kphi(1)
            dwg_s[:, cs] += _dot(xnT, dg)
            if c == 0:
                kphi(2)
            dwu_s[:, cs] += _dot(xnT, du)
            if c == 0:
                kphi(3)
            dwd_s[cs, :] += _dot(h, dout, TN)
            if c == 1 and nxt is not None:
                pv = _dot(wT_s[1024:1536, :], xn1, NT)
                for g in range(NG):
                    k_acc(g, phis[g], k_v(nxt, pv, g))
            o_c, d_c = ffn_mm(c, h, dg, du)
            o_acc = o_acc + o_c
            d_acc = d_c if d_acc is None else d_acc + d_c
        out_s[rows, :] = o_acc
        dxn_s[rows, :] = d_acc

    rr = _iota((144, 256), 0)
    cc = _iota((144, 256), 1)
    m144 = ((rr % 8) == (cc % 8)) & (rr < 136)

    def finish(acc_s, accm_s, accmT_s, col_s):
        for g in range(NG):
            m = jnp.where(m144, acc_s[g], 0.0)
            accm_s[g] = m.astype(bf16)
            mT = m.T
            accmT_s[:, g * 128:(g + 1) * 128] = mT[:, 0:128].astype(bf16)
            col_s[g] = jnp.broadcast_to(jnp.sum(mT[:, 128:144], axis=1, keepdims=True), (256, 128))

    dwg_s[...] = jnp.zeros_like(dwg_s)
    dwu_s[...] = jnp.zeros_like(dwu_s)
    dwd_s[...] = jnp.zeros_like(dwd_s)
    c_wphi.wait()
    w3 = wphi_v[...].reshape(256, 32)
    ym = jnp.where(dmask, _dot(w3, hsel), 0.0).astype(bf16)
    pmT_s[...] = jnp.where(hm4, _dot(rsel, ym), 0.0).astype(bf16)
    c_wv.start()
    c_x(1).start()
    c_x(0).wait()
    xn0 = layernorm(0)
    c_wk.wait()
    c_wdA.start()
    c_wgA.start()
    fold(1)
    pk0 = _dot(wT_s[512:1024, :], xn0, NT)
    for g in range(NG):
        k_phi(0, pk0, g)
    c_wv.wait()
    c_x(1).wait()
    c_wuA.start()
    c_do(0).start()
    c_x(2).start()
    xn1 = layernorm(1)
    fold(2)
    pv0 = _dot(wT_s[1024:1536, :], xn_s[0:T, :], NT)
    pk1 = _dot(wT_s[512:1536, :], xn1, NT)
    for g in range(NG):
        k_acc(g, phik_s[g * 256:(g + 1) * 256, 0:T], k_v(0, pv0, g), first=True)
    for g in range(NG):
        k_acc(g, *k_soft(1, pk1, g))
    c_wdA.wait()
    c_wgA.wait()
    c_wuA.wait()
    c_do(1).start()
    c_do(2).start()
    for t in range(3, NTILE):
        c_x(t).start()
        c_do(t).start()
    c_wq.start()
    c_wo.start()
    c_wgB.start()
    c_wuB.start()
    c_wdB.start()

    def p1_body(i, carry):
        ts = [i * U1 + k for k in range(U1)]
        for t in ts:
            c_do(t).wait()
            c_x(t + 2).wait()
        for t in ts:
            phase1(t, t + 2)
        return carry

    jax.lax.fori_loop(0, (NTILE - 2) // U1, p1_body, 0)
    c_do(NTILE - 2).wait()
    c_do(NTILE - 1).wait()

    c_wq.wait()
    c_wo.wait()

    def extra0():
        finish(kvT_s, kvz_s, kv_s, zc_s)

    def extra1():
        dkvT_s[...] = jnp.zeros_like(dkvT_s)
        gT_s[...] = jnp.zeros_like(gT_s)
        dwo_s[...] = jnp.zeros_like(dwo_s)
        fold(0)
        for g in range(NG):
            wop_s[g * 128:(g + 1) * 128, :] = _dot(permT, wo_v[g * 128:(g + 1) * 128, :]).astype(bf16)

    phase1(NTILE - 2, None, (extra0, extra1))
    phase1(NTILE - 1, None)
    c_wgB.wait()
    c_wuB.wait()
    c_wdB.wait()

    c0 = FA // FC

    def phase2(t, carry):
        rows = tile_rows(t)
        xn = xn_s[rows, :]
        dout = dout_v[rows, :]
        acc = {}

        def ffn1(c):
            return (ffn_dh(c, dout),) + ffn_gu(c, xn)

        def elem(c, st):
            dh, g_, u_ = st
            h, dg, du = ffn_elem(g_, u_, dh)
            cs = slice((c - c0) * FC, (c - c0 + 1) * FC)
            h_s[rows, cs] = h
            dg_s[rows, cs] = dg
            du_s[rows, cs] = du
            return h, dg, du

        def mm(c, e):
            o_c, d_c = ffn_mm(c, *e)
            acc['o'] = o_c + acc['o'] if 'o' in acc else o_c
            acc['d'] = d_c + acc['d'] if 'd' in acc else d_c

        pq = _dot(wT_s[0:512, :], xn, NT)
        ab = [_dual_softmax(pq[g * 128:(g + 1) * 128]) for g in range(NG)]
        phis = [jnp.concatenate([a.reshape(128, T), b.reshape(128, T)], axis=0).astype(bf16) for a, b in ab]
        doT = _dot(wop_s[...], dout, NT)
        oTs, dnums, ddens, dpqs = [], [], [], []

        def stage2(g):
            nd = _dot(kvz_s[g], phis[g])
            rden = 1.0 / (nd[128:136] + 1e-6)
            o3 = nd[0:128].reshape(16, 8, T) * rden[None]
            do3 = doT[g * 128:(g + 1) * 128].reshape(16, 8, T)
            dnums.append((do3 * rden[None]).reshape(128, T))
            ddens.append(-jnp.sum(do3 * o3, axis=0) * rden)
            oTs.append(o3.reshape(128, T))

        def stage3(g):
            dphi = _dot(kv_s[:, g * 128:(g + 1) * 128], dnums[g].astype(bf16))
            zc = jnp.concatenate([zc_s[g]] * (T // 128), axis=1).reshape(32, 8, T)
            dphi = dphi.reshape(32, 8, T) + zc * ddens[g][None]
            a, b = ab[g]
            dp = _dual_softmax_bwd(a, b, dphi[0:16], dphi[16:32])
            dpqs.append(dp.reshape(128, T))

        dh0 = ffn_dh(c0, dout)
        g0 = _dot(xn, w_g(c0))
        stage2(0)
        u0 = _dot(xn, w_u(c0))
        stage2(1)
        dh1 = ffn_dh(c0 + 1, dout)
        stage2(2)
        g1 = _dot(xn, w_g(c0 + 1))
        stage2(3)
        e0 = elem(c0, (dh0, g0, u0))
        u1 = _dot(xn, w_u(c0 + 1))
        st1 = (dh1, g1, u1)
        stage3(0)
        acc['o'] = _dot(e0[0], w_d(c0))
        stage3(1)
        acc['d'] = _dot(e0[1], w_g(c0), NT)
        stage3(2)
        acc['d'] = acc['d'] + _dot(e0[2], w_u(c0), NT)
        stage3(3)
        dpq = jnp.concatenate(dpqs, axis=0).astype(bf16)
        oT = jnp.concatenate(oTs, axis=0).astype(bf16)
        for g in range(NG):
            dn1 = jnp.concatenate([dnums[g], ddens[g], jnp.zeros_like(ddens[g])], axis=0).astype(bf16)
            dkvT_s[g] += _dot(dn1, phis[g], NT)
        e1 = elem(c0 + 1, st1)
        dwo_s[...] += _dot(oT, dout)
        acc['o'] = acc['o'] + _dot(oT, wop_s[...], TN)
        st2 = ffn1(c0 + 2)
        ra = pl.ds(pl.multiple_of(t * RA, RA), RA)
        rd = pl.ds(pl.multiple_of(t * RD, RD), RD)
        dwg_v[ra, 0:FA] = dwg_s[ra, :].astype(bf16)
        dwu_v[ra, 0:FA] = dwu_s[ra, :].astype(bf16)
        dwd_v[rd, :] = dwd_s[rd, :].astype(bf16)
        mm(c0 + 1, e1)
        e2 = elem(c0 + 2, st2)
        st3 = ffn1(c0 + 3)
        mm(c0 + 2, e2)
        e3 = elem(c0 + 3, st3)
        gT_s[0:512, :] += _dot(dpq, xn)
        mm(c0 + 3, e3)
        out_v[rows, :] = (out_s[rows, :] + acc['o']).astype(bf16)
        dxn_s[rows, :] += acc['d'] + _dot(dpq, wT_s[0:512, :], TN)
        return carry

    jax.lax.fori_loop(0, NTILE, phase2, 0, unroll=UNROLL2)
    o_out.start()
    for cpy in o_a:
        cpy.start()

    finish(dkvT_s, dkvTm_s, dkv_s, dzc_s)

    def unfold(part):
        for g in range(NG):
            m = pmT_s[:, g * 128:(g + 1) * 128] if part < 2 else permT
            cs = slice(part * 512 + g * 128, part * 512 + (g + 1) * 128)
            gblk = gT_s[cs, :].astype(bf16)
            dwqkv_v[:, cs] = _dot(gblk, m, TN).astype(bf16)
            if part == 0:
                aphi_s[:, g * 128:(g + 1) * 128] = _dot(gblk, wqkv_v[:, cs])
            elif part == 1:
                aphi_s[:, g * 128:(g + 1) * 128] += _dot(gblk, wqkv_v[:, cs])
        if part == 1:
            accm = jnp.where(hm4, aphi_s[...], 0.0).astype(bf16)
            z = jnp.where(dmask, _dot(rsel, accm, TN), 0.0).astype(bf16)
            dwphi_v[...] = _dot(z, hsel, NT).astype(bf16).reshape(16, 16, 32)

    unfold(0)
    for g in range(NG):
        dwo_v[g * 128:(g + 1) * 128, :] = _dot(permT, dwo_s[g * 128:(g + 1) * 128, :].astype(bf16), TN).astype(bf16)
    o_wq.start()
    o_wo.start()

    def wgrad_gu(t, r0=0, r1=D):
        for j in range(BPI):
            blk = t * BPI + j
            cl = pl.ds(mo(blk * 128, 128), 128)
            cb = pl.ds(mo(FA + blk * 128, 128), 128)
            dgu = _dot(xnT_s[r0:r1, :], jnp.concatenate([dg_s[:, cl], du_s[:, cl]], axis=1))
            dwg_v[r0:r1, cb] = dgu[:, 0:128].astype(bf16)
            dwu_v[r0:r1, cb] = dgu[:, 128:256].astype(bf16)

    def wgrad_d(t, c0_, c1_):
        for j in range(BPI):
            blk = t * BPI + j
            cl = pl.ds(mo(blk * 128, 128), 128)
            cb = pl.ds(mo(FA + blk * 128, 128), 128)
            dwd_v[cb, c0_:c1_] = _dot(h_s[:, cl], dout_v[:, c0_:c1_], TN).astype(bf16)

    def phase3(t, last):
        rows = tile_rows(t)
        xn = xn_s[rows, :]
        dout = dout_v[rows, :]
        phis = [phik_s[g * 256:(g + 1) * 256, rows] for g in range(NG)]
        def sm_bwd(gs):
            dphis = [_dot(dkv_s[:, g * 128:(g + 1) * 128], vT_s[g * 144:g * 144 + 128, rows]) for g in gs]
            for g, dphi in zip(gs, dphis):
                phif = phis[g].astype(f32).reshape(32, 8, T)
                dzc = jnp.concatenate([dzc_s[g]] * (T // 128), axis=1)
                dphi = (dphi + dzc).reshape(32, 8, T)
                dp = _dual_softmax_bwd(phif[0:16], phif[16:32], dphi[0:16], dphi[16:32])
                dp_s[g * 128:(g + 1) * 128, :] = dp.reshape(128, T).astype(bf16)

        sm_bwd([0])
        for g in range(NG):
            dp_s[512 + g * 128:512 + (g + 1) * 128, :] = _dot(dkvTm_s[g, 0:128, :], phis[g]).astype(bf16)
        sm_bwd([1])
        wgrad_d(t, 0, 256)
        sm_bwd([2])
        wgrad_d(t, 256, 384)
        sm_bwd([3])
        wgrad_d(t, 384, 512)
        dpkv = dp_s

        def ln_part(r, n):
            LB = T // n
            rw = pl.ds(mo(t * T + r * LB, LB), LB)
            dxn = dxn_s[rw, :] + _dot(dpkv[:, r * LB:(r + 1) * LB], wT_s[512:1536, :], TN)
            xnf = xn_s[rw, :].astype(f32)
            m1 = jnp.mean(dxn, axis=-1, keepdims=True)
            m2 = jnp.mean(dxn * xnf, axis=-1, keepdims=True)
            dx = rstd_s[rw, :] * (dxn - m1 - xnf * m2) + dout_v[rw, :].astype(f32)
            dx_v[rw, :] = dx.astype(bf16)

        ln_part(0, 2)
        gT_s[512:1024, :] += _dot(dpkv[0:512, :], xn)
        ln_part(1, 2)
        gT_s[1024:1536, :] += _dot(dpkv[512:1024, :], xn)
        if last:
            ob = o_b(t)
            unfold(1)
            unfold(2)
            wgrad_gu(t, 0, SPLIT)
            o_dx(t).start()
            ob[2].start()
            o_wkv.start()
            o_wphi.start()
            wgrad_gu(t, SPLIT, D)
            ob[0].start()
            ob[1].start()
        else:
            wgrad_gu(t)
            o_dx(t).start()
            for cpy in o_b(t):
                cpy.start()

    def p3_body(t, carry):
        phase3(t, False)
        return carry

    jax.lax.fori_loop(0, NTILE - 1, p3_body, 0)
    phase3(NTILE - 1, True)

    o_out.wait()
    for cpy in o_a:
        cpy.wait()
    o_wq.wait()
    o_wo.wait()
    for t in range(NTILE):
        o_dx(t).wait()
    o_wkv.wait()
    o_wphi.wait()
    for t in range(NTILE):
        for cpy in o_b(t):
            cpy.wait()


@jax.jit
def pallas_parallel_sum__linear_kernel_hedgehog__glu_gated_bilinear__prompt_kernel(A_x, A_wqkv, A_w_phi, A_wo, B_x, B_w_gate, B_w_up, B_w_down, grad_out):
    x = A_x.reshape(S, D)
    dout = grad_out.reshape(S, D)
    wphi = jnp.transpose(A_w_phi, (1, 2, 0))
    sds = jax.ShapeDtypeStruct
    io_shapes = ((S, D), (S, D), (D, 3 * D), (DH, DH, H), (D, D), (D, F), (D, F), (F, D))
    any_spec = pl.BlockSpec(memory_space=pl.ANY)
    io_scratch = [pltpu.VMEM(s, bf16) if len(s) == 3 else pltpu.VMEM((s[0] // 2, s[1]), jnp.uint32) for s in io_shapes]
    dma = pltpu.SemaphoreType.DMA
    outs = pl.pallas_call(
        kernel,
        out_shape=tuple(sds(s, bf16) for s in io_shapes),
        in_specs=[any_spec] * 8,
        out_specs=tuple([any_spec] * 8),
        scratch_shapes=io_scratch + io_scratch + [
            pltpu.VMEM((3 * D // 2, D), jnp.uint32),
            pltpu.VMEM((D // 2, D), jnp.uint32),
            pltpu.VMEM((64, 512), jnp.uint32),
            pltpu.VMEM((S // 2, D), jnp.uint32),
            pltpu.VMEM((D // 2, S), jnp.uint32),
            pltpu.VMEM((S, 1), f32),
            pltpu.VMEM((NG * 128, S), jnp.uint32),
            pltpu.VMEM((NG * 72, S), jnp.uint32),
            pltpu.VMEM((NG, 144, 256), f32),
            pltpu.VMEM((NG, 72, 256), jnp.uint32),
            pltpu.VMEM((128, NG * 128), jnp.uint32),
            pltpu.VMEM((NG, 256, 128), f32),
            pltpu.VMEM((NG, 144, 256), f32),
            pltpu.VMEM((NG, 72, 256), jnp.uint32),
            pltpu.VMEM((128, NG * 128), jnp.uint32),
            pltpu.VMEM((NG, 256, 128), f32),
            pltpu.VMEM((3 * D, D), f32),
            pltpu.VMEM((D, D), f32),
            pltpu.VMEM((D, FA), f32),
            pltpu.VMEM((D, FA), f32),
            pltpu.VMEM((FA, D), f32),
            pltpu.VMEM((S, D), f32),
            pltpu.VMEM((S, D), f32),
            pltpu.VMEM((S // 2, FB), jnp.uint32),
            pltpu.VMEM((S // 2, FB), jnp.uint32),
            pltpu.VMEM((S // 2, FB), jnp.uint32),
            pltpu.VMEM((128, 512), f32),
            pltpu.VMEM((D, T), jnp.uint32),
            dma((11,)), dma((NTILE,)), dma((NTILE,)), dma((NTILE,)), dma((NTILE,)),
            dma((3, NTILE)), dma((3, NTILE)), dma((4,)),
        ],
        compiler_params=pltpu.CompilerParams(vmem_limit_bytes=110 * 1024 * 1024),
    )(x, A_wqkv, wphi, A_wo, B_w_gate, B_w_up, B_w_down, dout)
    out, dx, dwqkv, dwphi, dwo, dwg, dwu, dwd = outs
    return (out.reshape(1, S, D), dx.reshape(1, S, D), dwqkv, jnp.transpose(dwphi, (2, 0, 1)), dwo, dwg, dwu, dwd)
```

```python
import jax
import jax.numpy as jnp
import jax.experimental.pallas as pl
import jax.experimental.pallas.tpu as pltpu

S, D, H, DH, F = 2048, 512, 32, 16, 1792
NG = 8
NBLK = 4
T = 256
NTILE = S // T
FC = 256
FA = 768
FB = F - FA
SPLIT = 128

f32 = jnp.float32
bf16 = jnp.bfloat16
u32 = jnp.uint32
NN = (((1,), (0,)), ((), ()))
NT = (((1,), (1,)), ((), ()))
TN = (((0,), (0,)), ((), ()))


def _dot(a, b, dn=NN):
    return jax.lax.dot_general(a, b, dn, preferred_element_type=f32)


def _head_reduce(x3, red, comb):
    r = red(x3, axis=0)
    return comb(r, pltpu.roll(r, 4, 0))


def _hsum(x3):
    return _head_reduce(x3, jnp.sum, jnp.add)


def _dual_softmax(p):
    p3 = p.reshape(8, 8, p.shape[-1])
    mx = _head_reduce(p3, jnp.max, jnp.maximum)
    mn = _head_reduce(p3, jnp.min, jnp.minimum)
    ea = jnp.exp(p3 - mx[None])
    eb = jnp.exp(mn[None] - p3)
    a = ea * (1.0 / _hsum(ea))[None]
    b = eb * (1.0 / _hsum(eb))[None]
    return a, b


def _dual_softmax_bwd(a, b, da, db):
    ta = a * da
    tb = b * db
    return (ta - a * _hsum(ta)[None]) - (tb - b * _hsum(tb)[None])


def _phi(a, b):
    return jnp.concatenate([a.reshape(64, T), b.reshape(64, T)], axis=0).astype(bf16)


def _iota(shape, dim):
    return jax.lax.broadcasted_iota(jnp.int32, shape, dim)


def kernel(x_hbm, wqkv_hbm, wphi_hbm, wo_hbm, wg_hbm, wu_hbm, wd_hbm, dout_hbm,
           out_hbm, dx_hbm, dwqkv_hbm, dwphi_hbm, dwo_hbm, dwg_hbm, dwu_hbm, dwd_hbm,
           x_v, dout_v, wqkv_v, wphi_v, wo_v, wg_v, wu_v, wd_v,
           out_v, dx_v, dwqkv_v, dwphi_v, dwo_v, dwg_v, dwu_v, dwd_v,
           wT_s, wop_s, pmT_s, xn_s, xnT_s, phik_s, vT_s, kvz_s, kv4_s, dkv4_s, dkv4T_s, h_s, dg_s, du_s, dp_s,
           rstd_s, kvT_s, dkvT_s, gT_s, dwo_s, dwg_s, dwu_s, dwd_s, out_s, dxn_s, aphi_s,
           sem_w, sem_x, sem_do, sem_out, sem_dx, sem_b, sem_e):
    (x_v, dout_v, wqkv_v, wo_v, wg_v, wu_v, wd_v, out_v, dx_v, dwqkv_v, dwo_v, dwg_v, dwu_v, dwd_v,
     wT_s, wop_s, pmT_s, xn_s, xnT_s, phik_s, vT_s, kvz_s, kv4_s, dkv4_s, dkv4T_s, h_s, dg_s, du_s, dp_s) = [
         r.bitcast(bf16) for r in (
             x_v, dout_v, wqkv_v, wo_v, wg_v, wu_v, wd_v, out_v, dx_v, dwqkv_v, dwo_v, dwg_v, dwu_v, dwd_v,
             wT_s, wop_s, pmT_s, xn_s, xnT_s, phik_s, vT_s, kvz_s, kv4_s, dkv4_s, dkv4T_s, h_s, dg_s, du_s, dp_s)]
    ALL = slice(None)

    def cp(src, dst, sem, *idx):
        if idx:
            src, dst = src.at[idx], dst.at[idx]
        return pltpu.make_async_copy(src, dst, sem)

    def mo(v, m):
        return v if isinstance(v, int) else pl.multiple_of(v, m)

    def tile_rows(t):
        return pl.ds(mo(t * T, T), T)

    def gl(g):
        return slice(g * 128, (g + 1) * 128)

    c_wphi = cp(wphi_hbm, wphi_v, sem_w.at[0])
    c_wk = cp(wqkv_hbm, wqkv_v, sem_w.at[1], ALL, slice(512, 1024))
    c_wv = cp(wqkv_hbm, wqkv_v, sem_w.at[10], ALL, slice(1024, 1536))
    c_wq = cp(wqkv_hbm, wqkv_v, sem_w.at[2], ALL, slice(0, 512))
    c_wo = cp(wo_hbm, wo_v, sem_w.at[3])
    c_wgA = cp(wg_hbm, wg_v, sem_w.at[4], ALL, slice(0, FA))
    c_wuA = cp(wu_hbm, wu_v, sem_w.at[5], ALL, slice(0, FA))
    c_wdA = cp(wd_hbm, wd_v, sem_w.at[6], slice(0, FA), ALL)
    c_wgB = cp(wg_hbm, wg_v, sem_w.at[7], ALL, slice(FA, F))
    c_wuB = cp(wu_hbm, wu_v, sem_w.at[8], ALL, slice(FA, F))
    c_wdB = cp(wd_hbm, wd_v, sem_w.at[9], slice(FA, F), ALL)

    def c_x(t):
        return cp(x_hbm, x_v, sem_x.at[t], tile_rows(t), ALL)

    def c_do(t):
        return cp(dout_hbm, dout_v, sem_do.at[t], tile_rows(t), ALL)

    c_wphi.start()
    c_x(0).start()
    c_wk.start()

    o_out = cp(out_v, out_hbm, sem_out.at[0])
    o_a = (cp(dwg_v, dwg_hbm, sem_out.at[1], ALL, slice(0, FA)),
           cp(dwu_v, dwu_hbm, sem_out.at[2], ALL, slice(0, FA)),
           cp(dwd_v, dwd_hbm, sem_out.at[3], slice(0, FA), ALL))

    def o_dx(t):
        return cp(dx_v, dx_hbm, sem_dx.at[t], tile_rows(t), ALL)

    def o_b(t):
        cb = pl.ds(mo(FA + t * 128, 128), 128)
        return (cp(dwg_v, dwg_hbm, sem_b.at[0, t], ALL, cb),
                cp(dwu_v, dwu_hbm, sem_b.at[1, t], ALL, cb),
                cp(dwd_v, dwd_hbm, sem_b.at[2, t], cb, ALL))

    o_wq = cp(dwqkv_v, dwqkv_hbm, sem_e.at[0], ALL, slice(0, 512))
    o_wkv = cp(dwqkv_v, dwqkv_hbm, sem_e.at[1], ALL, slice(512, 1536))
    o_wo = cp(dwo_v, dwo_hbm, sem_e.at[2])
    o_wphi = cp(dwphi_v, dwphi_hbm, sem_e.at[3])

    RA = D // NTILE
    RD = FA // NTILE

    def row_head(r):
        return (r // 64) * 4 + r % 4

    def row_feat(r):
        return ((r % 64) // 8) * 2 + (r % 8) // 4

    r_i = _iota((128, 128), 0)
    c_i = _iota((128, 128), 1)
    permT = jnp.where((row_head(r_i) == c_i // 16) & (row_feat(r_i) == c_i % 16), 1.0, 0.0).astype(bf16)
    hsel = jnp.where(_iota((32, 512), 0) == (_iota((32, 512), 1) // 16), 1.0, 0.0).astype(bf16)
    dmask = (_iota((256, 512), 0) // 16) == (_iota((256, 512), 1) % 16)
    rsel = jnp.where(row_feat(_iota((128, 256), 0)) == (_iota((128, 256), 1) % 16), 1.0, 0.0).astype(bf16)
    hm4 = row_head(_iota((128, 512), 0)) == ((_iota((128, 512), 1) // 16) % 8)
    ones16 = jnp.ones((16, T), f32)
    zeros8 = jnp.zeros((8, T), f32)
    rr = _iota((80, NG * 128), 0)
    same_head = (rr % 4) == (_iota((80, NG * 128), 1) % 4)

    def fold(part):
        for b in range(NBLK):
            m = pmT_s[:, b * 128:(b + 1) * 128] if part < 2 else permT
            cs = slice(part * 512 + b * 128, part * 512 + (b + 1) * 128)
            wT_s[cs, :] = _dot(m, wqkv_v[:, cs], NT).astype(bf16)

    def w_g(c):
        return wg_v[:, c * FC:(c + 1) * FC]

    def w_u(c):
        return wu_v[:, c * FC:(c + 1) * FC]

    def w_d(c):
        return wd_v[c * FC:(c + 1) * FC, :]

    def ffn_dh(c, dout):
        return _dot(dout, w_d(c), NT)

    def ffn_gu(c, xn):
        return _dot(xn, w_g(c)), _dot(xn, w_u(c))

    def ffn_elem(g_, u_, dh):
        return (g_ * u_).astype(bf16), (dh * u_).astype(bf16), (dh * g_).astype(bf16)

    def ffn_mm(c, h, dg, du):
        o_c = _dot(h, w_d(c))
        d_c = _dot(dg, w_g(c), NT) + _dot(du, w_u(c), NT)
        return o_c, d_c

    def layernorm(t):
        LB = 32
        for r in range(T // LB):
            rows = pl.ds(mo(t * T + r * LB, LB), LB)
            x = x_v[rows, :].astype(f32)
            mu = jnp.mean(x, axis=-1, keepdims=True)
            xc = x - mu
            var = jnp.mean(xc * xc, axis=-1, keepdims=True)
            rstd = jax.lax.rsqrt(var + 1e-5)
            xn_s[rows, :] = (xc * rstd).astype(bf16)
            rstd_s[rows, :] = rstd
        rows = tile_rows(t)
        xn = xn_s[rows, :]
        xnT_s[:, rows] = xn.T
        return xn

    def k_phi(t, xn, b):
        pk = _dot(wT_s[512 + b * 128:512 + (b + 1) * 128, :], xn, NT)
        res = []
        for i in range(2):
            g = 2 * b + i
            phi = _phi(*_dual_softmax(pk[i * 64:(i + 1) * 64]))
            phik_s[g * 128:(g + 1) * 128, tile_rows(t)] = phi
            res.append(phi)
        return res

    def k_acc(t, xn, phis, first=False):
        pv = _dot(wT_s[1024:1536, :], xn, NT)
        for g in range(NG):
            v1 = jnp.concatenate([pv[g * 64:(g + 1) * 64], ones16], axis=0).astype(bf16)
            vT_s[g * 80:(g + 1) * 80, tile_rows(t)] = v1
            r = _dot(v1, phis[g], NT)
            if first:
                kvT_s[:, gl(g)] = r
            else:
                kvT_s[:, gl(g)] += r

    def phase1(t, nxt, extra=None):
        rows = tile_rows(t)
        if nxt is not None:
            xn1 = layernorm(nxt)
        dout = dout_v[rows, :]
        xn = xn_s[rows, :]
        xnT = xnT_s[:, rows]
        nchunk = FA // FC
        phis = []

        def kphi(b):
            if nxt is not None:
                phis.extend(k_phi(nxt, xn1, b))

        st = (ffn_dh(0, dout),) + ffn_gu(0, xn)
        if extra is not None:
            extra[0]()
        kphi(0)
        o_acc = x_v[rows, :].astype(f32)
        d_acc = None
        for c in range(nchunk):
            cs = slice(c * FC, (c + 1) * FC)
            dh, g_, u_ = st
            if c + 1 < nchunk:
                dh1 = ffn_dh(c + 1, dout)
            h, dg, du = ffn_elem(g_, u_, dh)
            if c + 1 < nchunk:
                st = (dh1,) + ffn_gu(c + 1, xn)
            if extra is not None and c == 0:
                extra[1]()
            if c == 0:
                kphi(1)
            dwg_s[:, cs] += _dot(xnT, dg)
            if c == 0:
                kphi(2)
            dwu_s[:, cs] += _dot(xnT, du)
            if c == 0:
                kphi(3)
            dwd_s[cs, :] += _dot(h, dout, TN)
            if c == 1 and nxt is not None:
                k_acc(nxt, xn1, phis)
            o_c, d_c = ffn_mm(c, h, dg, du)
            o_acc = o_acc + o_c
            d_acc = d_c if d_acc is None else d_acc + d_c
        out_s[rows, :] = o_acc
        dxn_s[rows, :] = d_acc

    dwg_s[...] = jnp.zeros_like(dwg_s)
    dwu_s[...] = jnp.zeros_like(dwu_s)
    dwd_s[...] = jnp.zeros_like(dwd_s)
    c_wphi.wait()
    w3 = wphi_v[...].reshape(256, 32)
    ym = jnp.where(dmask, _dot(w3, hsel), 0.0).astype(bf16)
    pmT_s[...] = jnp.where(hm4, _dot(rsel, ym), 0.0).astype(bf16)
    c_wv.start()
    c_x(1).start()
    c_x(0).wait()
    xn0 = layernorm(0)
    c_wk.wait()
    c_wdA.start()
    c_wgA.start()
    fold(1)
    for b in range(NBLK):
        k_phi(0, xn0, b)
    c_wv.wait()
    c_x(1).wait()
    c_wuA.start()
    c_do(0).start()
    c_x(2).start()
    xn1 = layernorm(1)
    fold(2)
    k_acc(0, xn_s[0:T, :], [phik_s[g * 128:(g + 1) * 128, 0:T] for g in range(NG)], first=True)
    k_acc(1, xn1, sum([k_phi(1, xn1, b) for b in range(NBLK)], []))
    c_wdA.wait()
    c_wgA.wait()
    c_wuA.wait()
    c_do(1).start()
    c_do(2).start()
    for t in range(3, NTILE):
        c_x(t).start()
        c_do(t).start()
    c_wq.start()
    c_wo.start()
    c_wgB.start()
    c_wuB.start()
    c_wdB.start()

    def p1_body(t, carry):
        c_do(t).wait()
        c_x(t + 2).wait()
        phase1(t, t + 2)
        return carry

    jax.lax.fori_loop(0, NTILE - 2, p1_body, 0)
    c_do(NTILE - 2).wait()
    c_do(NTILE - 1).wait()

    c_wq.wait()
    c_wo.wait()

    def transposed(kv, dst):
        m = jnp.where(same_head & (rr < 68), kv, 0.0)
        m = jnp.concatenate([m, jnp.zeros((48, NG * 128), f32)], axis=0)
        for g in range(NG):
            dst[:, gl(g)] = m[:, gl(g)].T.astype(bf16)

    def extra0():
        kv = kvT_s[...]
        kvz_s[...] = jnp.where(same_head & (rr < 72), kv, 0.0).astype(bf16)
        transposed(kv, kv4_s)

    def extra1():
        dkvT_s[...] = jnp.zeros_like(dkvT_s)
        gT_s[...] = jnp.zeros_like(gT_s)
        dwo_s[...] = jnp.zeros_like(dwo_s)
        fold(0)
        for b in range(NBLK):
            wop_s[b * 128:(b + 1) * 128, :] = _dot(permT, wo_v[b * 128:(b + 1) * 128, :]).astype(bf16)

    phase1(NTILE - 2, None, (extra0, extra1))
    phase1(NTILE - 1, None)
    c_wgB.wait()
    c_wuB.wait()
    c_wdB.wait()

    c0 = FA // FC

    def phase2(t, carry):
        rows = tile_rows(t)
        xn = xn_s[rows, :]
        dout = dout_v[rows, :]
        acc = {}

        def ffn1(c):
            return (ffn_dh(c, dout),) + ffn_gu(c, xn)

        def elem(c, st):
            dh, g_, u_ = st
            h, dg, du = ffn_elem(g_, u_, dh)
            cs = slice((c - c0) * FC, (c - c0 + 1) * FC)
            h_s[rows, cs] = h
            dg_s[rows, cs] = dg
            du_s[rows, cs] = du
            return h, dg, du

        def mm(c, e):
            o_c, d_c = ffn_mm(c, *e)
            acc['o'] = o_c + acc['o']
            acc['d'] = d_c + acc['d']

        pq = _dot(wT_s[0:512, :], xn, NT)
        ab = [_dual_softmax(pq[g * 64:(g + 1) * 64]) for g in range(NG)]
        phis = [_phi(a, b) for a, b in ab]
        doT = _dot(wop_s[...], dout, NT)
        oTs, dn1s, dpqs = [], [], []

        def stage2(b):
            for g in (2 * b, 2 * b + 1):
                nd = _dot(kvz_s[:, gl(g)], phis[g])
                rden = 1.0 / (nd[64:72] + 1e-6)
                o3 = nd[0:64].reshape(8, 8, T) * rden[None]
                do3 = doT[g * 64:(g + 1) * 64].reshape(8, 8, T)
                dden = -_hsum(do3 * o3) * rden
                dn1s.append(jnp.concatenate([(do3 * rden[None]).reshape(64, T), dden, zeros8], axis=0).astype(bf16))
                oTs.append(o3.reshape(64, T))

        def stage3(b):
            for g in (2 * b, 2 * b + 1):
                dphi = _dot(kv4_s[:, g * 128:g * 128 + 80], dn1s[g]).reshape(16, 8, T)
                a, b_ = ab[g]
                dpqs.append(_dual_softmax_bwd(a, b_, dphi[0:8], dphi[8:16]).reshape(64, T))

        dh0 = ffn_dh(c0, dout)
        g0 = _dot(xn, w_g(c0))
        stage2(0)
        u0 = _dot(xn, w_u(c0))
        stage2(1)
        dh1 = ffn_dh(c0 + 1, dout)
        stage2(2)
        g1 = _dot(xn, w_g(c0 + 1))
        stage2(3)
        e0 = elem(c0, (dh0, g0, u0))
        u1 = _dot(xn, w_u(c0 + 1))
        st1 = (dh1, g1, u1)
        stage3(0)
        acc['o'] = _dot(e0[0], w_d(c0))
        stage3(1)
        acc['d'] = _dot(e0[1], w_g(c0), NT)
        stage3(2)
        acc['d'] = acc['d'] + _dot(e0[2], w_u(c0), NT)
        stage3(3)
        dpq = jnp.concatenate(dpqs, axis=0).astype(bf16)
        oT = jnp.concatenate(oTs, axis=0).astype(bf16)
        for g in range(NG):
            dkvT_s[:, gl(g)] += _dot(dn1s[g], phis[g], NT)
        e1 = elem(c0 + 1, st1)
        dwo_s[...] += _dot(oT, dout)
        acc['o'] = acc['o'] + _dot(oT, wop_s[...], TN)
        st2 = ffn1(c0 + 2)
        ra = pl.ds(pl.multiple_of(t * RA, RA), RA)
        rd = pl.ds(pl.multiple_of(t * RD, RD), RD)
        dwg_v[ra, 0:FA] = dwg_s[ra, :].astype(bf16)
        dwu_v[ra, 0:FA] = dwu_s[ra, :].astype(bf16)
        dwd_v[rd, :] = dwd_s[rd, :].astype(bf16)
        mm(c0 + 1, e1)
        e2 = elem(c0 + 2, st2)
        st3 = ffn1(c0 + 3)
        mm(c0 + 2, e2)
        e3 = elem(c0 + 3, st3)
        gT_s[0:512, :] += _dot(dpq, xn)
        mm(c0 + 3, e3)
        out_v[rows, :] = (out_s[rows, :] + acc['o']).astype(bf16)
        dxn_s[rows, :] += acc['d'] + _dot(dpq, wT_s[0:512, :], TN)
        return carry

    jax.lax.fori_loop(0, NTILE, phase2, 0, unroll=2)
    o_out.start()
    for cpy in o_a:
        cpy.start()

    dkv = dkvT_s[...]
    dkv4_s[...] = jnp.where(same_head, dkv, 0.0).astype(bf16)
    transposed(dkv, dkv4T_s)

    def unfold(part):
        for b in range(NBLK):
            m = pmT_s[:, b * 128:(b + 1) * 128] if part < 2 else permT
            cs = slice(part * 512 + b * 128, part * 512 + (b + 1) * 128)
            gblk = gT_s[cs, :].astype(bf16)
            dwqkv_v[:, cs] = _dot(gblk, m, TN).astype(bf16)
            if part == 0:
                aphi_s[:, b * 128:(b + 1) * 128] = _dot(gblk, wqkv_v[:, cs])
            elif part == 1:
                aphi_s[:, b * 128:(b + 1) * 128] += _dot(gblk, wqkv_v[:, cs])
        if part == 1:
            accm = jnp.where(hm4, aphi_s[...], 0.0).astype(bf16)
            z = jnp.where(dmask, _dot(rsel, accm, TN), 0.0).astype(bf16)
            dwphi_v[...] = _dot(z, hsel, NT).astype(bf16).reshape(16, 16, 32)

    unfold(0)
    for b in range(NBLK):
        dwo_v[b * 128:(b + 1) * 128, :] = _dot(permT, dwo_s[b * 128:(b + 1) * 128, :].astype(bf16), TN).astype(bf16)
    o_wq.start()
    o_wo.start()

    def wgrad_gu(t, r0=0, r1=D):
        cl = pl.ds(mo(t * 128, 128), 128)
        cb = pl.ds(mo(FA + t * 128, 128), 128)
        dgu = _dot(xnT_s[r0:r1, :], jnp.concatenate([dg_s[:, cl], du_s[:, cl]], axis=1))
        dwg_v[r0:r1, cb] = dgu[:, 0:128].astype(bf16)
        dwu_v[r0:r1, cb] = dgu[:, 128:256].astype(bf16)

    def wgrad_d(t, n0, n1):
        cl = pl.ds(mo(t * 128, 128), 128)
        cb = pl.ds(mo(FA + t * 128, 128), 128)
        dwd_v[cb, n0:n1] = _dot(h_s[:, cl], dout_v[:, n0:n1], TN).astype(bf16)

    def phase3(t, last):
        rows = tile_rows(t)
        xn = xn_s[rows, :]
        phis = [phik_s[g * 128:(g + 1) * 128, rows] for g in range(NG)]

        def sm_bwd(b):
            for g in (2 * b, 2 * b + 1):
                dphi = _dot(dkv4T_s[:, g * 128:g * 128 + 80], vT_s[g * 80:(g + 1) * 80, rows]).reshape(16, 8, T)
                phif = phis[g].astype(f32).reshape(16, 8, T)
                dp = _dual_softmax_bwd(phif[0:8], phif[8:16], dphi[0:8], dphi[8:16])
                dp_s[g * 64:(g + 1) * 64, :] = dp.reshape(64, T).astype(bf16)

        sm_bwd(0)
        for g in range(NG):
            dp_s[512 + g * 64:512 + (g + 1) * 64, :] = _dot(dkv4_s[0:64, gl(g)], phis[g]).astype(bf16)
        sm_bwd(1)
        wgrad_d(t, 0, 256)
        sm_bwd(2)
        wgrad_d(t, 256, 384)
        sm_bwd(3)
        wgrad_d(t, 384, 512)

        def ln_part(r, n):
            LB = T // n
            rw = pl.ds(mo(t * T + r * LB, LB), LB)
            dxn = dxn_s[rw, :] + _dot(dp_s[:, r * LB:(r + 1) * LB], wT_s[512:1536, :], TN)
            xnf = xn_s[rw, :].astype(f32)
            m1 = jnp.mean(dxn, axis=-1, keepdims=True)
            m2 = jnp.mean(dxn * xnf, axis=-1, keepdims=True)
            dx = rstd_s[rw, :] * (dxn - m1 - xnf * m2) + dout_v[rw, :].astype(f32)
            dx_v[rw, :] = dx.astype(bf16)

        ln_part(0, 2)
        gT_s[512:1024, :] += _dot(dp_s[0:512, :], xn)
        ln_part(1, 2)
        gT_s[1024:1536, :] += _dot(dp_s[512:1024, :], xn)
        ob = o_b(t)
        if last:
            unfold(1)
            unfold(2)
            wgrad_gu(t, 0, SPLIT)
            o_dx(t).start()
            ob[2].start()
            o_wkv.start()
            o_wphi.start()
            wgrad_gu(t, SPLIT, D)
            ob[0].start()
            ob[1].start()
        else:
            wgrad_gu(t)
            o_dx(t).start()
            for cpy in ob:
                cpy.start()

    def p3_body(t, carry):
        phase3(t, False)
        return carry

    jax.lax.fori_loop(0, NTILE - 1, p3_body, 0)
    phase3(NTILE - 1, True)

    o_out.wait()
    for cpy in o_a:
        cpy.wait()
    o_wq.wait()
    o_wo.wait()
    for t in range(NTILE):
        o_dx(t).wait()
    o_wkv.wait()
    o_wphi.wait()
    for t in range(NTILE):
        for cpy in o_b(t):
            cpy.wait()


@jax.jit
def pallas_parallel_sum__linear_kernel_hedgehog__glu_gated_bilinear__prompt_kernel(A_x, A_wqkv, A_w_phi, A_wo, B_x, B_w_gate, B_w_up, B_w_down, grad_out):
    x = A_x.reshape(S, D)
    dout = grad_out.reshape(S, D)
    wphi = jnp.transpose(A_w_phi, (1, 2, 0))
    sds = jax.ShapeDtypeStruct
    io_shapes = ((S, D), (S, D), (D, 3 * D), (DH, DH, H), (D, D), (D, F), (D, F), (F, D))
    any_spec = pl.BlockSpec(memory_space=pl.ANY)

    def packed(r, c):
        return pltpu.VMEM((r // 2, c), u32)

    io_scratch = [pltpu.VMEM(s, bf16) if len(s) == 3 else packed(*s) for s in io_shapes]
    dma = pltpu.SemaphoreType.DMA
    outs = pl.pallas_call(
        kernel,
        out_shape=tuple(sds(s, bf16) for s in io_shapes),
        in_specs=[any_spec] * 8,
        out_specs=tuple([any_spec] * 8),
        scratch_shapes=io_scratch + io_scratch + [
            packed(3 * D, D),
            packed(D, D),
            packed(128, 512),
            packed(S, D),
            packed(D, S),
            packed(NG * 128, S),
            packed(NG * 80, S),
            packed(80, NG * 128),
            packed(128, NG * 128),
            packed(80, NG * 128),
            packed(128, NG * 128),
            packed(S, FB),
            packed(S, FB),
            packed(S, FB),
            packed(2 * D, T),
            pltpu.VMEM((S, 1), f32),
            pltpu.VMEM((80, NG * 128), f32),
            pltpu.VMEM((80, NG * 128), f32),
            pltpu.VMEM((3 * D, D), f32),
            pltpu.VMEM((D, D), f32),
            pltpu.VMEM((D, FA), f32),
            pltpu.VMEM((D, FA), f32),
            pltpu.VMEM((FA, D), f32),
            pltpu.VMEM((S, D), f32),
            pltpu.VMEM((S, D), f32),
            pltpu.VMEM((128, 512), f32),
            dma((11,)), dma((NTILE,)), dma((NTILE,)), dma((4,)), dma((NTILE,)),
            dma((3, NTILE)), dma((4,)),
        ],
        compiler_params=pltpu.CompilerParams(vmem_limit_bytes=110 * 1024 * 1024),
    )(x, A_wqkv, wphi, A_wo, B_w_gate, B_w_up, B_w_down, dout)
    out, dx, dwqkv, dwphi, dwo, dwg, dwu, dwd = outs
    return (out.reshape(1, S, D), dx.reshape(1, S, D), dwqkv, jnp.transpose(dwphi, (2, 0, 1)), dwo, dwg, dwu, dwd)
```

```python
import jax
import jax.numpy as jnp
import jax.experimental.pallas as pl
import jax.experimental.pallas.tpu as pltpu

S, D, H, DH, F = 2048, 512, 32, 16, 1792
NG = 8
NBLK = 4
T = 256
NTILE = S // T
FC = 256
FA = 768
FA1 = 512
FB = F - FA
SPLIT = 128

f32 = jnp.float32
bf16 = jnp.bfloat16
u32 = jnp.uint32
NN = (((1,), (0,)), ((), ()))
NT = (((1,), (1,)), ((), ()))
TN = (((0,), (0,)), ((), ()))


def _dot(a, b, dn=NN):
    return jax.lax.dot_general(a, b, dn, preferred_element_type=f32)


def _head_reduce(x3, red, comb):
    r = red(x3, axis=0)
    return comb(r, pltpu.roll(r, 4, 0))


def _hsum(x3):
    return _head_reduce(x3, jnp.sum, jnp.add)


def _dual_softmax(p):
    p3 = p.reshape(8, 8, p.shape[-1])
    mx = _head_reduce(p3, jnp.max, jnp.maximum)
    mn = _head_reduce(p3, jnp.min, jnp.minimum)
    ea = jnp.exp(p3 - mx[None])
    eb = jnp.exp(mn[None] - p3)
    a = ea * (1.0 / _hsum(ea))[None]
    b = eb * (1.0 / _hsum(eb))[None]
    return a, b


def _dual_softmax_bwd(a, b, da, db):
    ta = a * da
    tb = b * db
    return (ta - a * _hsum(ta)[None]) - (tb - b * _hsum(tb)[None])


def _phi(a, b):
    return jnp.concatenate([a.reshape(64, T), b.reshape(64, T)], axis=0).astype(bf16)


def _iota(shape, dim):
    return jax.lax.broadcasted_iota(jnp.int32, shape, dim)


def kernel(x_hbm, wqkv_hbm, wphi_hbm, wo_hbm, wg_hbm, wu_hbm, wd_hbm, dout_hbm,
           out_hbm, dx_hbm, dwqkv_hbm, dwphi_hbm, dwo_hbm, dwg_hbm, dwu_hbm, dwd_hbm,
           x_v, dout_v, wqkv_v, wphi_v, wo_v, wg_v, wu_v, wd_v,
           out_v, dx_v, dwqkv_v, dwphi_v, dwo_v, dwg_v, dwu_v, dwd_v,
           wT_s, wop_s, pmT_s, xn_s, xnT_s, phik_s, vT_s, kvz_s, kv4_s, dkv4_s, dkv4T_s, h_s, dg_s, du_s, dp_s,
           rstd_s, kvT_s, dkvT_s, gT_s, dwo_s, dwg_s, dwu_s, dwd_s, out_s, dxn_s, aphi_s,
           sem):
    (x_v, dout_v, wqkv_v, wo_v, wg_v, wu_v, wd_v, out_v, dx_v, dwqkv_v, dwo_v, dwg_v, dwu_v, dwd_v,
     wT_s, wop_s, pmT_s, xn_s, xnT_s, phik_s, vT_s, kvz_s, kv4_s, dkv4_s, dkv4T_s, h_s, dg_s, du_s, dp_s) = [
         r.bitcast(bf16) for r in (
             x_v, dout_v, wqkv_v, wo_v, wg_v, wu_v, wd_v, out_v, dx_v, dwqkv_v, dwo_v, dwg_v, dwu_v, dwd_v,
             wT_s, wop_s, pmT_s, xn_s, xnT_s, phik_s, vT_s, kvz_s, kv4_s, dkv4_s, dkv4T_s, h_s, dg_s, du_s, dp_s)]
    ALL = slice(None)

    def cp(src, dst, sem, *idx):
        if idx:
            src, dst = src.at[idx], dst.at[idx]
        return pltpu.make_async_copy(src, dst, sem)

    def mo(v, m):
        return v if isinstance(v, int) else pl.multiple_of(v, m)

    def tile_rows(t):
        return pl.ds(mo(t * T, T), T)

    def gl(g):
        return slice(g * 128, (g + 1) * 128)

    c_wphi = cp(wphi_hbm, wphi_v, sem.at[6])
    c_wk = cp(wqkv_hbm, wqkv_v, sem.at[8], ALL, slice(512, 1024))
    c_wv = cp(wqkv_hbm, wqkv_v, sem.at[9], ALL, slice(1024, 1536))
    c_wq = cp(wqkv_hbm, wqkv_v, sem.at[11], ALL, slice(0, 512))
    c_wo = cp(wo_hbm, wo_v, sem.at[11])
    c_wgA = cp(wg_hbm, wg_v, sem.at[10], ALL, slice(0, FA1))
    c_wuA = cp(wu_hbm, wu_v, sem.at[10], ALL, slice(0, FA1))
    c_wdA = cp(wd_hbm, wd_v, sem.at[10], slice(0, FA1), ALL)
    c_wgB = cp(wg_hbm, wg_v, sem.at[11], ALL, slice(FA1, F))
    c_wuB = cp(wu_hbm, wu_v, sem.at[11], ALL, slice(FA1, F))
    c_wdB = cp(wd_hbm, wd_v, sem.at[11], slice(FA1, F), ALL)
    sem_o = sem.at[12]

    def c_x(t):
        s = {0: 7, 1: 9}.get(t, t - 2) if isinstance(t, int) else t - 2
        return cp(x_hbm, x_v, sem.at[s], tile_rows(t), ALL)

    def c_do(t):
        s = (t if t < NTILE - 2 else 11) if isinstance(t, int) else t
        return cp(dout_hbm, dout_v, sem.at[s], tile_rows(t), ALL)

    c_wphi.start()
    c_x(0).start()
    c_wk.start()

    o_out = cp(out_v, out_hbm, sem_o)
    o_a = (cp(dwg_v, dwg_hbm, sem_o, ALL, slice(0, FA)),
           cp(dwu_v, dwu_hbm, sem_o, ALL, slice(0, FA)),
           cp(dwd_v, dwd_hbm, sem_o, slice(0, FA), ALL))

    def o_dx(t):
        return cp(dx_v, dx_hbm, sem_o, tile_rows(t), ALL)

    def o_b(t):
        cb = pl.ds(mo(FA + t * 128, 128), 128)
        return (cp(dwg_v, dwg_hbm, sem_o, ALL, cb),
                cp(dwu_v, dwu_hbm, sem_o, ALL, cb),
                cp(dwd_v, dwd_hbm, sem_o, cb, ALL))

    o_wq = cp(dwqkv_v, dwqkv_hbm, sem_o, ALL, slice(0, 512))
    o_wkv = cp(dwqkv_v, dwqkv_hbm, sem_o, ALL, slice(512, 1536))
    o_wo = cp(dwo_v, dwo_hbm, sem_o)
    o_wphi = cp(dwphi_v, dwphi_hbm, sem_o)

    RA = D // NTILE
    RD = FA1 // NTILE

    def row_head(r):
        return (r // 64) * 4 + r % 4

    def row_feat(r):
        return ((r % 64) // 8) * 2 + (r % 8) // 4

    r_i = _iota((128, 128), 0)
    c_i = _iota((128, 128), 1)
    permT = jnp.where((row_head(r_i) == c_i // 16) & (row_feat(r_i) == c_i % 16), 1.0, 0.0).astype(bf16)
    hsel = jnp.where(_iota((32, 512), 0) == (_iota((32, 512), 1) // 16), 1.0, 0.0).astype(bf16)
    dmask = (_iota((256, 512), 0) // 16) == (_iota((256, 512), 1) % 16)
    rsel = jnp.where(row_feat(_iota((128, 256), 0)) == (_iota((128, 256), 1) % 16), 1.0, 0.0).astype(bf16)
    hm4 = row_head(_iota((128, 512), 0)) == ((_iota((128, 512), 1) // 16) % 8)
    ones16 = jnp.ones((16, T), f32)
    zeros8 = jnp.zeros((8, T), f32)
    rr = _iota((80, NG * 128), 0)
    same_head = (rr % 4) == (_iota((80, NG * 128), 1) % 4)

    def fold(part):
        for b in range(NBLK):
            m = pmT_s[:, b * 128:(b + 1) * 128] if part < 2 else permT
            cs = slice(part * 512 + b * 128, part * 512 + (b + 1) * 128)
            wT_s[cs, :] = _dot(m, wqkv_v[:, cs], NT).astype(bf16)

    def w_g(c):
        return wg_v[:, c * FC:(c + 1) * FC]

    def w_u(c):
        return wu_v[:, c * FC:(c + 1) * FC]

    def w_d(c):
        return wd_v[c * FC:(c + 1) * FC, :]

    def ffn_dh(c, dout):
        return _dot(dout, w_d(c), NT)

    def ffn_gu(c, xn):
        return _dot(xn, w_g(c)), _dot(xn, w_u(c))

    def ffn_elem(g_, u_, dh):
        return (g_ * u_).astype(bf16), (dh * u_).astype(bf16), (dh * g_).astype(bf16)

    def ffn_mm(c, h, dg, du):
        o_c = _dot(h, w_d(c))
        d_c = _dot(dg, w_g(c), NT) + _dot(du, w_u(c), NT)
        return o_c, d_c

    def layernorm(t):
        LB = 32
        for r in range(T // LB):
            rows = pl.ds(mo(t * T + r * LB, LB), LB)
            x = x_v[rows, :].astype(f32)
            mu = jnp.mean(x, axis=-1, keepdims=True)
            xc = x - mu
            var = jnp.mean(xc * xc, axis=-1, keepdims=True)
            rstd = jax.lax.rsqrt(var + 1e-5)
            xn_s[rows, :] = (xc * rstd).astype(bf16)
            rstd_s[rows, :] = rstd
        rows = tile_rows(t)
        xn = xn_s[rows, :]
        xnT_s[:, rows] = xn.T
        return xn

    def k_phi(t, xn, b):
        pk = _dot(wT_s[512 + b * 128:512 + (b + 1) * 128, :], xn, NT)
        res = []
        for i in range(2):
            g = 2 * b + i
            phi = _phi(*_dual_softmax(pk[i * 64:(i + 1) * 64]))
            phik_s[g * 128:(g + 1) * 128, tile_rows(t)] = phi
            res.append(phi)
        return res

    def k_acc(t, xn, phis, first=False):
        pv = _dot(wT_s[1024:1536, :], xn, NT)
        for g in range(NG):
            v1 = jnp.concatenate([pv[g * 64:(g + 1) * 64], ones16], axis=0).astype(bf16)
            vT_s[g * 80:(g + 1) * 80, tile_rows(t)] = v1
            r = _dot(v1, phis[g], NT)
            if first:
                kvT_s[:, gl(g)] = r
            else:
                kvT_s[:, gl(g)] += r

    def phase1(t, nxt, extra=None):
        rows = tile_rows(t)
        if nxt is not None:
            xn1 = layernorm(nxt)
        dout = dout_v[rows, :]
        xn = xn_s[rows, :]
        xnT = xnT_s[:, rows]
        nchunk = FA1 // FC
        phis = []

        def kphi(b):
            if nxt is not None:
                phis.extend(k_phi(nxt, xn1, b))

        st = (ffn_dh(0, dout),) + ffn_gu(0, xn)
        if extra is not None:
            extra[0]()
        kphi(0)
        o_acc = x_v[rows, :].astype(f32)
        d_acc = None
        for c in range(nchunk):
            cs = slice(c * FC, (c + 1) * FC)
            dh, g_, u_ = st
            if c + 1 < nchunk:
                dh1 = ffn_dh(c + 1, dout)
            h, dg, du = ffn_elem(g_, u_, dh)
            if c + 1 < nchunk:
                st = (dh1,) + ffn_gu(c + 1, xn)
            if extra is not None and c == 0:
                extra[1]()
            if c == 0:
                kphi(1)
            dwg_s[:, cs] += _dot(xnT, dg)
            if c == 0:
                kphi(2)
            dwu_s[:, cs] += _dot(xnT, du)
            if c == 0:
                kphi(3)
            dwd_s[cs, :] += _dot(h, dout, TN)
            if c == 1 and nxt is not None:
                k_acc(nxt, xn1, phis)
            o_c, d_c = ffn_mm(c, h, dg, du)
            o_acc = o_acc + o_c
            d_acc = d_c if d_acc is None else d_acc + d_c
        out_s[rows, :] = o_acc
        dxn_s[rows, :] = d_acc

    dwg_s[...] = jnp.zeros_like(dwg_s)
    dwu_s[...] = jnp.zeros_like(dwu_s)
    dwd_s[...] = jnp.zeros_like(dwd_s)
    c_wphi.wait()
    w3 = wphi_v[...].reshape(256, 32)
    ym = jnp.where(dmask, _dot(w3, hsel), 0.0).astype(bf16)
    pmT_s[...] = jnp.where(hm4, _dot(rsel, ym), 0.0).astype(bf16)
    c_wv.start()
    c_x(1).start()
    c_x(0).wait()
    xn0 = layernorm(0)
    c_wk.wait()
    c_wdA.start()
    c_wgA.start()
    fold(1)
    for b in range(NBLK):
        k_phi(0, xn0, b)
    c_wv.wait()
    c_x(1).wait()
    c_wuA.start()
    c_do(0).start()
    c_x(2).start()
    xn1 = layernorm(1)
    fold(2)
    k_acc(0, xn_s[0:T, :], [phik_s[g * 128:(g + 1) * 128, 0:T] for g in range(NG)], first=True)
    k_acc(1, xn1, sum([k_phi(1, xn1, b) for b in range(NBLK)], []))
    c_wdA.wait()
    c_wgA.wait()
    c_wuA.wait()
    c_do(1).start()
    c_do(2).start()
    for t in range(3, NTILE):
        c_x(t).start()
        c_do(t).start()
    c_wq.start()
    c_wo.start()
    c_wgB.start()
    c_wuB.start()
    c_wdB.start()

    def p1_body(t, carry):
        c_do(t).wait()
        c_x(t + 2).wait()
        phase1(t, t + 2)
        return carry

    jax.lax.fori_loop(0, NTILE - 2, p1_body, 0)
    c_do(NTILE - 2).wait()
    c_do(NTILE - 1).wait()

    c_wq.wait()
    c_wo.wait()
    c_wgB.wait()
    c_wuB.wait()
    c_wdB.wait()

    def transposed(kv, dst):
        m = jnp.where(same_head & (rr < 68), kv, 0.0)
        m = jnp.concatenate([m, jnp.zeros((48, NG * 128), f32)], axis=0)
        for g in range(NG):
            dst[:, gl(g)] = m[:, gl(g)].T.astype(bf16)

    def extra0():
        kv = kvT_s[...]
        kvz_s[...] = jnp.where(same_head & (rr < 72), kv, 0.0).astype(bf16)
        transposed(kv, kv4_s)

    def extra1():
        dkvT_s[...] = jnp.zeros_like(dkvT_s)
        gT_s[...] = jnp.zeros_like(gT_s)
        dwo_s[...] = jnp.zeros_like(dwo_s)
        fold(0)
        for b in range(NBLK):
            wop_s[b * 128:(b + 1) * 128, :] = _dot(permT, wo_v[b * 128:(b + 1) * 128, :]).astype(bf16)

    phase1(NTILE - 2, None, (extra0, extra1))
    phase1(NTILE - 1, None)

    c0 = FA // FC

    def phase2(t, carry):
        rows = tile_rows(t)
        xn = xn_s[rows, :]
        dout = dout_v[rows, :]
        acc = {}

        def ffn1(c):
            return (ffn_dh(c, dout),) + ffn_gu(c, xn)

        def elem(c, st):
            dh, g_, u_ = st
            h, dg, du = ffn_elem(g_, u_, dh)
            cs = slice((c - c0) * FC, (c - c0 + 1) * FC)
            h_s[rows, cs] = h
            dg_s[rows, cs] = dg
            du_s[rows, cs] = du
            return h, dg, du

        def mm(c, e):
            o_c, d_c = ffn_mm(c, *e)
            acc['o'] = o_c + acc['o']
            acc['d'] = d_c + acc['d']

        pq = _dot(wT_s[0:512, :], xn, NT)
        ab = [_dual_softmax(pq[g * 64:(g + 1) * 64]) for g in range(NG)]
        phis = [_phi(a, b) for a, b in ab]
        doT = _dot(wop_s[...], dout, NT)
        oTs, dn1s, dpqs = [], [], []

        def stage2(b):
            for g in (2 * b, 2 * b + 1):
                nd = _dot(kvz_s[:, gl(g)], phis[g])
                rden = 1.0 / (nd[64:72] + 1e-6)
                o3 = nd[0:64].reshape(8, 8, T) * rden[None]
                do3 = doT[g * 64:(g + 1) * 64].reshape(8, 8, T)
                dden = -_hsum(do3 * o3) * rden
                dn1s.append(jnp.concatenate([(do3 * rden[None]).reshape(64, T), dden, zeros8], axis=0).astype(bf16))
                oTs.append(o3.reshape(64, T))

        def stage3(b):
            for g in (2 * b, 2 * b + 1):
                dphi = _dot(kv4_s[:, g * 128:g * 128 + 80], dn1s[g]).reshape(16, 8, T)
                a, b_ = ab[g]
                dpqs.append(_dual_softmax_bwd(a, b_, dphi[0:8], dphi[8:16]).reshape(64, T))

        dh0 = ffn_dh(c0, dout)
        g0 = _dot(xn, w_g(c0))
        stage2(0)
        u0 = _dot(xn, w_u(c0))
        stage2(1)
        dh1 = ffn_dh(c0 + 1, dout)
        stage2(2)
        g1 = _dot(xn, w_g(c0 + 1))
        stage2(3)
        e0 = elem(c0, (dh0, g0, u0))
        u1 = _dot(xn, w_u(c0 + 1))
        st1 = (dh1, g1, u1)
        stage3(0)
        acc['o'] = _dot(e0[0], w_d(c0))
        stage3(1)
        acc['d'] = _dot(e0[1], w_g(c0), NT)
        stage3(2)
        acc['d'] = acc['d'] + _dot(e0[2], w_u(c0), NT)
        stage3(3)
        dpq = jnp.concatenate(dpqs, axis=0).astype(bf16)
        oT = jnp.concatenate(oTs, axis=0).astype(bf16)
        for g in range(NG):
            dkvT_s[:, gl(g)] += _dot(dn1s[g], phis[g], NT)
        e1 = elem(c0 + 1, st1)
        dwo_s[...] += _dot(oT, dout)
        acc['o'] = acc['o'] + _dot(oT, wop_s[...], TN)
        st2 = ffn1(c0 + 2)
        ra = pl.ds(pl.multiple_of(t * RA, RA), RA)
        rd = pl.ds(pl.multiple_of(t * RD, RD), RD)
        dwg_v[ra, 0:FA1] = dwg_s[ra, 0:FA1].astype(bf16)
        dwu_v[ra, 0:FA1] = dwu_s[ra, 0:FA1].astype(bf16)
        dwd_v[rd, :] = dwd_s[rd, :].astype(bf16)
        mm(c0 + 1, e1)
        e2 = elem(c0 + 2, st2)
        st3 = ffn1(c0 + 3)
        mm(c0 + 2, e2)
        e3 = elem(c0 + 3, st3)
        st4 = ffn1(c0 - 1)
        mm(c0 + 3, e3)
        e4 = ffn_elem(st4[1], st4[2], st4[0])
        gT_s[0:512, :] += _dot(dpq, xn)
        xnT = xnT_s[:, rows]
        dwg_s[:, FA1:FA] += _dot(xnT, e4[1])
        dwu_s[:, FA1:FA] += _dot(xnT, e4[2])
        dwd_s[FA1:FA, :] += _dot(e4[0], dout, TN)
        mm(c0 - 1, e4)
        out_v[rows, :] = (out_s[rows, :] + acc['o']).astype(bf16)
        dxn_s[rows, :] += acc['d'] + _dot(dpq, wT_s[0:512, :], TN)
        return carry

    jax.lax.fori_loop(0, NTILE, phase2, 0)
    o_out.start()

    dwg_v[:, FA1:FA] = dwg_s[:, FA1:FA].astype(bf16)
    dwu_v[:, FA1:FA] = dwu_s[:, FA1:FA].astype(bf16)
    dwd_v[FA1:FA, :] = dwd_s[FA1:FA, :].astype(bf16)
    dkv = dkvT_s[...]
    dkv4_s[...] = jnp.where(same_head, dkv, 0.0).astype(bf16)
    transposed(dkv, dkv4T_s)

    def unfold(part):
        for b in range(NBLK):
            m = pmT_s[:, b * 128:(b + 1) * 128] if part < 2 else permT
            cs = slice(part * 512 + b * 128, part * 512 + (b + 1) * 128)
            gblk = gT_s[cs, :].astype(bf16)
            dwqkv_v[:, cs] = _dot(gblk, m, TN).astype(bf16)
            if part == 0:
                aphi_s[:, b * 128:(b + 1) * 128] = _dot(gblk, wqkv_v[:, cs])
            elif part == 1:
                aphi_s[:, b * 128:(b + 1) * 128] += _dot(gblk, wqkv_v[:, cs])
        if part == 1:
            accm = jnp.where(hm4, aphi_s[...], 0.0).astype(bf16)
            z = jnp.where(dmask, _dot(rsel, accm, TN), 0.0).astype(bf16)
            dwphi_v[...] = _dot(z, hsel, NT).astype(bf16).reshape(16, 16, 32)

    unfold(0)
    for b in range(NBLK):
        dwo_v[b * 128:(b + 1) * 128, :] = _dot(permT, dwo_s[b * 128:(b + 1) * 128, :].astype(bf16), TN).astype(bf16)
    o_wq.start()
    o_wo.start()
    for cpy in o_a:
        cpy.start()

    def wgrad_gu(t, r0=0, r1=D):
        cl = pl.ds(mo(t * 128, 128), 128)
        cb = pl.ds(mo(FA + t * 128, 128), 128)
        dgu = _dot(xnT_s[r0:r1, :], jnp.concatenate([dg_s[:, cl], du_s[:, cl]], axis=1))
        dwg_v[r0:r1, cb] = dgu[:, 0:128].astype(bf16)
        dwu_v[r0:r1, cb] = dgu[:, 128:256].astype(bf16)

    def wgrad_d(t, n0, n1):
        cl = pl.ds(mo(t * 128, 128), 128)
        cb = pl.ds(mo(FA + t * 128, 128), 128)
        dwd_v[cb, n0:n1] = _dot(h_s[:, cl], dout_v[:, n0:n1], TN).astype(bf16)

    def phase3(t, last):
        rows = tile_rows(t)
        xn = xn_s[rows, :]
        phis = [phik_s[g * 128:(g + 1) * 128, rows] for g in range(NG)]

        def sm_bwd(b):
            for g in (2 * b, 2 * b + 1):
                dphi = _dot(dkv4T_s[:, g * 128:g * 128 + 80], vT_s[g * 80:(g + 1) * 80, rows]).reshape(16, 8, T)
                phif = phis[g].astype(f32).reshape(16, 8, T)
                dp = _dual_softmax_bwd(phif[0:8], phif[8:16], dphi[0:8], dphi[8:16])
                dp_s[g * 64:(g + 1) * 64, :] = dp.reshape(64, T).astype(bf16)

        sm_bwd(0)
        for g in range(NG):
            dp_s[512 + g * 64:512 + (g + 1) * 64, :] = _dot(dkv4_s[0:64, gl(g)], phis[g]).astype(bf16)
        sm_bwd(1)
        wgrad_d(t, 0, 256)
        sm_bwd(2)
        wgrad_d(t, 256, 384)
        sm_bwd(3)
        wgrad_d(t, 384, 512)

        def ln_part(r, n):
            LB = T // n
            rw = pl.ds(mo(t * T + r * LB, LB), LB)
            dxn = dxn_s[rw, :] + _dot(dp_s[:, r * LB:(r + 1) * LB], wT_s[512:1536, :], TN)
            xnf = xn_s[rw, :].astype(f32)
            m1 = jnp.mean(dxn, axis=-1, keepdims=True)
            m2 = jnp.mean(dxn * xnf, axis=-1, keepdims=True)
            dx = rstd_s[rw, :] * (dxn - m1 - xnf * m2) + dout_v[rw, :].astype(f32)
            dx_v[rw, :] = dx.astype(bf16)

        ln_part(0, 2)
        gT_s[512:1024, :] += _dot(dp_s[0:512, :], xn)
        ln_part(1, 2)
        gT_s[1024:1536, :] += _dot(dp_s[512:1024, :], xn)
        ob = o_b(t)
        if last:
            unfold(1)
            unfold(2)
            wgrad_gu(t, 0, SPLIT)
            o_dx(t).start()
            ob[2].start()
            o_wkv.start()
            o_wphi.start()
            wgrad_gu(t, SPLIT, D)
            ob[0].start()
            ob[1].start()
        else:
            wgrad_gu(t)
            o_dx(t).start()
            for cpy in ob:
                cpy.start()

    def p3_body(t, carry):
        phase3(t, False)
        return carry

    jax.lax.fori_loop(0, NTILE - 1, p3_body, 0)
    phase3(NTILE - 1, True)

    o_out.wait()
    for cpy in o_a:
        cpy.wait()
    o_wq.wait()
    o_wo.wait()
    for t in range(NTILE):
        o_dx(t).wait()
    o_wkv.wait()
    o_wphi.wait()
    for t in range(NTILE):
        for cpy in o_b(t):
            cpy.wait()


@jax.jit
def pallas_parallel_sum__linear_kernel_hedgehog__glu_gated_bilinear__prompt_kernel(A_x, A_wqkv, A_w_phi, A_wo, B_x, B_w_gate, B_w_up, B_w_down, grad_out):
    x = A_x.reshape(S, D)
    dout = grad_out.reshape(S, D)
    wphi = jnp.transpose(A_w_phi, (1, 2, 0))
    sds = jax.ShapeDtypeStruct
    io_shapes = ((S, D), (S, D), (D, 3 * D), (DH, DH, H), (D, D), (D, F), (D, F), (F, D))
    any_spec = pl.BlockSpec(memory_space=pl.ANY)

    def packed(r, c):
        return pltpu.VMEM((r // 2, c), u32)

    io_scratch = [pltpu.VMEM(s, bf16) if len(s) == 3 else packed(*s) for s in io_shapes]
    dma = pltpu.SemaphoreType.DMA
    outs = pl.pallas_call(
        kernel,
        out_shape=tuple(sds(s, bf16) for s in io_shapes),
        in_specs=[any_spec] * 8,
        out_specs=tuple([any_spec] * 8),
        scratch_shapes=io_scratch + io_scratch + [
            packed(3 * D, D),
            packed(D, D),
            packed(128, 512),
            packed(S, D),
            packed(D, S),
            packed(NG * 128, S),
            packed(NG * 80, S),
            packed(80, NG * 128),
            packed(128, NG * 128),
            packed(80, NG * 128),
            packed(128, NG * 128),
            packed(S, FB),
            packed(S, FB),
            packed(S, FB),
            packed(2 * D, T),
            pltpu.VMEM((S, 1), f32),
            pltpu.VMEM((80, NG * 128), f32),
            pltpu.VMEM((80, NG * 128), f32),
            pltpu.VMEM((3 * D, D), f32),
            pltpu.VMEM((D, D), f32),
            pltpu.VMEM((D, FA), f32),
            pltpu.VMEM((D, FA), f32),
            pltpu.VMEM((FA, D), f32),
            pltpu.VMEM((S, D), f32),
            pltpu.VMEM((S, D), f32),
            pltpu.VMEM((128, 512), f32),
            dma((13,)),
        ],
        compiler_params=pltpu.CompilerParams(vmem_limit_bytes=110 * 1024 * 1024),
    )(x, A_wqkv, wphi, A_wo, B_w_gate, B_w_up, B_w_down, dout)
    out, dx, dwqkv, dwphi, dwo, dwg, dwu, dwd = outs
    return (out.reshape(1, S, D), dx.reshape(1, S, D), dwqkv, jnp.transpose(dwphi, (2, 0, 1)), dwo, dwg, dwu, dwd)
```

```python
import jax
import jax.numpy as jnp
import jax.experimental.pallas as pl
import jax.experimental.pallas.tpu as pltpu

S, D, H, DH, F = 2048, 512, 32, 16, 1792
NG = 8
NBLK = 4
T = 256
NTILE = S // T
FC = 256
FA = 768
FA1 = 512
FB = F - FA
SPLIT = 128

f32 = jnp.float32
bf16 = jnp.bfloat16
u32 = jnp.uint32
NN = (((1,), (0,)), ((), ()))
NT = (((1,), (1,)), ((), ()))
TN = (((0,), (0,)), ((), ()))


def _dot(a, b, dn=NN):
    return jax.lax.dot_general(a, b, dn, preferred_element_type=f32)


def _head_reduce(x3, red, comb):
    r = red(x3, axis=0)
    return comb(r, pltpu.roll(r, 4, 0))


def _hsum(x3):
    return _head_reduce(x3, jnp.sum, jnp.add)


def _dual_softmax(p):
    p3 = p.reshape(8, 8, p.shape[-1])
    mx = _head_reduce(p3, jnp.max, jnp.maximum)
    mn = _head_reduce(p3, jnp.min, jnp.minimum)
    ea = jnp.exp(p3 - mx[None])
    eb = jnp.exp(mn[None] - p3)
    a = ea * (1.0 / _hsum(ea))[None]
    b = eb * (1.0 / _hsum(eb))[None]
    return a, b


def _dual_softmax_bwd(a, b, da, db):
    ta = a * da
    tb = b * db
    return (ta - a * _hsum(ta)[None]) - (tb - b * _hsum(tb)[None])


def _phi(a, b):
    return jnp.concatenate([a.reshape(64, T), b.reshape(64, T)], axis=0).astype(bf16)


def _iota(shape, dim):
    return jax.lax.broadcasted_iota(jnp.int32, shape, dim)


def kernel(x_hbm, wqkv_hbm, wphi_hbm, wo_hbm, wg_hbm, wu_hbm, wd_hbm, dout_hbm,
           out_hbm, dx_hbm, dwqkv_hbm, dwphi_hbm, dwo_hbm, dwg_hbm, dwu_hbm, dwd_hbm,
           x_v, dout_v, wqkv_v, wphi_v, wo_v, wg_v, wu_v, wd_v,
           out_v, dx_v, dwqkv_v, dwphi_v, dwo_v, dwg_v, dwu_v, dwd_v,
           wT_s, wop_s, pmT_s, xn_s, xnT_s, phik_s, vT_s, kvz_s, kv4_s, dkv4_s, dkv4T_s, h_s, dg_s, du_s, dp_s,
           rstd_s, kvT_s, dkvT_s, gT_s, dwo_s, dwg_s, dwu_s, dwd_s, out_s, dxn_s, aphi_s,
           sem):
    (x_v, dout_v, wqkv_v, wo_v, wg_v, wu_v, wd_v, out_v, dx_v, dwqkv_v, dwo_v, dwg_v, dwu_v, dwd_v,
     wT_s, wop_s, pmT_s, xn_s, xnT_s, phik_s, vT_s, kvz_s, kv4_s, dkv4_s, dkv4T_s, h_s, dg_s, du_s, dp_s) = [
         r.bitcast(bf16) for r in (
             x_v, dout_v, wqkv_v, wo_v, wg_v, wu_v, wd_v, out_v, dx_v, dwqkv_v, dwo_v, dwg_v, dwu_v, dwd_v,
             wT_s, wop_s, pmT_s, xn_s, xnT_s, phik_s, vT_s, kvz_s, kv4_s, dkv4_s, dkv4T_s, h_s, dg_s, du_s, dp_s)]
    ALL = slice(None)

    def cp(src, dst, sem, *idx):
        if idx:
            src, dst = src.at[idx], dst.at[idx]
        return pltpu.make_async_copy(src, dst, sem)

    def mo(v, m):
        return v if isinstance(v, int) else pl.multiple_of(v, m)

    def tile_rows(t):
        return pl.ds(mo(t * T, T), T)

    def gl(g):
        return slice(g * 128, (g + 1) * 128)

    c_wphi = cp(wphi_hbm, wphi_v, sem.at[6])
    c_wk = cp(wqkv_hbm, wqkv_v, sem.at[8], ALL, slice(512, 1024))
    c_wv = cp(wqkv_hbm, wqkv_v, sem.at[9], ALL, slice(1024, 1536))
    c_wq = cp(wqkv_hbm, wqkv_v, sem.at[11], ALL, slice(0, 512))
    c_wo = cp(wo_hbm, wo_v, sem.at[11])
    c_wgA = cp(wg_hbm, wg_v, sem.at[10], ALL, slice(0, FA1))
    c_wuA = cp(wu_hbm, wu_v, sem.at[10], ALL, slice(0, FA1))
    c_wdA = cp(wd_hbm, wd_v, sem.at[10], slice(0, FA1), ALL)
    c_wgB = cp(wg_hbm, wg_v, sem.at[11], ALL, slice(FA1, F))
    c_wuB = cp(wu_hbm, wu_v, sem.at[11], ALL, slice(FA1, F))
    c_wdB = cp(wd_hbm, wd_v, sem.at[11], slice(FA1, F), ALL)
    sem_o = sem.at[12]

    def c_x(t):
        s = {0: 7, 1: 9}.get(t, t - 2) if isinstance(t, int) else t - 2
        return cp(x_hbm, x_v, sem.at[s], tile_rows(t), ALL)

    def c_do(t):
        s = (t if t < NTILE - 2 else 11) if isinstance(t, int) else t
        return cp(dout_hbm, dout_v, sem.at[s], tile_rows(t), ALL)

    c_wphi.start()
    c_x(0).start()
    c_wk.start()

    o_out = cp(out_v, out_hbm, sem_o)
    o_a = (cp(dwg_v, dwg_hbm, sem_o, ALL, slice(0, FA)),
           cp(dwu_v, dwu_hbm, sem_o, ALL, slice(0, FA)),
           cp(dwd_v, dwd_hbm, sem_o, slice(0, FA), ALL))

    def o_dx(t):
        return cp(dx_v, dx_hbm, sem_o, tile_rows(t), ALL)

    def o_b(t):
        cb = pl.ds(mo(FA + t * 128, 128), 128)
        return (cp(dwg_v, dwg_hbm, sem_o, ALL, cb),
                cp(dwu_v, dwu_hbm, sem_o, ALL, cb),
                cp(dwd_v, dwd_hbm, sem_o, cb, ALL))

    o_wq = cp(dwqkv_v, dwqkv_hbm, sem_o, ALL, slice(0, 512))
    o_wkv = cp(dwqkv_v, dwqkv_hbm, sem_o, ALL, slice(512, 1536))
    o_wo = cp(dwo_v, dwo_hbm, sem_o)
    o_wphi = cp(dwphi_v, dwphi_hbm, sem_o)

    RA = D // NTILE
    RD = FA1 // NTILE

    def row_head(r):
        return (r // 64) * 4 + r % 4

    def row_feat(r):
        return ((r % 64) // 8) * 2 + (r % 8) // 4

    r_i = _iota((128, 128), 0)
    c_i = _iota((128, 128), 1)
    permT = jnp.where((row_head(r_i) == c_i // 16) & (row_feat(r_i) == c_i % 16), 1.0, 0.0).astype(bf16)
    hsel = jnp.where(_iota((32, 512), 0) == (_iota((32, 512), 1) // 16), 1.0, 0.0).astype(bf16)
    dmask = (_iota((256, 512), 0) // 16) == (_iota((256, 512), 1) % 16)
    rsel = jnp.where(row_feat(_iota((128, 256), 0)) == (_iota((128, 256), 1) % 16), 1.0, 0.0).astype(bf16)
    hm4 = row_head(_iota((128, 512), 0)) == ((_iota((128, 512), 1) // 16) % 8)
    ones16 = jnp.ones((16, T), f32)
    zeros8 = jnp.zeros((8, T), f32)
    rr = _iota((80, NG * 128), 0)
    same_head = (rr % 4) == (_iota((80, NG * 128), 1) % 4)

    def fold(part):
        for b in range(NBLK):
            m = pmT_s[:, b * 128:(b + 1) * 128] if part < 2 else permT
            cs = slice(part * 512 + b * 128, part * 512 + (b + 1) * 128)
            wT_s[cs, :] = _dot(m, wqkv_v[:, cs], NT).astype(bf16)

    def w_g(c):
        return wg_v[:, c * FC:(c + 1) * FC]

    def w_u(c):
        return wu_v[:, c * FC:(c + 1) * FC]

    def w_d(c):
        return wd_v[c * FC:(c + 1) * FC, :]

    def ffn_dh(c, dout):
        return _dot(dout, w_d(c), NT)

    def ffn_gu(c, xn):
        return _dot(xn, w_g(c)), _dot(xn, w_u(c))

    def ffn_elem(g_, u_, dh):
        return (g_ * u_).astype(bf16), (dh * u_).astype(bf16), (dh * g_).astype(bf16)

    def ffn_mm(c, h, dg, du):
        o_c = _dot(h, w_d(c))
        d_c = _dot(dg, w_g(c), NT) + _dot(du, w_u(c), NT)
        return o_c, d_c

    def layernorm(t):
        LB = 32
        for r in range(T // LB):
            rows = pl.ds(mo(t * T + r * LB, LB), LB)
            x = x_v[rows, :].astype(f32)
            mu = jnp.mean(x, axis=-1, keepdims=True)
            xc = x - mu
            var = jnp.mean(xc * xc, axis=-1, keepdims=True)
            rstd = jax.lax.rsqrt(var + 1e-5)
            xn_s[rows, :] = (xc * rstd).astype(bf16)
            rstd_s[rows, :] = rstd
        rows = tile_rows(t)
        xn = xn_s[rows, :]
        xnT_s[:, rows] = xn.T
        return xn

    def k_phi(t, xn, b):
        pk = _dot(wT_s[512 + b * 128:512 + (b + 1) * 128, :], xn, NT)
        res = []
        for i in range(2):
            g = 2 * b + i
            phi = _phi(*_dual_softmax(pk[i * 64:(i + 1) * 64]))
            phik_s[g * 128:(g + 1) * 128, tile_rows(t)] = phi
            res.append(phi)
        return res

    def k_acc(t, xn, phis, first=False):
        pv = _dot(wT_s[1024:1536, :], xn, NT)
        for g in range(NG):
            v1 = jnp.concatenate([pv[g * 64:(g + 1) * 64], ones16], axis=0).astype(bf16)
            vT_s[g * 80:(g + 1) * 80, tile_rows(t)] = v1
            r = _dot(v1, phis[g], NT)
            if first:
                kvT_s[:, gl(g)] = r
            else:
                kvT_s[:, gl(g)] += r

    def phase1(t, nxt, extra=None):
        rows = tile_rows(t)
        if nxt is not None:
            xn1 = layernorm(nxt)
        dout = dout_v[rows, :]
        xn = xn_s[rows, :]
        xnT = xnT_s[:, rows]
        nchunk = FA1 // FC
        phis = []

        def kphi(b):
            if nxt is not None:
                phis.extend(k_phi(nxt, xn1, b))

        st = (ffn_dh(0, dout),) + ffn_gu(0, xn)
        if extra is not None:
            extra[0]()
        kphi(0)
        o_acc = x_v[rows, :].astype(f32)
        d_acc = None
        for c in range(nchunk):
            cs = slice(c * FC, (c + 1) * FC)
            dh, g_, u_ = st
            if c + 1 < nchunk:
                dh1 = ffn_dh(c + 1, dout)
            h, dg, du = ffn_elem(g_, u_, dh)
            if c + 1 < nchunk:
                st = (dh1,) + ffn_gu(c + 1, xn)
            if extra is not None and c == 0:
                extra[1]()
            if c == 0:
                kphi(1)
            dwg_s[:, cs] += _dot(xnT, dg)
            if c == 0:
                kphi(2)
            dwu_s[:, cs] += _dot(xnT, du)
            if c == 0:
                kphi(3)
            dwd_s[cs, :] += _dot(h, dout, TN)
            if c == 1 and nxt is not None:
                k_acc(nxt, xn1, phis)
            o_c, d_c = ffn_mm(c, h, dg, du)
            o_acc = o_acc + o_c
            d_acc = d_c if d_acc is None else d_acc + d_c
        out_s[rows, :] = o_acc
        dxn_s[rows, :] = d_acc

    dwg_s[...] = jnp.zeros_like(dwg_s)
    dwu_s[...] = jnp.zeros_like(dwu_s)
    dwd_s[...] = jnp.zeros_like(dwd_s)
    c_wphi.wait()
    w3 = wphi_v[...].reshape(256, 32)
    ym = jnp.where(dmask, _dot(w3, hsel), 0.0).astype(bf16)
    pmT_s[...] = jnp.where(hm4, _dot(rsel, ym), 0.0).astype(bf16)
    c_wv.start()
    c_x(1).start()
    c_x(0).wait()
    xn0 = layernorm(0)
    c_wk.wait()
    c_wdA.start()
    c_wgA.start()
    fold(1)
    for b in range(NBLK):
        k_phi(0, xn0, b)
    c_wv.wait()
    c_x(1).wait()
    c_wuA.start()
    c_do(0).start()
    c_x(2).start()
    xn1 = layernorm(1)
    fold(2)
    k_acc(0, xn_s[0:T, :], [phik_s[g * 128:(g + 1) * 128, 0:T] for g in range(NG)], first=True)
    k_acc(1, xn1, sum([k_phi(1, xn1, b) for b in range(NBLK)], []))
    c_wdA.wait()
    c_wgA.wait()
    c_wuA.wait()
    c_do(1).start()
    c_do(2).start()
    for t in range(3, NTILE):
        c_x(t).start()
        c_do(t).start()
    c_wq.start()
    c_wo.start()
    c_wgB.start()
    c_wuB.start()
    c_wdB.start()

    def p1_body(t, carry):
        c_do(t).wait()
        c_x(t + 2).wait()
        phase1(t, t + 2)
        return carry

    jax.lax.fori_loop(0, NTILE - 2, p1_body, 0)
    c_do(NTILE - 2).wait()
    c_do(NTILE - 1).wait()

    c_wq.wait()
    c_wo.wait()
    c_wgB.wait()
    c_wuB.wait()
    c_wdB.wait()

    def transposed(kv, dst):
        m = jnp.where(same_head & (rr < 68), kv, 0.0)
        m = jnp.concatenate([m, jnp.zeros((48, NG * 128), f32)], axis=0)
        for g in range(NG):
            mT = m[:, gl(g)].T
            halves = []
            for i in range(2):
                m3 = mT[i * 64:(i + 1) * 64].reshape(8, 8, 128)
                halves.append((m3 - (_hsum(m3) * (1.0 / DH))[None]).reshape(64, 128))
            dst[:, gl(g)] = jnp.concatenate(halves, axis=0).astype(bf16)

    def extra0():
        kv = kvT_s[...]
        kvz_s[...] = jnp.where(same_head & (rr < 72), kv, 0.0).astype(bf16)
        transposed(kv, kv4_s)

    def extra1():
        dkvT_s[...] = jnp.zeros_like(dkvT_s)
        gT_s[...] = jnp.zeros_like(gT_s)
        dwo_s[...] = jnp.zeros_like(dwo_s)
        fold(0)
        for b in range(NBLK):
            wop_s[b * 128:(b + 1) * 128, :] = _dot(permT, wo_v[b * 128:(b + 1) * 128, :]).astype(bf16)

    phase1(NTILE - 2, None, (extra0, extra1))
    phase1(NTILE - 1, None)

    c0 = FA // FC

    def phase2(t, carry):
        rows = tile_rows(t)
        xn = xn_s[rows, :]
        dout = dout_v[rows, :]
        acc = {}

        def ffn1(c):
            return (ffn_dh(c, dout),) + ffn_gu(c, xn)

        def elem(c, st):
            dh, g_, u_ = st
            h, dg, du = ffn_elem(g_, u_, dh)
            cs = slice((c - c0) * FC, (c - c0 + 1) * FC)
            h_s[rows, cs] = h
            dg_s[rows, cs] = dg
            du_s[rows, cs] = du
            return h, dg, du

        def mm(c, e):
            o_c, d_c = ffn_mm(c, *e)
            acc['o'] = o_c + acc['o']
            acc['d'] = d_c + acc['d']

        pq = _dot(wT_s[0:512, :], xn, NT)
        ab = [_dual_softmax(pq[g * 64:(g + 1) * 64]) for g in range(NG)]
        phis = [_phi(a, b) for a, b in ab]
        doT = _dot(wop_s[...], dout, NT)
        oTs, dn1s, dpqs = [], [], []

        def stage2(b):
            for g in (2 * b, 2 * b + 1):
                nd = _dot(kvz_s[:, gl(g)], phis[g])
                rden = 1.0 / (nd[64:72] + 1e-6)
                o3 = nd[0:64].reshape(8, 8, T) * rden[None]
                do3 = doT[g * 64:(g + 1) * 64].reshape(8, 8, T)
                dden = -_hsum(do3 * o3) * rden
                dn1s.append(jnp.concatenate([(do3 * rden[None]).reshape(64, T), dden, zeros8], axis=0).astype(bf16))
                oTs.append(o3.reshape(64, T))

        def stage3(b):
            for g in (2 * b, 2 * b + 1):
                dphi = _dot(kv4_s[:, g * 128:g * 128 + 80], dn1s[g]).reshape(16, 8, T)
                a, b_ = ab[g]
                dpqs.append(_dual_softmax_bwd(a, b_, dphi[0:8], dphi[8:16]).reshape(64, T))

        dh0 = ffn_dh(c0, dout)
        g0 = _dot(xn, w_g(c0))
        stage2(0)
        u0 = _dot(xn, w_u(c0))
        stage2(1)
        dh1 = ffn_dh(c0 + 1, dout)
        stage2(2)
        g1 = _dot(xn, w_g(c0 + 1))
        stage2(3)
        e0 = elem(c0, (dh0, g0, u0))
        u1 = _dot(xn, w_u(c0 + 1))
        st1 = (dh1, g1, u1)
        stage3(0)
        acc['o'] = _dot(e0[0], w_d(c0))
        stage3(1)
        acc['d'] = _dot(e0[1], w_g(c0), NT)
        stage3(2)
        acc['d'] = acc['d'] + _dot(e0[2], w_u(c0), NT)
        stage3(3)
        dpq = jnp.concatenate(dpqs, axis=0).astype(bf16)
        oT = jnp.concatenate(oTs, axis=0).astype(bf16)
        for g in range(NG):
            dkvT_s[:, gl(g)] += _dot(dn1s[g], phis[g], NT)
        e1 = elem(c0 + 1, st1)
        dwo_s[...] += _dot(oT, dout)
        acc['o'] = acc['o'] + _dot(oT, wop_s[...], TN)
        st2 = ffn1(c0 + 2)
        ra = pl.ds(pl.multiple_of(t * RA, RA), RA)
        rd = pl.ds(pl.multiple_of(t * RD, RD), RD)
        dwg_v[ra, 0:FA1] = dwg_s[ra, 0:FA1].astype(bf16)
        dwu_v[ra, 0:FA1] = dwu_s[ra, 0:FA1].astype(bf16)
        dwd_v[rd, :] = dwd_s[rd, :].astype(bf16)
        mm(c0 + 1, e1)
        e2 = elem(c0 + 2, st2)
        st3 = ffn1(c0 + 3)
        mm(c0 + 2, e2)
        e3 = elem(c0 + 3, st3)
        st4 = ffn1(c0 - 1)
        mm(c0 + 3, e3)
        e4 = ffn_elem(st4[1], st4[2], st4[0])
        gT_s[0:512, :] += _dot(dpq, xn)
        xnT = xnT_s[:, rows]
        dwg_s[:, FA1:FA] += _dot(xnT, e4[1])
        dwu_s[:, FA1:FA] += _dot(xnT, e4[2])
        dwd_s[FA1:FA, :] += _dot(e4[0], dout, TN)
        mm(c0 - 1, e4)
        out_v[rows, :] = (out_s[rows, :] + acc['o']).astype(bf16)
        dxn_s[rows, :] += acc['d'] + _dot(dpq, wT_s[0:512, :], TN)
        return carry

    jax.lax.fori_loop(0, NTILE, phase2, 0)
    o_out.start()

    dwg_v[:, FA1:FA] = dwg_s[:, FA1:FA].astype(bf16)
    dwu_v[:, FA1:FA] = dwu_s[:, FA1:FA].astype(bf16)
    dwd_v[FA1:FA, :] = dwd_s[FA1:FA, :].astype(bf16)
    dkv = dkvT_s[...]
    dkv4_s[...] = jnp.where(same_head, dkv, 0.0).astype(bf16)
    transposed(dkv, dkv4T_s)

    def unfold(part):
        for b in range(NBLK):
            m = pmT_s[:, b * 128:(b + 1) * 128] if part < 2 else permT
            cs = slice(part * 512 + b * 128, part * 512 + (b + 1) * 128)
            gblk = gT_s[cs, :].astype(bf16)
            dwqkv_v[:, cs] = _dot(gblk, m, TN).astype(bf16)
            if part == 0:
                aphi_s[:, b * 128:(b + 1) * 128] = _dot(gblk, wqkv_v[:, cs])
            elif part == 1:
                aphi_s[:, b * 128:(b + 1) * 128] += _dot(gblk, wqkv_v[:, cs])
        if part == 1:
            accm = jnp.where(hm4, aphi_s[...], 0.0).astype(bf16)
            z = jnp.where(dmask, _dot(rsel, accm, TN), 0.0).astype(bf16)
            dwphi_v[...] = _dot(z, hsel, NT).astype(bf16).reshape(16, 16, 32)

    unfold(0)
    for b in range(NBLK):
        dwo_v[b * 128:(b + 1) * 128, :] = _dot(permT, dwo_s[b * 128:(b + 1) * 128, :].astype(bf16), TN).astype(bf16)
    o_wq.start()
    o_wo.start()
    for cpy in o_a:
        cpy.start()

    def wgrad_gu(t, r0=0, r1=D):
        cl = pl.ds(mo(t * 128, 128), 128)
        cb = pl.ds(mo(FA + t * 128, 128), 128)
        dgu = _dot(xnT_s[r0:r1, :], jnp.concatenate([dg_s[:, cl], du_s[:, cl]], axis=1))
        dwg_v[r0:r1, cb] = dgu[:, 0:128].astype(bf16)
        dwu_v[r0:r1, cb] = dgu[:, 128:256].astype(bf16)

    def wgrad_d(t, n0, n1):
        cl = pl.ds(mo(t * 128, 128), 128)
        cb = pl.ds(mo(FA + t * 128, 128), 128)
        dwd_v[cb, n0:n1] = _dot(h_s[:, cl], dout_v[:, n0:n1], TN).astype(bf16)

    def phase3(t, last):
        rows = tile_rows(t)
        xn = xn_s[rows, :]
        phis = [phik_s[g * 128:(g + 1) * 128, rows] for g in range(NG)]

        def sm_bwd(b):
            for g in (2 * b, 2 * b + 1):
                dphi = _dot(dkv4T_s[:, g * 128:g * 128 + 80], vT_s[g * 80:(g + 1) * 80, rows]).reshape(16, 8, T)
                phif = phis[g].astype(f32).reshape(16, 8, T)
                dp = _dual_softmax_bwd(phif[0:8], phif[8:16], dphi[0:8], dphi[8:16])
                dp_s[g * 64:(g + 1) * 64, :] = dp.reshape(64, T).astype(bf16)

        sm_bwd(0)
        for g in range(NG):
            dp_s[512 + g * 64:512 + (g + 1) * 64, :] = _dot(dkv4_s[0:64, gl(g)], phis[g]).astype(bf16)
        sm_bwd(1)
        wgrad_d(t, 0, 256)
        sm_bwd(2)
        wgrad_d(t, 256, 384)
        sm_bwd(3)
        wgrad_d(t, 384, 512)

        def ln_part(r, n):
            LB = T // n
            rw = pl.ds(mo(t * T + r * LB, LB), LB)
            dxn = dxn_s[rw, :] + _dot(dp_s[:, r * LB:(r + 1) * LB], wT_s[512:1536, :], TN)
            xnf = xn_s[rw, :].astype(f32)
            m1 = jnp.mean(dxn, axis=-1, keepdims=True)
            m2 = jnp.mean(dxn * xnf, axis=-1, keepdims=True)
            dx = rstd_s[rw, :] * (dxn - m1 - xnf * m2) + dout_v[rw, :].astype(f32)
            dx_v[rw, :] = dx.astype(bf16)

        ln_part(0, 2)
        gT_s[512:1024, :] += _dot(dp_s[0:512, :], xn)
        ln_part(1, 2)
        gT_s[1024:1536, :] += _dot(dp_s[512:1024, :], xn)
        ob = o_b(t)
        if last:
            unfold(1)
            unfold(2)
            wgrad_gu(t, 0, SPLIT)
            o_dx(t).start()
            ob[2].start()
            o_wkv.start()
            o_wphi.start()
            wgrad_gu(t, SPLIT, D)
            ob[0].start()
            ob[1].start()
        else:
            wgrad_gu(t)
            o_dx(t).start()
            for cpy in ob:
                cpy.start()

    def p3_body(t, carry):
        phase3(t, False)
        return carry

    jax.lax.fori_loop(0, NTILE - 1, p3_body, 0)
    phase3(NTILE - 1, True)

    o_out.wait()
    for cpy in o_a:
        cpy.wait()
    o_wq.wait()
    o_wo.wait()
    for t in range(NTILE):
        o_dx(t).wait()
    o_wkv.wait()
    o_wphi.wait()
    for t in range(NTILE):
        for cpy in o_b(t):
            cpy.wait()


@jax.jit
def pallas_parallel_sum__linear_kernel_hedgehog__glu_gated_bilinear__prompt_kernel(
        A_x, A_wqkv, A_w_phi, A_wo, B_x, B_w_gate, B_w_up, B_w_down, grad_out):
    x = A_x.reshape(S, D)
    dout = grad_out.reshape(S, D)
    wphi = jnp.transpose(A_w_phi, (1, 2, 0))
    sds = jax.ShapeDtypeStruct
    io_shapes = ((S, D), (S, D), (D, 3 * D), (DH, DH, H), (D, D), (D, F), (D, F), (F, D))
    any_spec = pl.BlockSpec(memory_space=pl.ANY)

    def packed(r, c):
        return pltpu.VMEM((r // 2, c), u32)

    io_scratch = [pltpu.VMEM(s, bf16) if len(s) == 3 else packed(*s) for s in io_shapes]
    dma = pltpu.SemaphoreType.DMA
    outs = pl.pallas_call(
        kernel,
        out_shape=tuple(sds(s, bf16) for s in io_shapes),
        in_specs=[any_spec] * 8,
        out_specs=tuple([any_spec] * 8),
        scratch_shapes=io_scratch + io_scratch + [
            packed(3 * D, D),
            packed(D, D),
            packed(128, 512),
            packed(S, D),
            packed(D, S),
            packed(NG * 128, S),
            packed(NG * 80, S),
            packed(80, NG * 128),
            packed(128, NG * 128),
            packed(80, NG * 128),
            packed(128, NG * 128),
            packed(S, FB),
            packed(S, FB),
            packed(S, FB),
            packed(2 * D, T),
            pltpu.VMEM((S, 1), f32),
            pltpu.VMEM((80, NG * 128), f32),
            pltpu.VMEM((80, NG * 128), f32),
            pltpu.VMEM((3 * D, D), f32),
            pltpu.VMEM((D, D), f32),
            pltpu.VMEM((D, FA), f32),
            pltpu.VMEM((D, FA), f32),
            pltpu.VMEM((FA, D), f32),
            pltpu.VMEM((S, D), f32),
            pltpu.VMEM((S, D), f32),
            pltpu.VMEM((128, 512), f32),
            dma((13,)),
        ],
        compiler_params=pltpu.CompilerParams(vmem_limit_bytes=110 * 1024 * 1024),
    )(x, A_wqkv, wphi, A_wo, B_w_gate, B_w_up, B_w_down, dout)
    out, dx, dwqkv, dwphi, dwo, dwg, dwu, dwd = outs
    return (out.reshape(1, S, D), dx.reshape(1, S, D), dwqkv, jnp.transpose(dwphi, (2, 0, 1)), dwo, dwg, dwu, dwd)
```

```python
import jax
import jax.numpy as jnp
import jax.experimental.pallas as pl
import jax.experimental.pallas.tpu as pltpu

S, D, H, DH, F = 2048, 512, 32, 16, 1792
NG = 8
NBLK = 4
T = 256
NTILE = S // T
FC = 256
FA = 768
FA1 = 512
FB = F - FA
SPLIT = 128

f32 = jnp.float32
bf16 = jnp.bfloat16
u32 = jnp.uint32
NN = (((1,), (0,)), ((), ()))
NT = (((1,), (1,)), ((), ()))
TN = (((0,), (0,)), ((), ()))


def _dot(a, b, dn=NN):
    return jax.lax.dot_general(a, b, dn, preferred_element_type=f32)


def _head_reduce(x3, red, comb):
    r = red(x3, axis=0)
    return comb(r, pltpu.roll(r, 4, 0))


def _hsum(x3):
    return _head_reduce(x3, jnp.sum, jnp.add)


def _dual_softmax(p):
    p3 = p.reshape(8, 8, p.shape[-1])
    mx = _head_reduce(p3, jnp.max, jnp.maximum)
    mn = _head_reduce(p3, jnp.min, jnp.minimum)
    ea = jnp.exp(p3 - mx[None])
    eb = jnp.exp(mn[None] - p3)
    a = ea * (1.0 / _hsum(ea))[None]
    b = eb * (1.0 / _hsum(eb))[None]
    return a, b


def _dual_softmax_bwd(a, b, da, db):
    ta = a * da
    tb = b * db
    return (ta - a * _hsum(ta)[None]) - (tb - b * _hsum(tb)[None])


def _phi(a, b):
    return jnp.concatenate([a.reshape(64, T), b.reshape(64, T)], axis=0).astype(bf16)


_RP = (0, 2, 6, 5, 3, 4, 1)


def _blocks(x):
    r, c = x.shape[0] // 2, x.shape[1] // 2
    return x[:r, :c], x[:r, c:], x[r:, :c], x[r:, c:]


def _l7(x11, x12, x21, x22):
    return [v.astype(bf16) for v in (x11 + x22, x21 + x22, x11, x22, x11 + x12, x21 - x11, x12 - x22)]


def _r7(*blk):
    l = _l7(*blk)
    return [l[j] for j in _RP]


def _combine(m):
    m1, m2, m3, m4, m5, m6, m7 = m
    return m1 + m4 - m5 + m7, m3 + m5, m2 + m4, m1 - m2 + m3 + m6


def _cat22(c11, c12, c21, c22):
    return jnp.concatenate([jnp.concatenate([c11, c12], axis=1), jnp.concatenate([c21, c22], axis=1)], axis=0)


def _iota(shape, dim):
    return jax.lax.broadcasted_iota(jnp.int32, shape, dim)


def kernel(x_hbm, wqkv_hbm, wphi_hbm, wo_hbm, wg_hbm, wu_hbm, wd_hbm, dout_hbm,
           out_hbm, dx_hbm, dwqkv_hbm, dwphi_hbm, dwo_hbm, dwg_hbm, dwu_hbm, dwd_hbm,
           x_v, dout_v, wqkv_v, wphi_v, wo_v, wg_v, wu_v, wd_v,
           out_v, dx_v, dwqkv_v, dwphi_v, dwo_v, dwg_v, dwu_v, dwd_v,
           wT_s, wop_s, pmT_s, xn_s, phik_s, vT_s, kvz_s, kv4_s, dkv4_s, dkv4T_s, h_s, dg_s, dp_s,
           xl_s, xt_s, yl_s, yt_s, gu_s, ds_s,
           rstd_s, kvT_s, dkvT_s, gT_s, dwo_s, dgu_a, dwd_s, out_s, dxn_s, aphi_s, mg_s,
           sem):
    (x_v, dout_v, wqkv_v, wo_v, wg_v, wu_v, wd_v, out_v, dx_v, dwqkv_v, dwo_v, dwg_v, dwu_v, dwd_v,
     wT_s, wop_s, pmT_s, xn_s, phik_s, vT_s, kvz_s, kv4_s, dkv4_s, dkv4T_s, h_s, dg_s, dp_s,
           xl_s, xt_s, yl_s, yt_s, gu_s, ds_s) = [
         r.bitcast(bf16) for r in (
             x_v, dout_v, wqkv_v, wo_v, wg_v, wu_v, wd_v, out_v, dx_v, dwqkv_v, dwo_v, dwg_v, dwu_v, dwd_v,
             wT_s, wop_s, pmT_s, xn_s, phik_s, vT_s, kvz_s, kv4_s, dkv4_s, dkv4T_s, h_s, dg_s, dp_s,
           xl_s, xt_s, yl_s, yt_s, gu_s, ds_s)]
    ALL = slice(None)

    def cp(src, dst, sem, *idx):
        if idx:
            src, dst = src.at[idx], dst.at[idx]
        return pltpu.make_async_copy(src, dst, sem)

    def mo(v, m):
        return v if isinstance(v, int) else pl.multiple_of(v, m)

    def tile_rows(t):
        return pl.ds(mo(t * T, T), T)

    def gl(g):
        return slice(g * 128, (g + 1) * 128)

    c_wphi = cp(wphi_hbm, wphi_v, sem.at[6])
    c_wk = cp(wqkv_hbm, wqkv_v, sem.at[8], ALL, slice(512, 1024))
    c_wv = cp(wqkv_hbm, wqkv_v, sem.at[9], ALL, slice(1024, 1536))
    c_wq = cp(wqkv_hbm, wqkv_v, sem.at[11], ALL, slice(0, 512))
    c_wo = cp(wo_hbm, wo_v, sem.at[11])
    c_wgA = cp(wg_hbm, wg_v, sem.at[10], ALL, slice(0, FA1))
    c_wuA = cp(wu_hbm, wu_v, sem.at[10], ALL, slice(0, FA1))
    c_wdA = cp(wd_hbm, wd_v, sem.at[10], slice(0, FA1), ALL)

    def c_wB(c):
        cs = pl.ds(mo(c * FC, FC), FC)
        return (cp(wg_hbm, wg_v, sem.at[c - 2], ALL, cs), cp(wu_hbm, wu_v, sem.at[c - 2], ALL, cs),
                cp(wd_hbm, wd_v, sem.at[c - 2], cs, ALL))

    sem_o = sem.at[12]

    def c_x(t):
        s = {0: 7, 1: 9, 2: 10}.get(t, t - 3) if isinstance(t, int) else t - 3
        return cp(x_hbm, x_v, sem.at[s], tile_rows(t), ALL)

    def c_do(t):
        s = {0: 10, 6: 11, 7: 11}.get(t, t - 1) if isinstance(t, int) else t - 1
        return cp(dout_hbm, dout_v, sem.at[s], tile_rows(t), ALL)

    c_wphi.start()
    c_x(0).start()
    c_wk.start()

    o_out = cp(out_v, out_hbm, sem_o)
    o_a = (cp(dwg_v, dwg_hbm, sem_o, ALL, slice(0, FA)),
           cp(dwu_v, dwu_hbm, sem_o, ALL, slice(0, FA)),
           cp(dwd_v, dwd_hbm, sem_o, slice(0, FA), ALL))

    def o_dx(t):
        return cp(dx_v, dx_hbm, sem_o, tile_rows(t), ALL)

    def o_b(t):
        cb = pl.ds(mo(FA + (t // 2) * FC, FC), FC)
        res = []
        for half in range(2):
            rs = pl.ds(mo(half * 256 + (t % 2) * 128, 128), 128)
            res.append(cp(dwd_v, dwd_hbm, sem_o, cb, rs))
        for half in range(2):
            rs = pl.ds(mo(half * 256 + (t % 2) * 128, 128), 128)
            res.append(cp(dwg_v, dwg_hbm, sem_o, rs, cb))
            res.append(cp(dwu_v, dwu_hbm, sem_o, rs, cb))
        return res

    o_wq = cp(dwqkv_v, dwqkv_hbm, sem_o, ALL, slice(0, 512))
    o_wkv = cp(dwqkv_v, dwqkv_hbm, sem_o, ALL, slice(512, 1536))
    o_wo = cp(dwo_v, dwo_hbm, sem_o)
    o_wphi = cp(dwphi_v, dwphi_hbm, sem_o)

    RA = D // NTILE
    RD = FA1 // NTILE

    def row_head(r):
        return (r // 64) * 4 + r % 4

    def row_feat(r):
        return ((r % 64) // 8) * 2 + (r % 8) // 4

    r_i = _iota((128, 128), 0)
    c_i = _iota((128, 128), 1)
    permT = jnp.where((row_head(r_i) == c_i // 16) & (row_feat(r_i) == c_i % 16), 1.0, 0.0).astype(bf16)
    hsel = jnp.where(_iota((32, 512), 0) == (_iota((32, 512), 1) // 16), 1.0, 0.0).astype(bf16)
    dmask = (_iota((256, 512), 0) // 16) == (_iota((256, 512), 1) % 16)
    rsel = jnp.where(row_feat(_iota((128, 256), 0)) == (_iota((128, 256), 1) % 16), 1.0, 0.0).astype(bf16)
    hm4 = row_head(_iota((128, 512), 0)) == ((_iota((128, 512), 1) // 16) % 8)
    ones16 = jnp.ones((16, T), f32)
    zeros8 = jnp.zeros((8, T), f32)
    rr = _iota((80, NG * 128), 0)
    same_head = (rr % 4) == (_iota((80, NG * 128), 1) % 4)

    def fold(part):
        for b in range(NBLK):
            m = pmT_s[:, b * 128:(b + 1) * 128] if part < 2 else permT
            cs = slice(part * 512 + b * 128, part * 512 + (b + 1) * 128)
            wT_s[cs, :] = _dot(m, wqkv_v[:, cs], NT).astype(bf16)

    def sl(c, i):
        return slice((c * 7 + i) * 128, (c * 7 + i + 1) * 128)

    def sums9(b11, b12, b21, b22):
        return [v.astype(bf16) for v in (b11 + b22, b12 - b22, b21 - b11, b11 + b12, b21 + b22,
                                         b21 - b22, b12 - b11, b11 + b21, b12 + b22)]

    def weight_sets(c, part=None):
        c1 = pl.ds(mo(c * FC, 128), 128)
        c2 = pl.ds(mo(c * FC + 128, 128), 128)
        for p in (range(4) if part is None else [part]):
            for q in range(2):
                r = p * 64 + q * 32
                for j, w_v in enumerate((wg_v, wu_v)):
                    blk = [w_v[r0:r0 + 32, cc_].astype(f32) for r0 in (r, 256 + r) for cc_ in (c1, c2)]
                    for k, v in enumerate(sums9(*blk)):
                        gu_s[pl.ds(mo((c * 9 + k) * 256 + r, 32), 32), j * 128:(j + 1) * 128] = v
            for q in range(2):
                r = p * 32 + q * 16
                blk = [wd_v[pl.ds(mo(c * FC + r0, 16), 16), cc_].astype(f32)
                       for r0 in (r, 128 + r) for cc_ in (slice(0, 256), slice(256, 512))]
                for k, v in enumerate(sums9(*blk)):
                    ds_s[pl.ds(mo((c * 9 + k) * 128 + r, 16), 16), :] = v

    _KN = (0, None, 1, 2, None, 3, 4)
    _KT = (0, None, 5, 6, None, 7, 8)

    def w_gu(c, i, tab):
        if tab[i] is not None:
            return gu_s[(c * 9 + tab[i]) * 256:(c * 9 + tab[i] + 1) * 256, :]
        hb = 0 if i == 1 else 1
        rs, cs = slice(hb * 256, (hb + 1) * 256), slice(c * FC + hb * 128, c * FC + (hb + 1) * 128)
        return jnp.concatenate([wg_v[rs, cs], wu_v[rs, cs]], axis=1)

    def w_dd(c, i, tab):
        if tab[i] is not None:
            return ds_s[(c * 9 + tab[i]) * 128:(c * 9 + tab[i] + 1) * 128, :]
        hb = 0 if i == 1 else 1
        return wd_v[c * FC + hb * 128:c * FC + (hb + 1) * 128, hb * 256:(hb + 1) * 256]

    def lrow(t, i):
        return pl.ds(mo((t * 7 + i) * 128, 128), 128)

    def hcol(t):
        return pl.ds(mo(t * 128, 128), 128)

    def act_sets(t, src_v, l_s, t_s):
        a11, a12, a21, a22 = _blocks(src_v[tile_rows(t), :].astype(f32))
        for i, v in enumerate(_l7(a11, a12, a21, a22)):
            l_s[lrow(t, i), :] = v
        for i, v in enumerate(_l7(a11, a21, a12, a22)):
            t_s[i * 256:(i + 1) * 256, hcol(t)] = v.T

    def ffn_dh(c, t):
        return _combine([_dot(yl_s[lrow(t, i), :], w_dd(c, i, _KT), NT) for i in range(7)])

    def ffn_gu(c, t, lo=0, hi=7):
        return [_dot(xl_s[lrow(t, i), :], w_gu(c, i, _KN)) for i in range(lo, hi)]

    def ffn_elem(dh, gu):
        gu = _combine(gu)
        g_ = [v[:, 0:128] for v in gu]
        u_ = [v[:, 128:256] for v in gu]
        return (_l7(*[a * b for a, b in zip(g_, u_)]),
                _l7(*[jnp.concatenate([d * b, d * a], axis=1) for d, a, b in zip(dh, g_, u_)]))

    def acc7(acc, key, prods):
        acc[key] = prods if key not in acc else [a + b for a, b in zip(acc[key], prods)]

    def mm_o(c, acc, h7):
        acc7(acc, 'o', [_dot(h7[i], w_dd(c, i, _KN)) for i in range(7)])

    def mm_d(c, acc, e7):
        acc7(acc, 'd', [_dot(e7[i], w_gu(c, i, _KT), NT) for i in range(7)])

    def ffn_mm(c, acc, e):
        mm_o(c, acc, e[0])
        mm_d(c, acc, e[1])

    def sl2(c, i):
        return slice((c * 7 + i) * 256, (c * 7 + i + 1) * 256)

    def wacc_gu(c, t, e7, lo=0, hi=7):
        for i in range(lo, hi):
            dgu_a[:, sl2(c, i)] += _dot(xt_s[i * 256:(i + 1) * 256, hcol(t)], e7[_RP[i]])

    def wacc(c, t, a_s, t_s, e7):
        for i in range(7):
            a_s[:, sl(c, i)] += _dot(t_s[i * 256:(i + 1) * 256, hcol(t)], e7[_RP[i]])

    def wconv(c, r0, r1):
        cs = slice(c * FC, (c + 1) * FC)
        c11, c12, c21, c22 = _combine([dgu_a[r0, sl2(c, i)] for i in range(7)])
        for j, o_v in enumerate((dwg_v, dwu_v)):
            js = slice(j * 128, (j + 1) * 128)
            o_v[r0, cs] = jnp.concatenate([c11[:, js], c12[:, js]], axis=1).astype(bf16)
            o_v[r1, cs] = jnp.concatenate([c21[:, js], c22[:, js]], axis=1).astype(bf16)

    def wconv_d(c):
        cs = slice(c * FC, (c + 1) * FC)
        full = _cat22(*_combine([dwd_s[:, sl(c, i)] for i in range(7)]))
        dwd_v[cs, :] = full.astype(bf16).T

    def layernorm(t):
        LB = 32
        for r in range(T // LB):
            rows = pl.ds(mo(t * T + r * LB, LB), LB)
            x = x_v[rows, :].astype(f32)
            mu = jnp.mean(x, axis=-1, keepdims=True)
            xc = x - mu
            var = jnp.mean(xc * xc, axis=-1, keepdims=True)
            rstd = jax.lax.rsqrt(var + 1e-5)
            xn_s[rows, :] = (xc * rstd).astype(bf16)
            rstd_s[rows, :] = rstd
        return xn_s[tile_rows(t), :]

    def k_phi(t, xn, b):
        pk = _dot(wT_s[512 + b * 128:512 + (b + 1) * 128, :], xn, NT)
        res = []
        for i in range(2):
            g = 2 * b + i
            phi = _phi(*_dual_softmax(pk[i * 64:(i + 1) * 64]))
            phik_s[g * 128:(g + 1) * 128, tile_rows(t)] = phi
            res.append(phi)
        return res

    def k_acc(t, xn, phis, first=False):
        pv = _dot(wT_s[1024:1536, :], xn, NT)
        for g in range(NG):
            v1 = jnp.concatenate([pv[g * 64:(g + 1) * 64], ones16], axis=0).astype(bf16)
            vT_s[g * 80:(g + 1) * 80, tile_rows(t)] = v1
            r = _dot(v1, phis[g], NT)
            if first:
                kvT_s[:, gl(g)] = r
            else:
                kvT_s[:, gl(g)] += r

    def phase1(t, nxt, extra=None):
        rows = tile_rows(t)
        if nxt is not None:
            xn1 = layernorm(nxt)
        phis = []
        acc = {}

        def kphi(b):
            if nxt is not None:
                phis.extend(k_phi(nxt, xn1, b))

        def ex(i):
            if extra is not None and i < len(extra):
                extra[i]()

        def ws(p):
            if nxt is not None:
                weight_sets(t + 2, p)

        st0 = (ffn_dh(0, t), ffn_gu(0, t))
        ex(0)
        kphi(0)
        dh1 = ffn_dh(1, t)
        e0 = ffn_elem(*st0)
        st1 = (dh1, ffn_gu(1, t))
        ws(0)
        ws(1)
        ex(1)
        kphi(1)
        wacc_gu(0, t, e0[1], 0, 4)
        kphi(2)
        wacc_gu(0, t, e0[1], 4, 7)
        kphi(3)
        wacc(0, t, dwd_s, yt_s, e0[0])
        e1 = ffn_elem(*st1)
        if nxt is not None:
            act_sets(nxt, xn_s, xl_s, xt_s)
        if not (isinstance(t, int) and t == NTILE - 1):
            act_sets(t + 1, dout_v, yl_s, yt_s)
        ffn_mm(0, acc, e0)
        if nxt is not None:
            k_acc(nxt, xn1, phis)
        ffn_mm(1, acc, e1)
        ws(2)
        ws(3)
        out_s[rows, :] = x_v[rows, :].astype(f32) + _cat22(*_combine(acc['o']))
        dxn_s[rows, :] = _cat22(*_combine(acc['d']))
        wacc_gu(1, t, e1[1])
        wacc(1, t, dwd_s, yt_s, e1[0])

    dwd_s[:, 0:14 * 128] = jnp.zeros((256, 14 * 128), f32)
    dgu_a[:, 0:7 * 256] = jnp.zeros((256, 7 * 256), f32)
    c_wphi.wait()
    w3 = wphi_v[...].reshape(256, 32)
    ym = jnp.where(dmask, _dot(w3, hsel), 0.0).astype(bf16)
    pmT_s[...] = jnp.where(hm4, _dot(rsel, ym), 0.0).astype(bf16)
    c_wv.start()
    c_x(1).start()
    c_x(0).wait()
    xn0 = layernorm(0)
    c_wk.wait()
    c_wdA.start()
    c_wgA.start()
    fold(1)
    act_sets(0, xn_s, xl_s, xt_s)
    for b in range(NBLK):
        k_phi(0, xn0, b)
    c_wv.wait()
    c_x(1).wait()
    c_wuA.start()
    c_do(0).start()
    c_x(2).start()
    xn1 = layernorm(1)
    fold(2)
    act_sets(1, xn_s, xl_s, xt_s)
    dgu_a[:, 7 * 256:14 * 256] = jnp.zeros((256, 7 * 256), f32)
    k_acc(0, xn_s[0:T, :], [phik_s[g * 128:(g + 1) * 128, 0:T] for g in range(NG)], first=True)
    k_acc(1, xn1, sum([k_phi(1, xn1, b) for b in range(NBLK)], []))
    c_wdA.wait()
    c_wgA.wait()
    c_wuA.wait()
    c_do(0).wait()
    c_x(2).wait()
    c_do(1).start()
    c_x(3).start()
    for cpy in c_wB(2):
        cpy.start()
    xn2 = layernorm(2)
    weight_sets(0)
    phis2 = sum([k_phi(2, xn2, b) for b in range(NBLK)], [])
    act_sets(0, dout_v, yl_s, yt_s)
    weight_sets(1)
    k_acc(2, xn2, phis2)
    act_sets(2, xn_s, xl_s, xt_s)
    for t in range(1, NTILE - 3):
        c_do(t + 1).start()
        c_x(t + 3).start()
        for cpy in c_wB(t + 2):
            cpy.start()
    c_do(NTILE - 2).start()
    c_do(NTILE - 1).start()
    c_wq.start()
    c_wo.start()

    def p1_body(t, carry):
        c_do(t + 1).wait()
        c_x(t + 3).wait()
        for cpy in c_wB(t + 2):
            cpy.wait()
        phase1(t, t + 3)
        return carry

    jax.lax.fori_loop(0, NTILE - 3, p1_body, 0)
    c_do(NTILE - 2).wait()
    c_do(NTILE - 1).wait()

    c_wq.wait()
    c_wo.wait()

    def transposed(kv, dst):
        m = jnp.where(same_head & (rr < 68), kv, 0.0)
        m = jnp.concatenate([m, jnp.zeros((48, NG * 128), f32)], axis=0)
        for g in range(NG):
            mT = m[:, gl(g)].T
            halves = []
            for i in range(2):
                m3 = mT[i * 64:(i + 1) * 64].reshape(8, 8, 128)
                halves.append((m3 - (_hsum(m3) * (1.0 / DH))[None]).reshape(64, 128))
            dst[:, gl(g)] = jnp.concatenate(halves, axis=0).astype(bf16)

    def extra0():
        kv = kvT_s[...]
        kvz_s[...] = jnp.where(same_head & (rr < 72), kv, 0.0).astype(bf16)
        transposed(kv, kv4_s)

    def extra1():
        dwd_s[:, 14 * 128:21 * 128] = jnp.zeros((256, 7 * 128), f32)
        dgu_a[:, 14 * 256:21 * 256] = jnp.zeros((256, 7 * 256), f32)
        dkvT_s[...] = jnp.zeros_like(dkvT_s)
        gT_s[...] = jnp.zeros_like(gT_s)
        dwo_s[...] = jnp.zeros_like(dwo_s)
        fold(0)
        for b in range(NBLK):
            wop_s[b * 128:(b + 1) * 128, :] = _dot(permT, wo_v[b * 128:(b + 1) * 128, :]).astype(bf16)

    phase1(NTILE - 3, None, (extra0, extra1))
    phase1(NTILE - 2, None)
    phase1(NTILE - 1, None)

    c0 = FA // FC

    def phase2(t, carry):
        rows = tile_rows(t)
        xn = xn_s[rows, :]
        dout = dout_v[rows, :]
        acc = {}

        def ffn1(c):
            return ffn_dh(c, t), ffn_gu(c, t)

        def elem(c, st):
            e = ffn_elem(*st)
            for i in range(7):
                h_s[hcol(t), sl(c - c0, i)] = e[0][_RP[i]]
                dg_s[hcol(t), sl2(c - c0, i)] = e[1][_RP[i]]
            return e

        def mm(c, e):
            ffn_mm(c, acc, e)

        pq = _dot(wT_s[0:512, :], xn, NT)
        ab = [_dual_softmax(pq[g * 64:(g + 1) * 64]) for g in range(NG)]
        phis = [_phi(a, b) for a, b in ab]
        doT = _dot(wop_s[...], dout, NT)
        oTs, dn1s, dpqs = [], [], []

        def stage2(b):
            for g in (2 * b, 2 * b + 1):
                nd = _dot(kvz_s[:, gl(g)], phis[g])
                rden = 1.0 / (nd[64:72] + 1e-6)
                o3 = nd[0:64].reshape(8, 8, T) * rden[None]
                do3 = doT[g * 64:(g + 1) * 64].reshape(8, 8, T)
                dden = -_hsum(do3 * o3) * rden
                dn1s.append(jnp.concatenate([(do3 * rden[None]).reshape(64, T), dden, zeros8], axis=0).astype(bf16))
                oTs.append(o3.reshape(64, T))

        def stage3(b):
            for g in (2 * b, 2 * b + 1):
                dphi = _dot(kv4_s[:, g * 128:g * 128 + 80], dn1s[g]).reshape(16, 8, T)
                a, b_ = ab[g]
                dpqs.append(_dual_softmax_bwd(a, b_, dphi[0:8], dphi[8:16]).reshape(64, T))

        dh0 = ffn_dh(c0, t)
        gu0 = ffn_gu(c0, t, 0, 4)
        stage2(0)
        gu0 += ffn_gu(c0, t, 4, 7)
        stage2(1)
        dh1 = ffn_dh(c0 + 1, t)
        stage2(2)
        gu1 = ffn_gu(c0 + 1, t, 0, 4)
        stage2(3)
        e0 = elem(c0, (dh0, gu0))
        gu1 += ffn_gu(c0 + 1, t, 4, 7)
        st1 = (dh1, gu1)
        stage3(0)
        mm_o(c0, acc, e0[0])
        stage3(1)
        stage3(2)
        mm_d(c0, acc, e0[1])
        stage3(3)
        dpq = jnp.concatenate(dpqs, axis=0).astype(bf16)
        oT = jnp.concatenate(oTs, axis=0).astype(bf16)
        for g in range(NG):
            dkvT_s[:, gl(g)] += _dot(dn1s[g], phis[g], NT)
        e1 = elem(c0 + 1, st1)
        dwo_s[...] += _dot(oT, dout)
        o_att = _dot(oT, wop_s[...], TN)
        st2 = ffn1(c0 + 2)
        ra = pl.ds(pl.multiple_of(t * 32, 32), 32)
        rb = pl.ds(pl.multiple_of(256 + t * 32, 32), 32)
        wconv(0, ra, rb)
        wconv(1, ra, rb)
        mm(c0 + 1, e1)
        e2 = elem(c0 + 2, st2)
        st3 = ffn1(c0 + 3)
        mm(c0 + 2, e2)
        e3 = elem(c0 + 3, st3)
        st4 = ffn1(c0 - 1)
        mm(c0 + 3, e3)
        e4 = ffn_elem(*st4)
        gT_s[0:512, :] += _dot(dpq, xn)
        d_att = _dot(dpq, wT_s[0:512, :], TN)
        mm(c0 - 1, e4)
        out_v[rows, :] = (out_s[rows, :] + o_att + _cat22(*_combine(acc['o']))).astype(bf16)
        dxn_s[rows, :] += d_att + _cat22(*_combine(acc['d']))
        wacc_gu(c0 - 1, t, e4[1])
        wacc(c0 - 1, t, dwd_s, yt_s, e4[0])
        return carry

    jax.lax.fori_loop(0, NTILE, phase2, 0)
    o_out.start()

    wconv(c0 - 1, pl.ds(0, 256), pl.ds(256, 256))
    for c in range(c0):
        wconv_d(c)
    dkv = dkvT_s[...]
    dkv4_s[...] = jnp.where(same_head, dkv, 0.0).astype(bf16)
    transposed(dkv, dkv4T_s)

    def unfold(part):
        for b in range(NBLK):
            m = pmT_s[:, b * 128:(b + 1) * 128] if part < 2 else permT
            cs = slice(part * 512 + b * 128, part * 512 + (b + 1) * 128)
            gblk = gT_s[cs, :].astype(bf16)
            dwqkv_v[:, cs] = _dot(gblk, m, TN).astype(bf16)
            if part == 0:
                aphi_s[:, b * 128:(b + 1) * 128] = _dot(gblk, wqkv_v[:, cs])
            elif part == 1:
                aphi_s[:, b * 128:(b + 1) * 128] += _dot(gblk, wqkv_v[:, cs])
        if part == 1:
            accm = jnp.where(hm4, aphi_s[...], 0.0).astype(bf16)
            z = jnp.where(dmask, _dot(rsel, accm, TN), 0.0).astype(bf16)
            dwphi_v[...] = _dot(z, hsel, NT).astype(bf16).reshape(16, 16, 32)

    unfold(0)
    for b in range(NBLK):
        dwo_v[b * 128:(b + 1) * 128, :] = _dot(permT, dwo_s[b * 128:(b + 1) * 128, :].astype(bf16), TN).astype(bf16)
    o_wq.start()
    o_wo.start()
    for cpy in o_a:
        cpy.start()

    def wsl(t, i):
        return pl.ds(mo(((t // 2) * 7 + i) * 128, 128), 128)

    def wrow(t, i):
        return pl.ds(mo(i * 256 + (t % 2) * 128, 128), 128)

    def gu_prod(t, i):
        return _dot(xt_s[wrow(t, i), :], dg_s[:, pl.ds(mo(((t // 2) * 7 + i) * 256, 256), 256)])

    def d_prod(t, i):
        return _dot(yt_s[wrow(t, i), :], h_s[:, wsl(t, i)])

    def gu_store(t, m):
        cb = pl.ds(mo(FA + (t // 2) * FC, FC), FC)
        c11, c12, c21, c22 = _combine(m)
        for half, (ca, cc_) in enumerate(((c11, c12), (c21, c22))):
            rs = pl.ds(mo(half * 256 + (t % 2) * 128, 128), 128)
            dwg_v[rs, cb] = jnp.concatenate([ca[:, 0:128], cc_[:, 0:128]], axis=1).astype(bf16)
            dwu_v[rs, cb] = jnp.concatenate([ca[:, 128:256], cc_[:, 128:256]], axis=1).astype(bf16)

    def d_store(t, m):
        cb = pl.ds(mo(FA + (t // 2) * FC, FC), FC)
        c11, c12, c21, c22 = _combine(m)
        for half, (ca, cc_) in enumerate(((c11, c12), (c21, c22))):
            rs = pl.ds(mo(half * 256 + (t % 2) * 128, 128), 128)
            dwd_v[cb, rs] = jnp.concatenate([ca, cc_], axis=1).astype(bf16).T

    def phase3(t, last):
        rows = tile_rows(t)
        xn = xn_s[rows, :]
        phis = [phik_s[g * 128:(g + 1) * 128, rows] for g in range(NG)]

        def sm_bwd(b):
            for g in (2 * b, 2 * b + 1):
                dphi = _dot(dkv4T_s[:, g * 128:g * 128 + 80], vT_s[g * 80:(g + 1) * 80, rows]).reshape(16, 8, T)
                phif = phis[g].astype(f32).reshape(16, 8, T)
                dp = _dual_softmax_bwd(phif[0:8], phif[8:16], dphi[0:8], dphi[8:16])
                dp_s[g * 64:(g + 1) * 64, :] = dp.reshape(64, T).astype(bf16)

        sm_bwd(0)
        for g in range(NG):
            dp_s[512 + g * 64:512 + (g + 1) * 64, :] = _dot(dkv4_s[0:64, gl(g)], phis[g]).astype(bf16)
        sm_bwd(1)
        md = [d_prod(t, i) for i in range(3)]
        sm_bwd(2)
        md += [d_prod(t, i) for i in range(3, 5)]
        sm_bwd(3)
        md += [d_prod(t, i) for i in range(5, 7)]
        d_store(t, md)

        def ln_part(r, n):
            LB = T // n
            rw = pl.ds(mo(t * T + r * LB, LB), LB)
            dxn = dxn_s[rw, :] + _dot(dp_s[:, r * LB:(r + 1) * LB], wT_s[512:1536, :], TN)
            xnf = xn_s[rw, :].astype(f32)
            m1 = jnp.mean(dxn, axis=-1, keepdims=True)
            m2 = jnp.mean(dxn * xnf, axis=-1, keepdims=True)
            dx = rstd_s[rw, :] * (dxn - m1 - xnf * m2) + dout_v[rw, :].astype(f32)
            dx_v[rw, :] = dx.astype(bf16)

        ln_part(0, 2)
        gT_s[512:1024, :] += _dot(dp_s[0:512, :], xn)
        ln_part(1, 2)
        gT_s[1024:1536, :] += _dot(dp_s[512:1024, :], xn)
        ob = o_b(t)
        if last:
            unfold(1)
            unfold(2)
            mg = [gu_prod(t, i) for i in range(2)]
            for i in range(2):
                mg_s[i] = mg[i]
            o_dx(t).start()
            ob[0].start()
            ob[1].start()
            o_wkv.start()
            o_wphi.start()
            gu_store(t, [mg_s[0], mg_s[1]] + [gu_prod(t, i) for i in range(2, 7)])
            for cpy in ob[2:]:
                cpy.start()
        else:
            gu_store(t, [gu_prod(t, i) for i in range(7)])
            o_dx(t).start()
            for cpy in ob:
                cpy.start()

    def p3_body(t, carry):
        phase3(t, False)
        return carry

    jax.lax.fori_loop(0, NTILE - 1, p3_body, 0)
    phase3(NTILE - 1, True)

    o_out.wait()
    for cpy in o_a:
        cpy.wait()
    o_wq.wait()
    o_wo.wait()
    for t in range(NTILE):
        o_dx(t).wait()
    o_wkv.wait()
    o_wphi.wait()
    for t in range(NTILE):
        for cpy in o_b(t):
            cpy.wait()


@jax.jit
def pallas_parallel_sum__linear_kernel_hedgehog__glu_gated_bilinear__prompt_kernel(
        A_x, A_wqkv, A_w_phi, A_wo, B_x, B_w_gate, B_w_up, B_w_down, grad_out):
    x = A_x.reshape(S, D)
    dout = grad_out.reshape(S, D)
    wphi = jnp.transpose(A_w_phi, (1, 2, 0))
    sds = jax.ShapeDtypeStruct
    io_shapes = ((S, D), (S, D), (D, 3 * D), (DH, DH, H), (D, D), (D, F), (D, F), (F, D))
    any_spec = pl.BlockSpec(memory_space=pl.ANY)

    def packed(r, c):
        return pltpu.VMEM((r // 2, c), u32)

    io_scratch = [pltpu.VMEM(s, bf16) if len(s) == 3 else packed(*s) for s in io_shapes]
    dma = pltpu.SemaphoreType.DMA
    outs = pl.pallas_call(
        kernel,
        out_shape=tuple(sds(s, bf16) for s in io_shapes),
        in_specs=[any_spec] * 8,
        out_specs=tuple([any_spec] * 8),
        scratch_shapes=io_scratch + io_scratch + [
            packed(3 * D, D),
            packed(D, D),
            packed(128, 512),
            packed(S, D),
            packed(NG * 128, S),
            packed(NG * 80, S),
            packed(80, NG * 128),
            packed(128, NG * 128),
            packed(80, NG * 128),
            packed(128, NG * 128),
            packed(S // 2, 4 * 896),
            packed(S // 2, 8 * 896),
            packed(2 * D, T),
            packed(NTILE * 896, 256),
            packed(7 * 256, S // 2),
            packed(NTILE * 896, 256),
            packed(7 * 256, S // 2),
            packed(63 * 256, 256),
            packed(63 * 128, 256),
            pltpu.VMEM((S, 1), f32),
            pltpu.VMEM((80, NG * 128), f32),
            pltpu.VMEM((80, NG * 128), f32),
            pltpu.VMEM((3 * D, D), f32),
            pltpu.VMEM((D, D), f32),
            pltpu.VMEM((256, 6 * 896), f32),
            pltpu.VMEM((256, 3 * 896), f32),
            pltpu.VMEM((S, D), f32),
            pltpu.VMEM((S, D), f32),
            pltpu.VMEM((128, 512), f32),
            pltpu.VMEM((2, 128, 256), f32),
            dma((13,)),
        ],
        compiler_params=pltpu.CompilerParams(vmem_limit_bytes=120 * 1024 * 1024),
    )(x, A_wqkv, wphi, A_wo, B_w_gate, B_w_up, B_w_down, dout)
    out, dx, dwqkv, dwphi, dwo, dwg, dwu, dwd = outs
    return (out.reshape(1, S, D), dx.reshape(1, S, D), dwqkv, jnp.transpose(dwphi, (2, 0, 1)), dwo, dwg, dwu, dwd)
```

```python
import jax
import jax.numpy as jnp
import jax.experimental.pallas as pl
import jax.experimental.pallas.tpu as pltpu

S, D, H, DH, F = 2048, 512, 32, 16, 1792
NG = 8
NBLK = 4
T = 256
NTILE = S // T
FC = 256
FA = 768
FA1 = 512
FB = F - FA
SPLIT = 128

f32 = jnp.float32
bf16 = jnp.bfloat16
u32 = jnp.uint32
NN = (((1,), (0,)), ((), ()))
NT = (((1,), (1,)), ((), ()))
TN = (((0,), (0,)), ((), ()))


def _dot(a, b, dn=NN):
    return jax.lax.dot_general(a, b, dn, preferred_element_type=f32)


def _head_reduce(x3, red, comb):
    r = red(x3, axis=0)
    return comb(r, pltpu.roll(r, 4, 0))


def _hsum(x3):
    return _head_reduce(x3, jnp.sum, jnp.add)


def _dual_softmax(p):
    p3 = p.reshape(8, 8, p.shape[-1])
    mx = _head_reduce(p3, jnp.max, jnp.maximum)
    mn = _head_reduce(p3, jnp.min, jnp.minimum)
    ea = jnp.exp(p3 - mx[None])
    eb = jnp.exp(mn[None] - p3)
    a = ea * (1.0 / _hsum(ea))[None]
    b = eb * (1.0 / _hsum(eb))[None]
    return a, b


def _dual_softmax_bwd(a, b, da, db):
    ta = a * da
    tb = b * db
    return (ta - a * _hsum(ta)[None]) - (tb - b * _hsum(tb)[None])


def _phi(a, b):
    return jnp.concatenate([a.reshape(64, T), b.reshape(64, T)], axis=0).astype(bf16)


_RP = (0, 2, 6, 5, 3, 4, 1)


def _blocks(x):
    r, c = x.shape[0] // 2, x.shape[1] // 2
    return x[:r, :c], x[:r, c:], x[r:, :c], x[r:, c:]


def _l7(x11, x12, x21, x22):
    return [v.astype(bf16) for v in (x11 + x22, x21 + x22, x11, x22, x11 + x12, x21 - x11, x12 - x22)]


def _r7(*blk):
    l = _l7(*blk)
    return [l[j] for j in _RP]


def _combine(m):
    m1, m2, m3, m4, m5, m6, m7 = m
    return m1 + m4 - m5 + m7, m3 + m5, m2 + m4, m1 - m2 + m3 + m6


def _m7(x11, x12, x21, x22):
    return [v.astype(bf16) for v in (x11 - x22, x21 - x22, x11, x22, x11 - x12, x21 - x11, x22 - x12)]


def _combine_t(p):
    return p[0] + p[3] - p[4] - p[6], p[2] - p[4], p[1] + p[3], p[1] - p[0] + p[2] + p[5]


def _combine_w(q):
    return q[0] + q[3] + q[4] + q[6], q[4] - q[2], q[1] + q[3], q[1] - q[0] - q[2] - q[5]


_XI = (0, 2, 1, 4, 3, 5, 6)


def _combine_b(p):
    return p[0] - p[3] + p[4] - p[6], p[2] + p[4], p[1] - p[3], p[1] - p[0] + p[2] + p[5]


def _combine_tn(p):
    return p[0] - p[3] - p[4] + p[6], p[2] + p[4], p[1] + p[3], p[5] - p[0] - p[1] - p[2]


_TI = (0, 6, 2, 3, 5, 4, 1)


def _w5(w11, w12, w21, w22):
    return [v.astype(bf16) for v in (w11 - w22, w12 + w22, w21 + w11, w11 + w12, w21 + w22)]


def _cat22(c11, c12, c21, c22):
    return jnp.concatenate([jnp.concatenate([c11, c12], axis=1), jnp.concatenate([c21, c22], axis=1)], axis=0)


def _iota(shape, dim):
    return jax.lax.broadcasted_iota(jnp.int32, shape, dim)


def kernel(x_hbm, wqkv_hbm, wphi_hbm, wo_hbm, wg_hbm, wu_hbm, wd_hbm, dout_hbm,
           out_hbm, dx_hbm, dwqkv_hbm, dwphi_hbm, dwo_hbm, dwg_hbm, dwu_hbm, dwd_hbm,
           x_v, dout_v, wqkv_v, wphi_v, wo_v, wg_v, wu_v, wd_v,
           out_v, dx_v, dwqkv_v, dwphi_v, dwo_v, dwg_v, dwu_v, dwd_v,
           wT_s, wop_s, pmT_s, xn_s, phik_s, vT_s, kvz_s, kv4_s, dkv4_s, dkv4T_s, h_s, dg_s, dp_s,
           xl_s, xt_s, yl_s, yt_s, gu_s, ds_s, guA_s, dsA_s, tmpx_s, tmpy_s, wkvR_s, dps_s, sq_s, os_s, xnN_s, xlN_s,
           rstd_s, kvT_s, dkvT_s, gT_s, dwo_s, out_s, dxn_s, aphi_s, mg_s, gkv_a, gq_a,
           sem):
    (x_v, dout_v, wqkv_v, wo_v, wg_v, wu_v, wd_v, out_v, dx_v, dwqkv_v, dwo_v, dwg_v, dwu_v, dwd_v,
     wT_s, wop_s, pmT_s, xn_s, phik_s, vT_s, kvz_s, kv4_s, dkv4_s, dkv4T_s, h_s, dg_s, dp_s,
           xl_s, xt_s, yl_s, yt_s, gu_s, ds_s, guA_s, dsA_s, tmpx_s, tmpy_s, wkvR_s, dps_s, sq_s, os_s, xnN_s, xlN_s) = [
         r.bitcast(bf16) for r in (
             x_v, dout_v, wqkv_v, wo_v, wg_v, wu_v, wd_v, out_v, dx_v, dwqkv_v, dwo_v, dwg_v, dwu_v, dwd_v,
             wT_s, wop_s, pmT_s, xn_s, phik_s, vT_s, kvz_s, kv4_s, dkv4_s, dkv4T_s, h_s, dg_s, dp_s,
           xl_s, xt_s, yl_s, yt_s, gu_s, ds_s, guA_s, dsA_s, tmpx_s, tmpy_s, wkvR_s, dps_s, sq_s, os_s, xnN_s, xlN_s)]
    ALL = slice(None)

    def cp(src, dst, sem, *idx):
        if idx:
            src, dst = src.at[idx], dst.at[idx]
        return pltpu.make_async_copy(src, dst, sem)

    def mo(v, m):
        return v if isinstance(v, int) else pl.multiple_of(v, m)

    def tile_rows(t):
        return pl.ds(mo(t * T, T), T)

    def gl(g):
        return slice(g * 128, (g + 1) * 128)

    c_wphi = cp(wphi_hbm, wphi_v, sem.at[6])
    c_wk = cp(wqkv_hbm, wqkv_v, sem.at[8], ALL, slice(512, 1024))
    c_wv = cp(wqkv_hbm, wqkv_v, sem.at[9], ALL, slice(1024, 1536))
    c_wq = cp(wqkv_hbm, wqkv_v, sem.at[11], ALL, slice(0, 512))
    c_wo = cp(wo_hbm, wo_v, sem.at[11])
    c_wgA = cp(wg_hbm, wg_v, sem.at[10], ALL, slice(0, FA1))
    c_wuA = cp(wu_hbm, wu_v, sem.at[10], ALL, slice(0, FA1))
    c_wdA = cp(wd_hbm, wd_v, sem.at[10], slice(0, FA1), ALL)

    def c_wB(c):
        cs = pl.ds(mo(c * FC, FC), FC)
        return (cp(wg_hbm, wg_v, sem.at[c - 2], ALL, cs), cp(wu_hbm, wu_v, sem.at[c - 2], ALL, cs),
                cp(wd_hbm, wd_v, sem.at[c - 2], cs, ALL))

    sem_o = sem.at[12]

    def c_x(t):
        s = {0: 7, 1: 9, 2: 10}.get(t, t - 3) if isinstance(t, int) else t - 3
        return cp(x_hbm, x_v, sem.at[s], tile_rows(t), ALL)

    def c_do(t):
        s = {0: 10, 6: 11, 7: 11}.get(t, t - 1) if isinstance(t, int) else t - 1
        return cp(dout_hbm, dout_v, sem.at[s], tile_rows(t), ALL)

    c_wphi.start()
    c_x(0).start()
    c_wk.start()

    o_out = cp(out_v, out_hbm, sem_o)

    def o_dx(t):
        return cp(dx_v, dx_hbm, sem_o, tile_rows(t), ALL)

    def o_b(c):
        cb = pl.ds(mo(c * FC, FC), FC)
        if isinstance(c, int) and c == F // FC - 1:
            return (cp(dwd_v, dwd_hbm, sem_o, cb, ALL),)
        return (cp(dwd_v, dwd_hbm, sem_o, cb, ALL), cp(dwg_v, dwg_hbm, sem_o, ALL, cb), cp(dwu_v, dwu_hbm, sem_o, ALL, cb))

    def o_half(h):
        cb, rs = slice(F - FC, F), slice(h * 256, (h + 1) * 256)
        return cp(dwg_v, dwg_hbm, sem_o, rs, cb), cp(dwu_v, dwu_hbm, sem_o, rs, cb)

    o_wq = cp(dwqkv_v, dwqkv_hbm, sem_o, ALL, slice(0, 512))
    o_wkv = cp(dwqkv_v, dwqkv_hbm, sem_o, ALL, slice(512, 1536))
    o_wo = cp(dwo_v, dwo_hbm, sem_o)
    o_wphi = cp(dwphi_v, dwphi_hbm, sem_o)

    RA = D // NTILE
    RD = FA1 // NTILE

    def row_head(r):
        return (r // 64) * 4 + r % 4

    def row_feat(r):
        return ((r % 64) // 8) * 2 + (r % 8) // 4

    r_i = _iota((128, 128), 0)
    c_i = _iota((128, 128), 1)
    permT = jnp.where((row_head(r_i) == c_i // 16) & (row_feat(r_i) == c_i % 16), 1.0, 0.0).astype(bf16)
    hsel = jnp.where(_iota((32, 512), 0) == (_iota((32, 512), 1) // 16), 1.0, 0.0).astype(bf16)
    dmask = (_iota((256, 512), 0) // 16) == (_iota((256, 512), 1) % 16)
    rsel = jnp.where(row_feat(_iota((128, 256), 0)) == (_iota((128, 256), 1) % 16), 1.0, 0.0).astype(bf16)
    hm4 = row_head(_iota((128, 512), 0)) == ((_iota((128, 512), 1) // 16) % 8)
    ones16 = jnp.ones((16, T), f32)
    zeros8 = jnp.zeros((8, T), f32)
    rr = _iota((80, NG * 128), 0)
    same_head = (rr % 4) == (_iota((80, NG * 128), 1) % 4)

    def fold(part):
        for b in range(NBLK):
            m = pmT_s[:, b * 128:(b + 1) * 128] if part < 2 else permT
            cs = slice(part * 512 + b * 128, part * 512 + (b + 1) * 128)
            wT_s[cs, :] = _dot(m, wqkv_v[:, cs], NT).astype(bf16)

    def sl(c, i):
        return slice((c * 7 + i) * 128, (c * 7 + i + 1) * 128)

    def sums9(b11, b12, b21, b22):
        return [v.astype(bf16) for v in (b11 + b22, b12 - b22, b21 - b11, b11 + b12, b21 + b22)]

    def weight_sets(c, part=None):
        c1 = pl.ds(mo(c * FC, 128), 128)
        c2 = pl.ds(mo(c * FC + 128, 128), 128)
        gu_d, ds_d, cr = (guA_s, dsA_s, c) if isinstance(c, int) and c < 2 else (gu_s, ds_s, c - 2)
        for p in (range(4) if part is None else [part]):
            for q in range(2):
                r = p * 64 + q * 32
                for j, w_v in enumerate((wg_v, wu_v)):
                    blk = [w_v[r0:r0 + 32, cc_].astype(f32) for r0 in (r, 256 + r) for cc_ in (c1, c2)]
                    for k, v in enumerate(sums9(*blk)):
                        gu_d[pl.ds(mo((cr * 5 + k) * 256 + r, 32), 32), j * 128:(j + 1) * 128] = v
            for q in range(2):
                r = p * 32 + q * 16
                blk = [wd_v[pl.ds(mo(c * FC + r0, 16), 16), cc_].astype(f32)
                       for r0 in (r, 128 + r) for cc_ in (slice(0, 256), slice(256, 512))]
                for k, v in enumerate(sums9(*blk)):
                    ds_d[pl.ds(mo((cr * 5 + k) * 128 + r, 16), 16), :] = v

    _KN = (0, None, 1, 2, None, 3, 4)
    _KT = (0, None, 4, 3, None, 2, 1)

    def w_gu(c, i, tab):
        if tab[i] is not None:
            ref, cr = (guA_s, c) if c < 2 else (gu_s, c - 2)
            return ref[(cr * 5 + tab[i]) * 256:(cr * 5 + tab[i] + 1) * 256, :]
        hb = 0 if i == 1 else 1
        rs, cs = slice(hb * 256, (hb + 1) * 256), slice(c * FC + hb * 128, c * FC + (hb + 1) * 128)
        return jnp.concatenate([wg_v[rs, cs], wu_v[rs, cs]], axis=1)

    def w_dd(c, i, tab):
        if tab[i] is not None:
            ref, cr = (dsA_s, c) if c < 2 else (ds_s, c - 2)
            return ref[(cr * 5 + tab[i]) * 128:(cr * 5 + tab[i] + 1) * 128, :]
        hb = 0 if i == 1 else 1
        return wd_v[c * FC + hb * 128:c * FC + (hb + 1) * 128, hb * 256:(hb + 1) * 256]

    _KL = (0, 1, None, None, 2, 3, 4)

    def sums5(x11, x12, x21, x22):
        return [v.astype(bf16) for v in (x11 + x22, x21 + x22, x11 + x12, x21 - x11, x12 - x22)]

    def hcol(t):
        return pl.ds(mo(t * 128, 128), 128)

    def l_op(src_v, l_s, t, i):
        if _KL[i] is not None:
            return l_s[pl.ds(mo((t * 5 + _KL[i]) * 128, 128), 128), :]
        hb = i - 2
        return src_v[pl.ds(mo(t * T + hb * 128, 128), 128), hb * 256:(hb + 1) * 256]

    def l_store(l_s, t, r, n, xa, xb, mod=False):
        blk = (xa[:, 0:256], xa[:, 256:512], xb[:, 0:256], xb[:, 256:512])
        sums = [v for i, v in enumerate(_m7(*blk)) if i not in (2, 3)] if mod else sums5(*blk)
        for k, v in enumerate(sums):
            l_s[pl.ds(mo((t * 5 + k) * 128 + r, n), n), :] = v

    def l_sets(t, src_v, l_s):
        for r in range(0, 128, 16):
            xa = src_v[pl.ds(mo(t * T + r, 16), 16), :].astype(f32)
            xb = src_v[pl.ds(mo(t * T + 128 + r, 16), 16), :].astype(f32)
            l_store(l_s, t, r, 16, xa, xb, mod=True)

    def t_sets(t, src_v, t_s, tmp_s):
        for hb in range(2):
            xT = src_v[pl.ds(mo(t * T + hb * 128, 128), 128), :].T
            tmp_s[:, hb * 128:(hb + 1) * 128] = xT
        for r in range(0, 256, 32):
            blk = [tmp_s[r0:r0 + 32, cc_] for r0 in (r, 256 + r) for cc_ in (slice(0, 128), slice(128, 256))]
            t_s[2 * 256 + r:2 * 256 + r + 32, hcol(t)] = blk[0]
            t_s[3 * 256 + r:3 * 256 + r + 32, hcol(t)] = blk[3]
            for i, v in zip((0, 1, 4, 5, 6), sums5(*[b.astype(f32) for b in blk])):
                t_s[i * 256 + r:i * 256 + r + 32, hcol(t)] = v

    def ffn_dh(c, t):
        return _combine_t([_dot(l_op(dout_v, yl_s, t, i), w_dd(c, i, _KT), NT) for i in range(7)])

    def ffn_gu(c, t, lo=0, hi=7):
        return [_dot(l_op(xn_s, xl_s, t, i), w_gu(c, i, _KN)) for i in range(lo, hi)]

    def ffn_elem(dh, gu):
        gu = _combine(gu)
        g_ = [v[:, 0:128] for v in gu]
        u_ = [v[:, 128:256] for v in gu]
        return (_l7(*[a * b for a, b in zip(g_, u_)]),
                _m7(*[jnp.concatenate([d * b, d * a], axis=1) for d, a, b in zip(dh, g_, u_)]))

    def elem(c, t, st):
        e = ffn_elem(*st)
        for i in range(7):
            h_s[hcol(t), sl(c, i)] = e[0][_RP[i]]
            dg_s[hcol(t), sl2(c, i)] = e[1][_RP[i]]
        return e

    def acc7(acc, key, prods):
        acc[key] = prods if key not in acc else [a + b for a, b in zip(acc[key], prods)]

    def mm_o(c, acc, h7):
        acc7(acc, 'o', [_dot(h7[i], w_dd(c, i, _KN)) for i in range(7)])

    def mm_d(c, acc, e7):
        acc7(acc, 'd', [_dot(e7[i], w_gu(c, i, _KT), NT) for i in range(7)])

    def ffn_mm(c, acc, e):
        mm_o(c, acc, e[0])
        mm_d(c, acc, e[1])

    def sl2(c, i):
        return slice((c * 7 + i) * 256, (c * 7 + i + 1) * 256)

    _IRP = [_RP.index(i) for i in range(7)]

    def o_prods(t, cs_):
        return [sum(_dot(h_s[hcol(t), sl(c, _IRP[i])], w_dd(c, i, _KN)) for c in cs_) for i in range(7)]

    def d_prods(t, cs_, lo=0, hi=7):
        return [sum(_dot(dg_s[hcol(t), sl2(c, _IRP[i])], w_gu(c, i, _KT), NT) for c in cs_) for i in range(lo, hi)]

    def layernorm(t, staged=False):
        LB = 16
        xn_d, xl_d, td = (xnN_s, xlN_s, 0) if staged else (xn_s, xl_s, t)
        for r in range(0, 128, LB):
            pair = []
            for hb in range(2):
                rows = pl.ds(mo(t * T + hb * 128 + r, LB), LB)
                x = x_v[rows, :].astype(f32)
                mu = jnp.mean(x, axis=-1, keepdims=True)
                xc = x - mu
                var = jnp.mean(xc * xc, axis=-1, keepdims=True)
                rstd = jax.lax.rsqrt(var + 1e-5)
                xn = xc * rstd
                xn_d[pl.ds(mo(td * T + hb * 128 + r, LB), LB), :] = xn.astype(bf16)
                rstd_s[rows, :] = rstd
                pair.append(xn)
            l_store(xl_d, td, r, LB, *pair)
        return xn_d[tile_rows(td), :]

    def ln_commit(t):
        xn_s[tile_rows(t), :] = xnN_s[...]
        xl_s[pl.ds(mo(t * 640, 128), 640), :] = xlN_s[...]

    def k_phi(t, xn, b):
        pk = _dot(wT_s[512 + b * 128:512 + (b + 1) * 128, :], xn, NT)
        res = []
        for i in range(2):
            g = 2 * b + i
            phi = _phi(*_dual_softmax(pk[i * 64:(i + 1) * 64]))
            phik_s[g * 128:(g + 1) * 128, tile_rows(t)] = phi
            res.append(phi)
        return res

    def k_acc(t, xn, phis, first=False):
        pv = _dot(wT_s[1024:1536, :], xn, NT)
        for g in range(NG):
            v1 = jnp.concatenate([pv[g * 64:(g + 1) * 64], ones16], axis=0).astype(bf16)
            vT_s[g * 80:(g + 1) * 80, tile_rows(t)] = v1
            r = _dot(v1, phis[g], NT)
            if first:
                kvT_s[:, gl(g)] = r
            else:
                kvT_s[:, gl(g)] += r

    def phase1(t, nxt, extra=None):
        rows = tile_rows(t)
        phis = []
        acc = {}

        def kphi(b):
            if nxt is not None:
                phis.extend(k_phi(nxt, xn1, b))

        def ex(i):
            if extra is not None and i < len(extra):
                extra[i]()

        def ws(p):
            if nxt is not None:
                weight_sets(t + 2, p)

        if nxt is not None:
            xn1 = layernorm(nxt, staged=True)
        st0 = (ffn_dh(0, t), ffn_gu(0, t))
        gu1 = ffn_gu(1, t)
        ex(0)
        dh1 = ffn_dh(1, t)
        elem(0, t, st0)
        if nxt is not None:
            ln_commit(nxt)
        if not (isinstance(t, int) and t == NTILE - 1):
            l_sets(t + 1, dout_v, yl_s)
        ex(1)
        kphi(0)
        kphi(1)
        elem(1, t, (dh1, gu1))
        kphi(2)
        om = o_prods(t, (0, 1))
        kphi(3)
        dm = d_prods(t, (0, 1), 0, 4)
        out_s[rows, :] = x_v[rows, :].astype(f32) + _cat22(*_combine(om))
        if nxt is not None:
            k_acc(nxt, xn1, phis)
        dm += d_prods(t, (0, 1), 4, 7)
        for p in range(4):
            ws(p)
        dxn_s[rows, :] = _cat22(*_combine_t(dm))

    dkvT_s[...] = jnp.zeros_like(dkvT_s)
    gq_a[...] = jnp.zeros_like(gq_a)
    c_wphi.wait()
    w3 = wphi_v[...].reshape(256, 32)
    ym = jnp.where(dmask, _dot(w3, hsel), 0.0).astype(bf16)
    pmT_s[...] = jnp.where(hm4, _dot(rsel, ym), 0.0).astype(bf16)
    c_wv.start()
    c_x(1).start()
    c_x(0).wait()
    xn0 = layernorm(0)
    c_wk.wait()
    c_wdA.start()
    c_wgA.start()
    fold(1)
    for b in range(NBLK):
        k_phi(0, xn0, b)
    c_wv.wait()
    c_x(1).wait()
    c_wuA.start()
    c_do(0).start()
    c_x(2).start()
    xn1 = layernorm(1)
    fold(2)
    k_acc(0, xn_s[0:T, :], [phik_s[g * 128:(g + 1) * 128, 0:T] for g in range(NG)], first=True)
    k_acc(1, xn1, sum([k_phi(1, xn1, b) for b in range(NBLK)], []))
    c_wdA.wait()
    c_wgA.wait()
    c_wuA.wait()
    c_do(0).wait()
    c_x(2).wait()
    c_do(1).start()
    c_x(3).start()
    for cpy in c_wB(2):
        cpy.start()
    xn2 = layernorm(2)
    weight_sets(0)
    phis2 = sum([k_phi(2, xn2, b) for b in range(NBLK)], [])
    l_sets(0, dout_v, yl_s)
    weight_sets(1)
    k_acc(2, xn2, phis2)
    for t in range(1, NTILE - 3):
        c_do(t + 1).start()
        c_x(t + 3).start()
        for cpy in c_wB(t + 2):
            cpy.start()
    c_do(NTILE - 2).start()
    c_do(NTILE - 1).start()
    c_wq.start()
    c_wo.start()

    def p1_body(t, carry):
        c_do(t + 1).wait()
        c_x(t + 3).wait()
        for cpy in c_wB(t + 2):
            cpy.wait()
        phase1(t, t + 3)
        return carry

    jax.lax.fori_loop(0, NTILE - 3, p1_body, 0)
    c_do(NTILE - 2).wait()
    c_do(NTILE - 1).wait()

    c_wq.wait()
    c_wo.wait()

    def transposed(kv, dst):
        m = jnp.where(same_head & (rr < 68), kv, 0.0)
        m = jnp.concatenate([m, jnp.zeros((48, NG * 128), f32)], axis=0)
        for g in range(NG):
            mT = m[:, gl(g)].T
            halves = []
            for i in range(2):
                m3 = mT[i * 64:(i + 1) * 64].reshape(8, 8, 128)
                halves.append((m3 - (_hsum(m3) * (1.0 / DH))[None]).reshape(64, 128))
            dst[:, gl(g)] = jnp.concatenate(halves, axis=0).astype(bf16)

    def wkv_sets():
        for r in range(0, 512, 16):
            ra = 512 + (r // 256) * 512 + r % 256
            blk = [wT_s[r0:r0 + 16, cc_].astype(f32) for r0 in (ra, ra + 256) for cc_ in (slice(0, 256), slice(256, 512))]
            for k, v in enumerate(_w5(*blk)):
                wkvR_s[k * 512 + r:k * 512 + r + 16, :] = v

    def zero_gkv():
        gkv_a[...] = jnp.zeros_like(gkv_a)

    def wq_sets():
        for r in range(0, 256, 16):
            for j, w_s in enumerate((wT_s, wop_s)):
                blk = [w_s[r0:r0 + 16, cc_].astype(f32) for r0 in (r, 256 + r) for cc_ in (slice(0, 256), slice(256, 512))]
                first = [v for i, v in enumerate(_m7(*blk)) if i not in (2, 3)] if j == 0 else sums5(*blk)
                for k, v in enumerate(first + _w5(*blk)):
                    sq_s[(j * 10 + k) * 256 + r:(j * 10 + k) * 256 + r + 16, :] = v

    def sq_op(j, i, second):
        k = (_KN if second else _KL)[i]
        if k is not None:
            k += j * 10 + (5 if second else 0)
            return sq_s[k * 256:(k + 1) * 256, :]
        hb = (0 if i == 1 else 1) if second else i - 2
        return (wT_s, wop_s)[j][hb * 256:(hb + 1) * 256, hb * 256:(hb + 1) * 256]

    def extra0():
        kv = kvT_s[...]
        kvz_s[...] = jnp.where(same_head & (rr < 72), kv, 0.0).astype(bf16)
        transposed(kv, kv4_s)

    def extra1():
        fold(0)
        for b in range(NBLK):
            wop_s[b * 128:(b + 1) * 128, :] = _dot(permT, wo_v[b * 128:(b + 1) * 128, :]).astype(bf16)

    phase1(NTILE - 3, None, (extra0, extra1))
    phase1(NTILE - 2, None, (wkv_sets,))
    phase1(NTILE - 1, None, (zero_gkv, wq_sets))

    c0 = FA // FC

    def phase2(t, carry):
        rows = tile_rows(t)
        acc = {}

        def ffn1(c):
            return ffn_dh(c, t), ffn_gu(c, t)

        def mm(c, e):
            ffn_mm(c, acc, e)

        pq = _cat22(*_combine_t([_dot(sq_op(0, i, False), l_op(xn_s, xl_s, t, _XI[i]), NT) for i in range(7)]))
        ab = [_dual_softmax(pq[g * 64:(g + 1) * 64]) for g in range(NG)]
        phis = [_phi(a, b) for a, b in ab]
        doT = _cat22(*_combine_b([_dot(sq_op(1, i, False), l_op(dout_v, yl_s, t, _XI[i]), NT) for i in range(7)]))
        dn1s = {}

        def pair_sets(j, b, xa, xb):
            for i, v in enumerate(_l7(xa[:, 0:128], xa[:, 128:256], xb[:, 0:128], xb[:, 128:256])):
                os_s[b * 64:(b + 1) * 64, (j * 7 + i) * 128:(j * 7 + i + 1) * 128] = v

        def o_op(j, i):
            return os_s[:, (j * 7 + i) * 128:(j * 7 + i + 1) * 128]

        def stage2(b):
            pair = []
            for g in (b, b + 4):
                nd = _dot(kvz_s[:, gl(g)], phis[g])
                rden = 1.0 / (nd[64:72] + 1e-6)
                o3 = nd[0:64].reshape(8, 8, T) * rden[None]
                do3 = doT[g * 64:(g + 1) * 64].reshape(8, 8, T)
                dden = -_hsum(do3 * o3) * rden
                dn1s[g] = jnp.concatenate([(do3 * rden[None]).reshape(64, T), dden, zeros8], axis=0).astype(bf16)
                pair.append(o3.reshape(64, T))
            pair_sets(0, b, *pair)

        def stage3(b):
            pair = []
            for g in (b, b + 4):
                dphi = _dot(kv4_s[:, g * 128:g * 128 + 80], dn1s[g]).reshape(16, 8, T)
                a, b_ = ab[g]
                pair.append(_dual_softmax_bwd(a, b_, dphi[0:8], dphi[8:16]).reshape(64, T))
            pair_sets(1, b, *pair)

        def mm_o_all(cs_):
            acc7(acc, 'o', o_prods(t, cs_))

        def mm_d_all(cs_):
            return d_prods(t, cs_)

        dh0 = ffn_dh(c0, t)
        gu0 = ffn_gu(c0, t, 0, 4)
        stage2(0)
        gu0 += ffn_gu(c0, t, 4, 7)
        stage2(1)
        dh1 = ffn_dh(c0 + 1, t)
        stage2(2)
        gu1 = ffn_gu(c0 + 1, t, 0, 4)
        stage2(3)
        elem(c0, t, (dh0, gu0))
        gu1 += ffn_gu(c0 + 1, t, 4, 7)
        stage3(0)
        dh2 = ffn_dh(c0 + 2, t)
        stage3(1)
        gu2 = ffn_gu(c0 + 2, t, 0, 4)
        stage3(2)
        gu2 += ffn_gu(c0 + 2, t, 4, 7)
        stage3(3)
        for g in range(NG):
            dkvT_s[:, gl(g)] += _dot(dn1s[g], phis[g], NT)
        elem(c0 + 1, t, (dh1, gu1))
        o_att = _cat22(*_combine_tn([_dot(o_op(0, _TI[i]), sq_op(1, i, True), TN) for i in range(7)]))
        st3 = ffn1(c0 + 3)
        elem(c0 + 2, t, (dh2, gu2))
        st4 = ffn1(c0 - 1)
        elem(c0 + 3, t, st3)
        mm_o_all([c0, c0 + 1, c0 + 2])
        d_att = _cat22(*_combine_tn([_dot(o_op(1, _TI[i]), sq_op(0, i, True), TN) for i in range(7)]))
        elem(c0 - 1, t, st4)
        for i in range(7):
            gq_a[:, (7 + i) * 256:(8 + i) * 256] += _dot(o_op(0, i), l_op(dout_v, yl_s, t, _RP[i]))
        for i in range(7):
            gq_a[:, i * 256:(i + 1) * 256] += _dot(o_op(1, i), l_op(xn_s, xl_s, t, _RP[i]))
        mm_o_all([c0 + 3, c0 - 1])
        out_v[rows, :] = (out_s[rows, :] + o_att + _cat22(*_combine(acc['o']))).astype(bf16)
        t_sets(t, xn_s, xt_s, tmpx_s)
        t_sets(t, dout_v, yt_s, tmpy_s)
        dm = mm_d_all(range(c0 - 1, c0 + 4))
        dxn_s[rows, :] += d_att + _cat22(*_combine_t(dm))
        return carry

    jax.lax.fori_loop(0, NTILE, phase2, 0)
    o_out.start()

    dkv = dkvT_s[...]
    dkv4_s[...] = jnp.where(same_head, dkv, 0.0).astype(bf16)
    transposed(dkv, dkv4T_s)

    def unfold(part):
        for b in range(NBLK):
            m = pmT_s[:, b * 128:(b + 1) * 128] if part < 2 else permT
            cs = slice(part * 512 + b * 128, part * 512 + (b + 1) * 128)
            gblk = gT_s[cs, :].astype(bf16)
            dwqkv_v[:, cs] = _dot(gblk, m, TN).astype(bf16)
            if part == 0:
                aphi_s[:, b * 128:(b + 1) * 128] = _dot(gblk, wqkv_v[:, cs])
            elif part == 1:
                aphi_s[:, b * 128:(b + 1) * 128] += _dot(gblk, wqkv_v[:, cs])
        if part == 1:
            accm = jnp.where(hm4, aphi_s[...], 0.0).astype(bf16)
            z = jnp.where(dmask, _dot(rsel, accm, TN), 0.0).astype(bf16)
            dwphi_v[...] = _dot(z, hsel, NT).astype(bf16).reshape(16, 16, 32)

    def unfold_q():
        gT_s[0:512, :] = _cat22(*_combine([gq_a[:, i * 256:(i + 1) * 256] for i in range(7)]))
        unfold(0)

    def unperm_wo():
        dwo_s[...] = _cat22(*_combine_w([gq_a[:, (7 + i) * 256:(8 + i) * 256] for i in range(7)]))
        for b in range(NBLK):
            dwo_v[b * 128:(b + 1) * 128, :] = _dot(permT, dwo_s[b * 128:(b + 1) * 128, :].astype(bf16), TN).astype(bf16)

    def gu_prod(c, i):
        return _dot(xt_s[i * 256:(i + 1) * 256, :], dg_s[:, pl.ds(mo((c * 7 + i) * 256, 256), 256)])

    def d_prod(c, i):
        return _dot(yt_s[i * 256:(i + 1) * 256, :], h_s[:, pl.ds(mo((c * 7 + i) * 128, 128), 128)])

    def gu_store(c, m):
        cb = pl.ds(mo(c * FC, FC), FC)
        c11, c12, c21, c22 = _combine_w(m)
        for j, o_v in enumerate((dwg_v, dwu_v)):
            js = slice(j * 128, (j + 1) * 128)
            o_v[0:256, cb] = jnp.concatenate([c11[:, js], c12[:, js]], axis=1).astype(bf16)
            o_v[256:512, cb] = jnp.concatenate([c21[:, js], c22[:, js]], axis=1).astype(bf16)

    def d_store(c, m):
        dwd_v[pl.ds(mo(c * FC, FC), FC), :] = _cat22(*_combine(m)).astype(bf16).T

    def phase3(t, c, mode):
        rows = tile_rows(t)
        phis = [phik_s[g * 128:(g + 1) * 128, rows] for g in range(NG)]
        md = []

        def fill(k):
            if mode == 'first':
                if k == 0:
                    unfold_q()
                elif k == 1:
                    unperm_wo()
            else:
                md.extend(d_prod(c, i) for i in ((0, 1), (2, 3), (4, 5, 6))[k])

        def sm_bwd(b):
            for g in (2 * b, 2 * b + 1):
                dphi = _dot(dkv4T_s[:, g * 128:g * 128 + 80], vT_s[g * 80:(g + 1) * 80, rows]).reshape(16, 8, T)
                phif = phis[g].astype(f32).reshape(16, 8, T)
                dp = _dual_softmax_bwd(phif[0:8], phif[8:16], dphi[0:8], dphi[8:16])
                r0 = (g // 4) * 512 + (g % 4) * 64
                dp_s[r0:r0 + 64, :] = dp.reshape(64, T).astype(bf16)

        sm_bwd(0)
        for g in range(NG):
            r0 = (g // 4) * 512 + 256 + (g % 4) * 64
            dp_s[r0:r0 + 64, :] = _dot(dkv4_s[0:64, gl(g)], phis[g]).astype(bf16)
        sm_bwd(1)
        fill(0)
        sm_bwd(2)
        fill(1)
        sm_bwd(3)
        fill(2)
        if mode != 'first':
            d_store(c, md)

        for r in range(0, 512, 32):
            blk = [dp_s[r0:r0 + 32, cc_].astype(f32) for r0 in (r, 512 + r) for cc_ in (slice(0, 128), slice(128, 256))]
            for k, v in enumerate(sums5(*blk)):
                dps_s[r:r + 32, k * 128:(k + 1) * 128] = v

        def dp_op(i):
            if _KL[i] is not None:
                return dps_s[:, _KL[i] * 128:(_KL[i] + 1) * 128]
            hb = i - 2
            return dp_s[hb * 512:(hb + 1) * 512, hb * 128:(hb + 1) * 128]

        def dx_prod(i):
            k = _KN[i]
            hb = 0 if i == 1 else 1
            w = (wkvR_s[k * 512:(k + 1) * 512, :] if k is not None
                 else jnp.concatenate([wT_s[r0 + hb * 256:r0 + (hb + 1) * 256, hb * 256:(hb + 1) * 256]
                                       for r0 in (512, 1024)], axis=0))
            return _dot(dp_op(_TI[i]), w, TN)

        def g_acc(i):
            gkv_a[:, i * 256:(i + 1) * 256] += _dot(dp_op(i), l_op(xn_s, xl_s, t, _RP[i]))

        def ln_part(r, ca, cb_):
            rw = pl.ds(mo(t * T + r * 128, 128), 128)
            dxn = dxn_s[rw, :] + jnp.concatenate([ca, cb_], axis=1)
            xnf = xn_s[rw, :].astype(f32)
            m1 = jnp.mean(dxn, axis=-1, keepdims=True)
            m2 = jnp.mean(dxn * xnf, axis=-1, keepdims=True)
            dx = rstd_s[rw, :] * (dxn - m1 - xnf * m2) + dout_v[rw, :].astype(f32)
            dx_v[rw, :] = dx.astype(bf16)

        mg = []
        if mode != 'first':
            mg.append(gu_prod(c, 0))
        p = {i: dx_prod(i) for i in (2, 3, 0, 4, 6)}
        ln_part(0, p[0] - p[3] - p[4] + p[6], p[2] + p[4])
        for i in range(4):
            g_acc(i)
        p.update({i: dx_prod(i) for i in (1, 5)})
        ln_part(1, p[1] + p[3], p[5] - p[0] - p[1] - p[2])
        for i in range(4, 7):
            g_acc(i)
        if mode == 'first':
            o_dx(t).start()
            o_wq.start()
            o_wo.start()
        elif mode == 'last':
            ob = o_b(c)[0:1]
            for r in range(0, 512, 128):
                c11, c12, c21, c22 = _combine([gkv_a[r:r + 128, i * 256:(i + 1) * 256] for i in range(7)])
                ra = 512 + (r // 256) * 512 + r % 256
                gT_s[ra:ra + 128, :] = jnp.concatenate([c11, c12], axis=1)
                gT_s[ra + 256:ra + 384, :] = jnp.concatenate([c21, c22], axis=1)
            mg_s[0] = mg[0]
            mg_s[1] = gu_prod(c, 2)
            unfold(1)
            unfold(2)
            mg_s[2] = gu_prod(c, 3)
            o_dx(t).start()
            ob[0].start()
            o_wkv.start()
            o_wphi.start()
            cb = slice(c * FC, (c + 1) * FC)
            q4, q6 = gu_prod(c, 4), gu_prod(c, 6)
            c11, c12 = mg_s[0] + mg_s[2] + q4 + q6, q4 - mg_s[1]
            for j, o_v in enumerate((dwg_v, dwu_v)):
                js = slice(j * 128, (j + 1) * 128)
                o_v[0:256, cb] = jnp.concatenate([c11[:, js], c12[:, js]], axis=1).astype(bf16)
            for cpy in o_half(0):
                cpy.start()
            q1, q5 = gu_prod(c, 1), gu_prod(c, 5)
            c21, c22 = q1 + mg_s[2], q1 - mg_s[0] - mg_s[1] - q5
            for j, o_v in enumerate((dwg_v, dwu_v)):
                js = slice(j * 128, (j + 1) * 128)
                o_v[256:512, cb] = jnp.concatenate([c21[:, js], c22[:, js]], axis=1).astype(bf16)
            for cpy in o_half(1):
                cpy.start()
        else:
            gu_store(c, mg + [gu_prod(c, i) for i in range(1, 7)])
            o_dx(t).start()
            for cpy in o_b(c):
                cpy.start()

    def p3_body(c, carry):
        phase3(c + 1, c, 'mid')
        return carry

    phase3(0, None, 'first')
    jax.lax.fori_loop(0, NTILE - 2, p3_body, 0)
    phase3(NTILE - 1, NTILE - 2, 'last')

    o_out.wait()
    o_wq.wait()
    o_wo.wait()
    for t in range(NTILE):
        o_dx(t).wait()
    o_wkv.wait()
    o_wphi.wait()
    for c in range(F // FC):
        for cpy in o_b(c):
            cpy.wait()
    for cpy in o_half(0) + o_half(1):
        cpy.wait()


@jax.jit
def pallas_parallel_sum__linear_kernel_hedgehog__glu_gated_bilinear__prompt_kernel(
        A_x, A_wqkv, A_w_phi, A_wo, B_x, B_w_gate, B_w_up, B_w_down, grad_out):
    x = A_x.reshape(S, D)
    dout = grad_out.reshape(S, D)
    wphi = jnp.transpose(A_w_phi, (1, 2, 0))
    sds = jax.ShapeDtypeStruct
    io_shapes = ((S, D), (S, D), (D, 3 * D), (DH, DH, H), (D, D), (D, F), (D, F), (F, D))
    any_spec = pl.BlockSpec(memory_space=pl.ANY)

    def packed(r, c):
        return pltpu.VMEM((r // 2, c), u32)

    io_scratch = [pltpu.VMEM(s, bf16) if len(s) == 3 else packed(*s) for s in io_shapes]
    dma = pltpu.SemaphoreType.DMA
    outs = pl.pallas_call(
        kernel,
        out_shape=tuple(sds(s, bf16) for s in io_shapes),
        in_specs=[any_spec] * 8,
        out_specs=tuple([any_spec] * 8),
        scratch_shapes=io_scratch + io_scratch + [
            packed(3 * D, D),
            packed(D, D),
            packed(128, 512),
            packed(S, D),
            packed(NG * 128, S),
            packed(NG * 80, S),
            packed(80, NG * 128),
            packed(128, NG * 128),
            packed(80, NG * 128),
            packed(128, NG * 128),
            packed(S // 2, 7 * 896),
            packed(S // 2, 14 * 896),
            packed(2 * D, T),
            packed(NTILE * 640, 256),
            packed(7 * 256, S // 2),
            packed(NTILE * 640, 256),
            packed(7 * 256, S // 2),
            packed(25 * 256, 256),
            packed(25 * 128, 256),
            packed(10 * 256, 256),
            packed(10 * 128, 256),
            packed(512, 256),
            packed(512, 256),
            packed(5 * 512, 256),
            packed(512, 5 * 128),
            packed(20 * 256, 256),
            packed(256, 14 * 128),
            packed(T, D),
            packed(640, 256),
            pltpu.VMEM((S, 1), f32),
            pltpu.VMEM((80, NG * 128), f32),
            pltpu.VMEM((80, NG * 128), f32),
            pltpu.VMEM((3 * D, D), f32),
            pltpu.VMEM((D, D), f32),
            pltpu.VMEM((S, D), f32),
            pltpu.VMEM((S, D), f32),
            pltpu.VMEM((128, 512), f32),
            pltpu.VMEM((3, 256, 256), f32),
            pltpu.VMEM((512, 7 * 256), f32),
            pltpu.VMEM((256, 14 * 256), f32),
            dma((13,)),
        ],
        compiler_params=pltpu.CompilerParams(vmem_limit_bytes=126 * 1024 * 1024),
    )(x, A_wqkv, wphi, A_wo, B_w_gate, B_w_up, B_w_down, dout)
    out, dx, dwqkv, dwphi, dwo, dwg, dwu, dwd = outs
    return (out.reshape(1, S, D), dx.reshape(1, S, D), dwqkv, jnp.transpose(dwphi, (2, 0, 1)), dwo, dwg, dwu, dwd)
```

```python
import jax
import jax.numpy as jnp
import jax.experimental.pallas as pl
import jax.experimental.pallas.tpu as pltpu

S, D, H, DH, F = 2048, 512, 32, 16, 1792
NG = 8
NBLK = 4
T = 256
NTILE = S // T
FC = 256
FA1 = 2 * FC

f32 = jnp.float32
bf16 = jnp.bfloat16
u32 = jnp.uint32
NN = (((1,), (0,)), ((), ()))
NT = (((1,), (1,)), ((), ()))
TN = (((0,), (0,)), ((), ()))


def _dot(a, b, dn=NN):
    return jax.lax.dot_general(a, b, dn, preferred_element_type=f32)


def _head_reduce(x3, red, comb):
    r = red(x3, axis=0)
    return comb(r, pltpu.roll(r, 4, 0))


def _hsum(x3):
    return _head_reduce(x3, jnp.sum, jnp.add)


def _dual_softmax(p):
    p3 = p.reshape(8, 8, p.shape[-1])
    mx = _head_reduce(p3, jnp.max, jnp.maximum)
    mn = _head_reduce(p3, jnp.min, jnp.minimum)
    ea = jnp.exp(p3 - mx[None])
    eb = jnp.exp(mn[None] - p3)
    a = ea * (1.0 / _hsum(ea))[None]
    b = eb * (1.0 / _hsum(eb))[None]
    return a, b


def _dual_softmax_bwd(a, b, da, db):
    ta = a * da
    tb = b * db
    return (ta - a * _hsum(ta)[None]) - (tb - b * _hsum(tb)[None])


def _phi(a, b):
    return jnp.concatenate([a.reshape(64, T), b.reshape(64, T)], axis=0).astype(bf16)


_RP = (0, 2, 6, 5, 3, 4, 1)


def _l7(x11, x12, x21, x22):
    return [v.astype(bf16) for v in (x11 + x22, x21 + x22, x11, x22, x11 + x12, x21 - x11, x12 - x22)]


def _combine(m):
    m1, m2, m3, m4, m5, m6, m7 = m
    return m1 + m4 - m5 + m7, m3 + m5, m2 + m4, m1 - m2 + m3 + m6


def _m7(x11, x12, x21, x22):
    return [v.astype(bf16) for v in (x11 - x22, x21 - x22, x11, x22, x11 - x12, x21 - x11, x22 - x12)]


def _combine_t(p):
    return p[0] + p[3] - p[4] - p[6], p[2] - p[4], p[1] + p[3], p[1] - p[0] + p[2] + p[5]


def _combine_w(q):
    return q[0] + q[3] + q[4] + q[6], q[4] - q[2], q[1] + q[3], q[1] - q[0] - q[2] - q[5]


_XI = (0, 2, 1, 4, 3, 5, 6)


def _combine_b(p):
    return p[0] - p[3] + p[4] - p[6], p[2] + p[4], p[1] - p[3], p[1] - p[0] + p[2] + p[5]


def _combine_tn(p):
    return p[0] - p[3] - p[4] + p[6], p[2] + p[4], p[1] + p[3], p[5] - p[0] - p[1] - p[2]


_TI = (0, 6, 2, 3, 5, 4, 1)


def _w5(w11, w12, w21, w22):
    return [v.astype(bf16) for v in (w11 - w22, w12 + w22, w21 + w11, w11 + w12, w21 + w22)]


def _cat22(c11, c12, c21, c22):
    return jnp.concatenate([jnp.concatenate([c11, c12], axis=1), jnp.concatenate([c21, c22], axis=1)], axis=0)


def _iota(shape, dim):
    return jax.lax.broadcasted_iota(jnp.int32, shape, dim)


def kernel(x_hbm, wqkv_hbm, wphi_hbm, wo_hbm, wg_hbm, wu_hbm, wd_hbm, dout_hbm,
           out_hbm, dx_hbm, dwqkv_hbm, dwphi_hbm, dwo_hbm, dwg_hbm, dwu_hbm, dwd_hbm,
           x_v, dout_v, wqkv_v, wphi_v, wo_v, wg_v, wu_v, wd_v,
           out_v, dx_v, dwqkv_v, dwphi_v, dwo_v, dwg_v, dwu_v, dwd_v,
           wT_s, wop_s, pmT_s, xn_s, phik_s, vT_s, kvz_s, kv4_s, dkv4_s, dkv4T_s, h_s, dg_s,
           xl_s, xt_s, yl_s, yt_s, gu_s, ds_s, guA_s, dsA_s, tmpx_s, tmpy_s, wkvR_s, dps_s, sq_s, os_s, xnN_s, xlN_s,
           rstd_s, kvT_s, dkvT_s, gT_s, dwo_s, out_s, dxn_s, aphi_s, mg_s, gkv_a, gq_a, md_s,
           sem):
    (x_v, dout_v, wqkv_v, wo_v, wg_v, wu_v, wd_v, out_v, dx_v, dwqkv_v, dwo_v, dwg_v, dwu_v, dwd_v,
     wT_s, wop_s, pmT_s, xn_s, phik_s, vT_s, kvz_s, kv4_s, dkv4_s, dkv4T_s, h_s, dg_s,
           xl_s, xt_s, yl_s, yt_s, gu_s, ds_s, guA_s, dsA_s, tmpx_s, tmpy_s, wkvR_s, dps_s, sq_s, os_s, xnN_s, xlN_s) = [
         r.bitcast(bf16) for r in (
             x_v, dout_v, wqkv_v, wo_v, wg_v, wu_v, wd_v, out_v, dx_v, dwqkv_v, dwo_v, dwg_v, dwu_v, dwd_v,
             wT_s, wop_s, pmT_s, xn_s, phik_s, vT_s, kvz_s, kv4_s, dkv4_s, dkv4T_s, h_s, dg_s,
           xl_s, xt_s, yl_s, yt_s, gu_s, ds_s, guA_s, dsA_s, tmpx_s, tmpy_s, wkvR_s, dps_s, sq_s, os_s, xnN_s, xlN_s)]
    ALL = slice(None)

    def cp(src, dst, sem, *idx):
        if idx:
            src, dst = src.at[idx], dst.at[idx]
        return pltpu.make_async_copy(src, dst, sem)

    def mo(v, m):
        return v if isinstance(v, int) else pl.multiple_of(v, m)

    def tile_rows(t):
        return pl.ds(mo(t * T, T), T)

    def gl(g):
        return slice(g * 128, (g + 1) * 128)

    c_wphi = cp(wphi_hbm, wphi_v, sem.at[6])
    c_wk = cp(wqkv_hbm, wqkv_v, sem.at[8], ALL, slice(512, 1024))
    c_wv = cp(wqkv_hbm, wqkv_v, sem.at[9], ALL, slice(1024, 1536))
    c_wq = cp(wqkv_hbm, wqkv_v, sem.at[11], ALL, slice(0, 512))
    c_wo = cp(wo_hbm, wo_v, sem.at[11])
    c_wgA = cp(wg_hbm, wg_v, sem.at[10], ALL, slice(0, FA1))
    c_wuA = cp(wu_hbm, wu_v, sem.at[10], ALL, slice(0, FA1))
    c_wdA = cp(wd_hbm, wd_v, sem.at[10], slice(0, FA1), ALL)

    def c_wB(c):
        cs = pl.ds(mo(c * FC, FC), FC)
        return (cp(wg_hbm, wg_v, sem.at[c - 2], ALL, cs), cp(wu_hbm, wu_v, sem.at[c - 2], ALL, cs),
                cp(wd_hbm, wd_v, sem.at[c - 2], cs, ALL))

    sem_o = sem.at[5]

    def c_x(t):
        s = {0: 7, 1: 9, 2: 10}.get(t, t - 3) if isinstance(t, int) else t - 3
        return cp(x_hbm, x_v, sem.at[s], tile_rows(t), ALL)

    def c_do(t):
        s = {0: 10, 6: 11, 7: 11}.get(t, t - 1) if isinstance(t, int) else t - 1
        return cp(dout_hbm, dout_v, sem.at[s], tile_rows(t), ALL)

    c_wphi.start()
    c_x(0).start()
    c_wk.start()

    o_out = cp(out_v, out_hbm, sem_o)

    def o_dx(t):
        return cp(dx_v, dx_hbm, sem_o, tile_rows(t), ALL)

    def o_b(c):
        cb = pl.ds(mo(c * FC, FC), FC)
        if isinstance(c, int) and c == F // FC - 1:
            return (cp(dwd_v, dwd_hbm, sem_o, cb, ALL),)
        return (cp(dwd_v, dwd_hbm, sem_o, cb, ALL), cp(dwg_v, dwg_hbm, sem_o, ALL, cb), cp(dwu_v, dwu_hbm, sem_o, ALL, cb))

    def o_half(h):
        cb, rs = slice(F - FC, F), slice(h * 256, (h + 1) * 256)
        return cp(dwg_v, dwg_hbm, sem_o, rs, cb), cp(dwu_v, dwu_hbm, sem_o, rs, cb)

    o_wq = cp(dwqkv_v, dwqkv_hbm, sem_o, ALL, slice(0, 512))
    o_wkv = cp(dwqkv_v, dwqkv_hbm, sem_o, ALL, slice(512, 1536))
    o_wo = cp(dwo_v, dwo_hbm, sem_o)
    o_wphi = cp(dwphi_v, dwphi_hbm, sem_o)

    def row_head(r):
        return (r // 64) * 4 + r % 4

    def row_feat(r):
        return ((r % 64) // 8) * 2 + (r % 8) // 4

    r_i = _iota((128, 128), 0)
    c_i = _iota((128, 128), 1)
    permT = jnp.where((row_head(r_i) == c_i // 16) & (row_feat(r_i) == c_i % 16), 1.0, 0.0).astype(bf16)
    hsel = jnp.where(_iota((32, 512), 0) == (_iota((32, 512), 1) // 16), 1.0, 0.0).astype(bf16)
    dmask = (_iota((256, 512), 0) // 16) == (_iota((256, 512), 1) % 16)
    rsel = jnp.where(row_feat(_iota((128, 256), 0)) == (_iota((128, 256), 1) % 16), 1.0, 0.0).astype(bf16)
    hm4 = row_head(_iota((128, 512), 0)) == ((_iota((128, 512), 1) // 16) % 8)
    ones16 = jnp.ones((16, T), f32)
    zeros8 = jnp.zeros((8, T), f32)
    rr = _iota((80, NG * 128), 0)
    same_head = (rr % 4) == (_iota((80, NG * 128), 1) % 4)

    def fold(part):
        for b in range(NBLK):
            m = pmT_s[:, b * 128:(b + 1) * 128] if part < 2 else permT
            cs = slice(part * 512 + b * 128, part * 512 + (b + 1) * 128)
            wT_s[cs, :] = _dot(m, wqkv_v[:, cs], NT).astype(bf16)

    def sl(c, i):
        return slice((c * 7 + i) * 128, (c * 7 + i + 1) * 128)

    def wsums5(b11, b12, b21, b22):
        return [v.astype(bf16) for v in (b11 + b22, b12 - b22, b21 - b11, b11 + b12, b21 + b22)]

    def weight_sets(c, part=None):
        c1 = pl.ds(mo(c * FC, 128), 128)
        c2 = pl.ds(mo(c * FC + 128, 128), 128)
        gu_d, ds_d, cr = (guA_s, dsA_s, c) if isinstance(c, int) and c < 2 else (gu_s, ds_s, c - 2)
        for p in (range(4) if part is None else [part]):
            for q in range(2):
                r = p * 64 + q * 32
                for j, w_v in enumerate((wg_v, wu_v)):
                    blk = [w_v[r0:r0 + 32, cc_].astype(f32) for r0 in (r, 256 + r) for cc_ in (c1, c2)]
                    for k, v in enumerate(wsums5(*blk)):
                        gu_d[pl.ds(mo((cr * 5 + k) * 256 + r, 32), 32), j * 128:(j + 1) * 128] = v
            for q in range(2):
                r = p * 32 + q * 16
                blk = [wd_v[pl.ds(mo(c * FC + r0, 16), 16), cc_].astype(f32)
                       for r0 in (r, 128 + r) for cc_ in (slice(0, 256), slice(256, 512))]
                for k, v in enumerate(wsums5(*blk)):
                    ds_d[pl.ds(mo((cr * 5 + k) * 128 + r, 16), 16), :] = v

    _KN = (0, None, 1, 2, None, 3, 4)
    _KT = (0, None, 4, 3, None, 2, 1)

    def w_gu(c, i, tab):
        if tab[i] is not None:
            ref, cr = (guA_s, c) if c < 2 else (gu_s, c - 2)
            return ref[(cr * 5 + tab[i]) * 256:(cr * 5 + tab[i] + 1) * 256, :]
        hb = 0 if i == 1 else 1
        rs, cs = slice(hb * 256, (hb + 1) * 256), slice(c * FC + hb * 128, c * FC + (hb + 1) * 128)
        return jnp.concatenate([wg_v[rs, cs], wu_v[rs, cs]], axis=1)

    def w_dd(c, i, tab):
        if tab[i] is not None:
            ref, cr = (dsA_s, c) if c < 2 else (ds_s, c - 2)
            return ref[(cr * 5 + tab[i]) * 128:(cr * 5 + tab[i] + 1) * 128, :]
        hb = 0 if i == 1 else 1
        return wd_v[c * FC + hb * 128:c * FC + (hb + 1) * 128, hb * 256:(hb + 1) * 256]

    _KL = (0, 1, None, None, 2, 3, 4)

    def sums5(x11, x12, x21, x22):
        return [v.astype(bf16) for v in (x11 + x22, x21 + x22, x11 + x12, x21 - x11, x12 - x22)]

    def hcol(t):
        return pl.ds(mo(t * 128, 128), 128)

    def l_op(src_v, l_s, t, i):
        if _KL[i] is not None:
            return l_s[pl.ds(mo((t * 5 + _KL[i]) * 128, 128), 128), :]
        hb = i - 2
        return src_v[pl.ds(mo(t * T + hb * 128, 128), 128), hb * 256:(hb + 1) * 256]

    def l_store(l_s, t, r, n, xa, xb, mod=False):
        blk = (xa[:, 0:256], xa[:, 256:512], xb[:, 0:256], xb[:, 256:512])
        sums = [v for i, v in enumerate(_m7(*blk)) if i not in (2, 3)] if mod else sums5(*blk)
        for k, v in enumerate(sums):
            l_s[pl.ds(mo((t * 5 + k) * 128 + r, n), n), :] = v

    def l_sets(t, src_v, l_s):
        for r in range(0, 128, 16):
            xa = src_v[pl.ds(mo(t * T + r, 16), 16), :].astype(f32)
            xb = src_v[pl.ds(mo(t * T + 128 + r, 16), 16), :].astype(f32)
            l_store(l_s, t, r, 16, xa, xb, mod=True)

    def t_sets(t, src_v, t_s, tmp_s):
        for hb in range(2):
            xT = src_v[pl.ds(mo(t * T + hb * 128, 128), 128), :].T
            tmp_s[:, hb * 128:(hb + 1) * 128] = xT
        for r in range(0, 256, 32):
            blk = [tmp_s[r0:r0 + 32, cc_] for r0 in (r, 256 + r) for cc_ in (slice(0, 128), slice(128, 256))]
            t_s[2 * 256 + r:2 * 256 + r + 32, hcol(t)] = blk[0]
            t_s[3 * 256 + r:3 * 256 + r + 32, hcol(t)] = blk[3]
            for i, v in zip((0, 1, 4, 5, 6), sums5(*[b.astype(f32) for b in blk])):
                t_s[i * 256 + r:i * 256 + r + 32, hcol(t)] = v

    def ffn_dh(c, t):
        return _combine_t([_dot(l_op(dout_v, yl_s, t, i), w_dd(c, i, _KT), NT) for i in range(7)])

    def ffn_gu(c, t, lo=0, hi=7):
        return [_dot(l_op(xn_s, xl_s, t, i), w_gu(c, i, _KN)) for i in range(lo, hi)]

    def ffn_elem(dh, gu):
        gu = _combine(gu)
        g_ = [v[:, 0:128] for v in gu]
        u_ = [v[:, 128:256] for v in gu]
        return (_l7(*[a * b for a, b in zip(g_, u_)]),
                _m7(*[jnp.concatenate([d * b, d * a], axis=1) for d, a, b in zip(dh, g_, u_)]))

    def elem(c, t, st):
        e = ffn_elem(*st)
        for i in range(7):
            h_s[hcol(t), sl(c, i)] = e[0][_RP[i]]
            dg_s[hcol(t), sl2(c, i)] = e[1][_RP[i]]
        return e

    def acc7(acc, key, prods):
        acc[key] = prods if key not in acc else [a + b for a, b in zip(acc[key], prods)]

    def sl2(c, i):
        return slice((c * 7 + i) * 256, (c * 7 + i + 1) * 256)

    _IRP = [_RP.index(i) for i in range(7)]

    def o_prods(t, cs_):
        return [sum(_dot(h_s[hcol(t), sl(c, _IRP[i])], w_dd(c, i, _KN)) for c in cs_) for i in range(7)]

    def d_prods(t, cs_, lo=0, hi=7):
        return [sum(_dot(dg_s[hcol(t), sl2(c, _IRP[i])], w_gu(c, i, _KT), NT) for c in cs_) for i in range(lo, hi)]

    def layernorm(t, staged=False):
        LB = 16
        xn_d, xl_d, td = (xnN_s, xlN_s, 0) if staged else (xn_s, xl_s, t)
        for r in range(0, 128, LB):
            pair = []
            for hb in range(2):
                rows = pl.ds(mo(t * T + hb * 128 + r, LB), LB)
                x = x_v[rows, :].astype(f32)
                mu = jnp.mean(x, axis=-1, keepdims=True)
                xc = x - mu
                var = jnp.mean(xc * xc, axis=-1, keepdims=True)
                rstd = jax.lax.rsqrt(var + 1e-5)
                xn = xc * rstd
                xn_d[pl.ds(mo(td * T + hb * 128 + r, LB), LB), :] = xn.astype(bf16)
                rstd_s[rows, :] = rstd
                pair.append(xn)
            l_store(xl_d, td, r, LB, *pair)
        return xn_d[tile_rows(td), :]

    def ln_commit(t):
        xn_s[tile_rows(t), :] = xnN_s[...]
        xl_s[pl.ds(mo(t * 640, 128), 640), :] = xlN_s[...]

    def k_phi(t, xn, b):
        pk = _dot(wT_s[512 + b * 128:512 + (b + 1) * 128, :], xn, NT)
        res = []
        for i in range(2):
            g = 2 * b + i
            phi = _phi(*_dual_softmax(pk[i * 64:(i + 1) * 64]))
            phik_s[g * 128:(g + 1) * 128, tile_rows(t)] = phi
            res.append(phi)
        return res

    def k_acc(t, xn, phis, first=False):
        pv = _dot(wT_s[1024:1536, :], xn, NT)
        for g in range(NG):
            v1 = jnp.concatenate([pv[g * 64:(g + 1) * 64], ones16], axis=0).astype(bf16)
            vT_s[g * 80:(g + 1) * 80, tile_rows(t)] = v1
            r = _dot(v1, phis[g], NT)
            if first:
                kvT_s[:, gl(g)] = r
            else:
                kvT_s[:, gl(g)] += r

    def phase1(t, nxt, extra=None):
        rows = tile_rows(t)
        phis = []

        def kphi(b):
            if nxt is not None:
                phis.extend(k_phi(nxt, xn1, b))

        def ex(i):
            if extra is not None and i < len(extra):
                extra[i]()

        def ws(p):
            if nxt is not None:
                weight_sets(t + 2, p)

        if nxt is not None:
            xn1 = layernorm(nxt, staged=True)
        st0 = (ffn_dh(0, t), ffn_gu(0, t))
        gu1 = ffn_gu(1, t)
        ex(0)
        dh1 = ffn_dh(1, t)
        elem(0, t, st0)
        if nxt is not None:
            ln_commit(nxt)
        if not (isinstance(t, int) and t == NTILE - 1):
            l_sets(t + 1, dout_v, yl_s)
        ex(1)
        kphi(0)
        kphi(1)
        elem(1, t, (dh1, gu1))
        kphi(2)
        om = o_prods(t, (0, 1))
        kphi(3)
        dm = d_prods(t, (0, 1), 0, 4)
        out_s[rows, :] = x_v[rows, :].astype(f32) + _cat22(*_combine(om))
        if nxt is not None:
            k_acc(nxt, xn1, phis)
        dm += d_prods(t, (0, 1), 4, 7)
        for p in range(4):
            ws(p)
        dxn_s[rows, :] = _cat22(*_combine_t(dm))

    dkvT_s[...] = jnp.zeros_like(dkvT_s)
    gq_a[...] = jnp.zeros_like(gq_a)
    c_wphi.wait()
    w3 = wphi_v[...].reshape(256, 32)
    ym = jnp.where(dmask, _dot(w3, hsel), 0.0).astype(bf16)
    pmT_s[...] = jnp.where(hm4, _dot(rsel, ym), 0.0).astype(bf16)
    c_wv.start()
    c_x(1).start()
    c_x(0).wait()
    xn0 = layernorm(0)
    c_wk.wait()
    c_wdA.start()
    c_wgA.start()
    fold(1)
    for b in range(NBLK):
        k_phi(0, xn0, b)
    c_wv.wait()
    c_x(1).wait()
    c_wuA.start()
    c_do(0).start()
    c_x(2).start()
    xn1 = layernorm(1)
    fold(2)
    k_acc(0, xn_s[0:T, :], [phik_s[g * 128:(g + 1) * 128, 0:T] for g in range(NG)], first=True)
    k_acc(1, xn1, sum([k_phi(1, xn1, b) for b in range(NBLK)], []))
    c_wdA.wait()
    c_wgA.wait()
    c_wuA.wait()
    c_do(0).wait()
    c_x(2).wait()
    c_do(1).start()
    c_x(3).start()
    for cpy in c_wB(2):
        cpy.start()
    xn2 = layernorm(2)
    weight_sets(0)
    phis2 = sum([k_phi(2, xn2, b) for b in range(NBLK)], [])
    l_sets(0, dout_v, yl_s)
    weight_sets(1)
    k_acc(2, xn2, phis2)
    for t in range(1, NTILE - 3):
        c_do(t + 1).start()
        c_x(t + 3).start()
        for cpy in c_wB(t + 2):
            cpy.start()
    c_do(NTILE - 2).start()
    c_do(NTILE - 1).start()
    c_wq.start()
    c_wo.start()

    def p1_body(t, carry):
        c_do(t + 1).wait()
        c_x(t + 3).wait()
        for cpy in c_wB(t + 2):
            cpy.wait()
        phase1(t, t + 3)
        return carry

    jax.lax.fori_loop(0, NTILE - 3, p1_body, 0)
    c_do(NTILE - 2).wait()
    c_do(NTILE - 1).wait()

    c_wq.wait()
    c_wo.wait()

    def transposed(kv, dst):
        m = jnp.where(same_head & (rr < 68), kv, 0.0)
        m = jnp.concatenate([m, jnp.zeros((48, NG * 128), f32)], axis=0)
        for g in range(NG):
            mT = m[:, gl(g)].T
            halves = []
            for i in range(2):
                m3 = mT[i * 64:(i + 1) * 64].reshape(8, 8, 128)
                halves.append((m3 - (_hsum(m3) * (1.0 / DH))[None]).reshape(64, 128))
            dst[:, gl(g)] = jnp.concatenate(halves, axis=0).astype(bf16)

    def wkv_sets():
        for r in range(0, 512, 16):
            ra = 512 + (r // 256) * 512 + r % 256
            blk = [wT_s[r0:r0 + 16, cc_].astype(f32) for r0 in (ra, ra + 256) for cc_ in (slice(0, 256), slice(256, 512))]
            for k, v in enumerate(_w5(*blk)):
                wkvR_s[k * 512 + r:k * 512 + r + 16, :] = v

    def wq_sets():
        for r in range(0, 256, 16):
            for j, w_s in enumerate((wT_s, wop_s)):
                blk = [w_s[r0:r0 + 16, cc_].astype(f32) for r0 in (r, 256 + r) for cc_ in (slice(0, 256), slice(256, 512))]
                first = [v for i, v in enumerate(_m7(*blk)) if i not in (2, 3)] if j == 0 else sums5(*blk)
                for k, v in enumerate(first + _w5(*blk)):
                    sq_s[(j * 10 + k) * 256 + r:(j * 10 + k) * 256 + r + 16, :] = v

    def sq_op(j, i, second):
        k = (_KN if second else _KL)[i]
        if k is not None:
            k += j * 10 + (5 if second else 0)
            return sq_s[k * 256:(k + 1) * 256, :]
        hb = (0 if i == 1 else 1) if second else i - 2
        return (wT_s, wop_s)[j][hb * 256:(hb + 1) * 256, hb * 256:(hb + 1) * 256]

    def extra0():
        kv = kvT_s[...]
        kvz_s[...] = jnp.where(same_head & (rr < 72), kv, 0.0).astype(bf16)
        transposed(kv, kv4_s)

    def extra1():
        fold(0)
        for b in range(NBLK):
            wop_s[b * 128:(b + 1) * 128, :] = _dot(permT, wo_v[b * 128:(b + 1) * 128, :]).astype(bf16)

    phase1(NTILE - 3, None, (extra0, extra1))
    phase1(NTILE - 2, None, (wkv_sets,))
    phase1(NTILE - 1, None, (wq_sets,))

    c0 = 3

    def phase2(t, carry):
        rows = tile_rows(t)
        acc = {}

        def ffn1(c):
            return ffn_dh(c, t), ffn_gu(c, t)

        pq = _cat22(*_combine_t([_dot(sq_op(0, i, False), l_op(xn_s, xl_s, t, _XI[i]), NT) for i in range(7)]))
        ab = [_dual_softmax(pq[g * 64:(g + 1) * 64]) for g in range(NG)]
        phis = [_phi(a, b) for a, b in ab]
        doT = _cat22(*_combine_b([_dot(sq_op(1, i, False), l_op(dout_v, yl_s, t, _XI[i]), NT) for i in range(7)]))
        dn1s = {}

        def pair_sets(j, b, xa, xb):
            for i, v in enumerate(_l7(xa[:, 0:128], xa[:, 128:256], xb[:, 0:128], xb[:, 128:256])):
                os_s[b * 64:(b + 1) * 64, (j * 7 + i) * 128:(j * 7 + i + 1) * 128] = v

        def o_op(j, i):
            return os_s[:, (j * 7 + i) * 128:(j * 7 + i + 1) * 128]

        def stage2(b):
            pair = []
            for g in (b, b + 4):
                nd = _dot(kvz_s[:, gl(g)], phis[g])
                rden = 1.0 / (nd[64:72] + 1e-6)
                o3 = nd[0:64].reshape(8, 8, T) * rden[None]
                do3 = doT[g * 64:(g + 1) * 64].reshape(8, 8, T)
                dden = -_hsum(do3 * o3) * rden
                dn1s[g] = jnp.concatenate([(do3 * rden[None]).reshape(64, T), dden, zeros8], axis=0).astype(bf16)
                pair.append(o3.reshape(64, T))
            pair_sets(0, b, *pair)

        def stage3(b):
            pair = []
            for g in (b, b + 4):
                dphi = _dot(kv4_s[:, g * 128:g * 128 + 80], dn1s[g]).reshape(16, 8, T)
                a, b_ = ab[g]
                pair.append(_dual_softmax_bwd(a, b_, dphi[0:8], dphi[8:16]).reshape(64, T))
            pair_sets(1, b, *pair)

        def mm_o_all(cs_):
            acc7(acc, 'o', o_prods(t, cs_))

        def mm_d_all(cs_):
            return d_prods(t, cs_)

        dh0 = ffn_dh(c0, t)
        gu0 = ffn_gu(c0, t, 0, 4)
        stage2(0)
        gu0 += ffn_gu(c0, t, 4, 7)
        stage2(1)
        dh1 = ffn_dh(c0 + 1, t)
        stage2(2)
        gu1 = ffn_gu(c0 + 1, t, 0, 4)
        stage2(3)
        elem(c0, t, (dh0, gu0))
        gu1 += ffn_gu(c0 + 1, t, 4, 7)
        stage3(0)
        dh2 = ffn_dh(c0 + 2, t)
        stage3(1)
        gu2 = ffn_gu(c0 + 2, t, 0, 4)
        stage3(2)
        gu2 += ffn_gu(c0 + 2, t, 4, 7)
        stage3(3)
        for g in range(NG):
            dkvT_s[:, gl(g)] += _dot(dn1s[g], phis[g], NT)
        elem(c0 + 1, t, (dh1, gu1))
        o_att = _cat22(*_combine_tn([_dot(o_op(0, _TI[i]), sq_op(1, i, True), TN) for i in range(7)]))
        st3 = ffn1(c0 + 3)
        elem(c0 + 2, t, (dh2, gu2))
        st4 = ffn1(c0 - 1)
        elem(c0 + 3, t, st3)
        mm_o_all([c0, c0 + 1, c0 + 2])
        d_att = _cat22(*_combine_tn([_dot(o_op(1, _TI[i]), sq_op(0, i, True), TN) for i in range(7)]))
        elem(c0 - 1, t, st4)
        for i in range(7):
            gq_a[:, (7 + i) * 256:(8 + i) * 256] += _dot(o_op(0, i), l_op(dout_v, yl_s, t, _RP[i]))
        for i in range(7):
            gq_a[:, i * 256:(i + 1) * 256] += _dot(o_op(1, i), l_op(xn_s, xl_s, t, _RP[i]))
        mm_o_all([c0 + 3, c0 - 1])
        out_v[rows, :] = (out_s[rows, :] + o_att + _cat22(*_combine(acc['o']))).astype(bf16)
        t_sets(t, xn_s, xt_s, tmpx_s)
        t_sets(t, dout_v, yt_s, tmpy_s)
        dm = mm_d_all(range(c0 - 1, c0 + 4))
        dxn_s[rows, :] += d_att + _cat22(*_combine_t(dm))
        return carry

    jax.lax.fori_loop(0, NTILE, phase2, 0)
    o_out.start()

    dkv = dkvT_s[...]
    dkv4_s[...] = jnp.where(same_head, dkv, 0.0).astype(bf16)
    transposed(dkv, dkv4T_s)

    def unfold(part):
        for b in range(NBLK):
            m = pmT_s[:, b * 128:(b + 1) * 128] if part < 2 else permT
            cs = slice(part * 512 + b * 128, part * 512 + (b + 1) * 128)
            gblk = gT_s[cs, :].astype(bf16)
            dwqkv_v[:, cs] = _dot(gblk, m, TN).astype(bf16)
            if part == 0:
                aphi_s[:, b * 128:(b + 1) * 128] = _dot(gblk, wqkv_v[:, cs])
            elif part == 1:
                aphi_s[:, b * 128:(b + 1) * 128] += _dot(gblk, wqkv_v[:, cs])
        if part == 1:
            accm = jnp.where(hm4, aphi_s[...], 0.0).astype(bf16)
            z = jnp.where(dmask, _dot(rsel, accm, TN), 0.0).astype(bf16)
            dwphi_v[...] = _dot(z, hsel, NT).astype(bf16).reshape(16, 16, 32)

    def unfold_q():
        gT_s[0:512, :] = _cat22(*_combine([gq_a[:, i * 256:(i + 1) * 256] for i in range(7)]))
        unfold(0)

    def unperm_wo():
        dwo_s[...] = _cat22(*_combine_w([gq_a[:, (7 + i) * 256:(8 + i) * 256] for i in range(7)]))
        for b in range(NBLK):
            dwo_v[b * 128:(b + 1) * 128, :] = _dot(permT, dwo_s[b * 128:(b + 1) * 128, :].astype(bf16), TN).astype(bf16)

    def gu_prod(c, i):
        return _dot(xt_s[i * 256:(i + 1) * 256, :], dg_s[:, pl.ds(mo((c * 7 + i) * 256, 256), 256)])

    def d_prod(c, i):
        return _dot(yt_s[i * 256:(i + 1) * 256, :], h_s[:, pl.ds(mo((c * 7 + i) * 128, 128), 128)])

    def gu_store(c, m):
        cb = pl.ds(mo(c * FC, FC), FC)
        c11, c12, c21, c22 = _combine_w(m)
        for j, o_v in enumerate((dwg_v, dwu_v)):
            js = slice(j * 128, (j + 1) * 128)
            o_v[0:256, cb] = jnp.concatenate([c11[:, js], c12[:, js]], axis=1).astype(bf16)
            o_v[256:512, cb] = jnp.concatenate([c21[:, js], c22[:, js]], axis=1).astype(bf16)

    def d_store(c, m):
        dwd_v[pl.ds(mo(c * FC, FC), FC), :] = _cat22(*_combine(m)).astype(bf16).T

    def phase3(t, c, mode):
        rows = tile_rows(t)
        phis = [phik_s[g * 128:(g + 1) * 128, rows] for g in range(NG)]
        md = []

        CL = F // FC - 1

        def fill(k):
            if mode == 'first':
                if k == 0:
                    unfold_q()
                elif k == 1:
                    unperm_wo()
                else:
                    md_s[0] = d_prod(CL, 0)
                    md_s[1] = d_prod(CL, 1)
            elif mode == 'last':
                md.append(d_prod(c, 4 + k))
            else:
                md.extend(d_prod(c, i) for i in ((0, 1), (2, 3), (4, 5, 6))[k])

        def pair_sets(r0, xa, xb):
            for i, v in enumerate(_l7(xa[:, 0:128], xa[:, 128:256], xb[:, 0:128], xb[:, 128:256])):
                dps_s[r0:r0 + 64, i * 128:(i + 1) * 128] = v

        def sm_bwd(b):
            pair = []
            for g in (b, b + 4):
                dphi = _dot(dkv4T_s[:, g * 128:g * 128 + 80], vT_s[g * 80:(g + 1) * 80, rows]).reshape(16, 8, T)
                phif = phis[g].astype(f32).reshape(16, 8, T)
                pair.append(_dual_softmax_bwd(phif[0:8], phif[8:16], dphi[0:8], dphi[8:16]).reshape(64, T))
            pair_sets(b * 64, *pair)

        sm_bwd(0)
        for b in range(4):
            pair_sets(256 + b * 64, *[_dot(dkv4_s[0:64, gl(g)], phis[g]).astype(bf16).astype(f32) for g in (b, b + 4)])
        sm_bwd(1)
        fill(0)
        sm_bwd(2)
        fill(1)
        sm_bwd(3)
        fill(2)
        if mode == 'mid':
            d_store(c, md)
        elif mode == 'last':
            d_store(c, [md_s[i] for i in range(4)] + md)

        def dp_op(i):
            return dps_s[:, i * 128:(i + 1) * 128]

        def dx_prod(i):
            k = _KN[i]
            hb = 0 if i == 1 else 1
            w = (wkvR_s[k * 512:(k + 1) * 512, :] if k is not None
                 else jnp.concatenate([wT_s[r0 + hb * 256:r0 + (hb + 1) * 256, hb * 256:(hb + 1) * 256]
                                       for r0 in (512, 1024)], axis=0))
            return _dot(dp_op(_TI[i]), w, TN)

        def g_acc(i):
            r = _dot(dp_op(i), l_op(xn_s, xl_s, t, _RP[i]))
            if mode == 'first':
                gkv_a[:, i * 256:(i + 1) * 256] = r
            else:
                gkv_a[:, i * 256:(i + 1) * 256] += r

        def ln_part(r, ca, cb_):
            rw = pl.ds(mo(t * T + r * 128, 128), 128)
            dxn = dxn_s[rw, :] + jnp.concatenate([ca, cb_], axis=1)
            xnf = xn_s[rw, :].astype(f32)
            m1 = jnp.mean(dxn, axis=-1, keepdims=True)
            m2 = jnp.mean(dxn * xnf, axis=-1, keepdims=True)
            dx = rstd_s[rw, :] * (dxn - m1 - xnf * m2) + dout_v[rw, :].astype(f32)
            dx_v[rw, :] = dx.astype(bf16)

        mg = []
        if mode != 'first':
            mg.append(gu_prod(c, 0))
        else:
            md_s[2] = d_prod(CL, 2)
        p = {i: dx_prod(i) for i in (2, 3, 0, 4, 6)}
        ln_part(0, p[0] - p[3] - p[4] + p[6], p[2] + p[4])
        for i in range(4):
            g_acc(i)
        p.update({i: dx_prod(i) for i in (1, 5)})
        ln_part(1, p[1] + p[3], p[5] - p[0] - p[1] - p[2])
        for i in range(4, 7):
            g_acc(i)
        if mode == 'first':
            md_s[3] = d_prod(CL, 3)
            o_dx(t).start()
            o_wq.start()
            o_wo.start()
        elif mode == 'last':
            ob = o_b(c)
            for r in range(0, 512, 128):
                c11, c12, c21, c22 = _combine([gkv_a[r:r + 128, i * 256:(i + 1) * 256] for i in range(7)])
                ra = 512 + (r // 256) * 512 + r % 256
                gT_s[ra:ra + 128, :] = jnp.concatenate([c11, c12], axis=1)
                gT_s[ra + 256:ra + 384, :] = jnp.concatenate([c21, c22], axis=1)
            mg_s[0] = mg[0]
            mg_s[1] = gu_prod(c, 2)
            unfold(1)
            unfold(2)
            mg_s[2] = gu_prod(c, 3)
            o_dx(t).start()
            ob[0].start()
            o_wkv.start()
            o_wphi.start()
            cb = slice(c * FC, (c + 1) * FC)
            q4, q6 = gu_prod(c, 4), gu_prod(c, 6)
            c11, c12 = mg_s[0] + mg_s[2] + q4 + q6, q4 - mg_s[1]
            for j, o_v in enumerate((dwg_v, dwu_v)):
                js = slice(j * 128, (j + 1) * 128)
                o_v[0:256, cb] = jnp.concatenate([c11[:, js], c12[:, js]], axis=1).astype(bf16)
            for cpy in o_half(0):
                cpy.start()
            q1, q5 = gu_prod(c, 1), gu_prod(c, 5)
            c21, c22 = q1 + mg_s[2], q1 - mg_s[0] - mg_s[1] - q5
            for j, o_v in enumerate((dwg_v, dwu_v)):
                js = slice(j * 128, (j + 1) * 128)
                o_v[256:512, cb] = jnp.concatenate([c21[:, js], c22[:, js]], axis=1).astype(bf16)
            for cpy in o_half(1):
                cpy.start()
        else:
            gu_store(c, mg + [gu_prod(c, i) for i in range(1, 7)])
            o_dx(t).start()
            for cpy in o_b(c):
                cpy.start()

    def p3_body(c, carry):
        phase3(c + 1, c, 'mid')
        return carry

    phase3(0, None, 'first')
    jax.lax.fori_loop(0, NTILE - 2, p3_body, 0)
    phase3(NTILE - 1, NTILE - 2, 'last')

    o_out.wait()
    o_wq.wait()
    o_wo.wait()
    for t in range(NTILE):
        o_dx(t).wait()
    o_wkv.wait()
    o_wphi.wait()
    for c in range(F // FC):
        for cpy in o_b(c):
            cpy.wait()
    for cpy in o_half(0) + o_half(1):
        cpy.wait()


@jax.jit
def pallas_parallel_sum__linear_kernel_hedgehog__glu_gated_bilinear__prompt_kernel(
        A_x, A_wqkv, A_w_phi, A_wo, B_x, B_w_gate, B_w_up, B_w_down, grad_out):
    x = A_x.reshape(S, D)
    dout = grad_out.reshape(S, D)
    wphi = jnp.transpose(A_w_phi, (1, 2, 0))
    sds = jax.ShapeDtypeStruct
    io_shapes = ((S, D), (S, D), (D, 3 * D), (DH, DH, H), (D, D), (D, F), (D, F), (F, D))
    any_spec = pl.BlockSpec(memory_space=pl.ANY)

    def packed(r, c):
        return pltpu.VMEM((r // 2, c), u32)

    io_scratch = [pltpu.VMEM(s, bf16) if len(s) == 3 else packed(*s) for s in io_shapes]
    dma = pltpu.SemaphoreType.DMA
    outs = pl.pallas_call(
        kernel,
        out_shape=tuple(sds(s, bf16) for s in io_shapes),
        in_specs=[any_spec] * 8,
        out_specs=tuple([any_spec] * 8),
        scratch_shapes=io_scratch + io_scratch + [
            packed(3 * D, D),
            packed(D, D),
            packed(128, 512),
            packed(S, D),
            packed(NG * 128, S),
            packed(NG * 80, S),
            packed(80, NG * 128),
            packed(128, NG * 128),
            packed(80, NG * 128),
            packed(128, NG * 128),
            packed(S // 2, 7 * 896),
            packed(S // 2, 14 * 896),
            packed(NTILE * 640, 256),
            packed(7 * 256, S // 2),
            packed(NTILE * 640, 256),
            packed(7 * 256, S // 2),
            packed(25 * 256, 256),
            packed(25 * 128, 256),
            packed(10 * 256, 256),
            packed(10 * 128, 256),
            packed(512, 256),
            packed(512, 256),
            packed(5 * 512, 256),
            packed(512, 7 * 128),
            packed(20 * 256, 256),
            packed(256, 14 * 128),
            packed(T, D),
            packed(640, 256),
            pltpu.VMEM((S, 1), f32),
            pltpu.VMEM((80, NG * 128), f32),
            pltpu.VMEM((80, NG * 128), f32),
            pltpu.VMEM((3 * D, D), f32),
            pltpu.VMEM((D, D), f32),
            pltpu.VMEM((S, D), f32),
            pltpu.VMEM((S, D), f32),
            pltpu.VMEM((128, 512), f32),
            pltpu.VMEM((3, 256, 256), f32),
            pltpu.VMEM((512, 7 * 256), f32),
            pltpu.VMEM((256, 14 * 256), f32),
            pltpu.VMEM((4, 256, 128), f32),
            dma((12,)),
        ],
        compiler_params=pltpu.CompilerParams(vmem_limit_bytes=126 * 1024 * 1024),
    )(x, A_wqkv, wphi, A_wo, B_w_gate, B_w_up, B_w_down, dout)
    out, dx, dwqkv, dwphi, dwo, dwg, dwu, dwd = outs
    return (out.reshape(1, S, D), dx.reshape(1, S, D), dwqkv, jnp.transpose(dwphi, (2, 0, 1)), dwo, dwg, dwu, dwd)
```
